```python
import jax
import jax.numpy as jnp

def _softmax(x, axis=-1):
    return jax.nn.softmax(x, axis=axis)
def _gelu(x):
    return jax.nn.gelu(x, approximate=True)
def _silu(x):
    return jax.nn.silu(x)
def _sigmoid(x):
    return jax.nn.sigmoid(x)
def _layernorm(x, axis=-1, eps=1e-5):
    m = jnp.mean(x, axis=axis, keepdims=True)
    v = jnp.var(x, axis=axis, keepdims=True)
    return (x - m) / jnp.sqrt(v + eps)
def _scatter_add(tgt, idx, src, axis=0):
    return tgt.at[idx].add(src)
def _segment_sum(src, seg, n):
    return jax.ops.segment_sum(src, seg, n)
class _Rng:
    def __init__(self, key):
        self._k = key
    def _next(self):
        self._k, sub = jax.random.split(self._k)
        return sub
    def normal(self, shape):
        return jax.random.normal(self._next(), shape, dtype=jnp.bfloat16)
    def randint(self, lo, hi, shape):
        return jax.random.randint(self._next(), shape, lo, hi, dtype=jnp.int32)
    def uniform(self, shape, lo=0.0, hi=1.0):
        return jax.random.uniform(self._next(), shape, jnp.bfloat16, lo, hi)
    def permutation(self, n):
        return jax.random.permutation(self._next(), n)


kernel_name = 'interleave_layers__sliding_block_cached__glu_gated_glu__decode'

def setup_inputs():
    _rng = _Rng(jax.random.key(int.from_bytes(__import__("os").urandom(4), "little")))
    _w = (lambda a: (lambda t: t.astype(jnp.bfloat16) if jnp.issubdtype(t.dtype, jnp.floating) else t)(jnp.asarray(a)))
    def _A_setup():
        B, Sq, D = 1, 1, 640
        Hq, Hkv, Sk, Dh = 32, 32, 32768, 192
        assert Hq % Hkv == 0, (Hq, Hkv)
        return {
            "x": _w((lambda *s: _rng.normal(s) * 0.05)(B, Sq, D)),
            "k_cache": _w((lambda *s: _rng.normal(s) * 0.05)(B, Hkv, Sk, Dh)),
            "v_cache": _w((lambda *s: _rng.normal(s) * 0.05)(B, Hkv, Sk, Dh)),
            "wq": _w((lambda *s: _rng.normal(s) * 0.05)(D, Hq * Dh) * (D ** -0.5)),
            "wo": _w((lambda *s: _rng.normal(s) * 0.05)(Hq * Dh, D) * ((Hq * Dh) ** -0.5)),
        }
    _A_in = _A_setup()

    def _B_setup():
        B, S, D, F = 1, 1, 640, 1536
        return {
            "x": _w((lambda *s: _rng.normal(s) * 0.05)(B, S, D)),
            "w_gate": _w((lambda *s: _rng.normal(s) * 0.05)(D, F)),
            "w_up": _w((lambda *s: _rng.normal(s) * 0.05)(D, F)),
            "w_down": _w((lambda *s: _rng.normal(s) * 0.05)(F, D)),
        }
    _B_in = _B_setup()

    return {
        "A_x": _A_in["x"],
        "A_k_cache": _A_in["k_cache"],
        "A_v_cache": _A_in["v_cache"],
        "A_wq": _A_in["wq"],
        "A_wo": _A_in["wo"],
        "B_x": _B_in["x"],
        "B_w_gate": _B_in["w_gate"],
        "B_w_up": _B_in["w_up"],
        "B_w_down": _B_in["w_down"],
    }

def reference(A_x, A_k_cache, A_v_cache, A_wq, A_wo, B_x, B_w_gate, B_w_up, B_w_down):
    def _A_ref(x, k_cache, v_cache, wq, wo):
        B, Sq, D = x.shape
        Hq, Dh = 32, 192
        Hkv, Sk = k_cache.shape[1], k_cache.shape[2]
        W = min(4096, max(256, Sk // 4))
        rep = Hq // Hkv
        q = (lambda x, *d: x.transpose(*d))((x @ wq).reshape(B, Sq, Hq, Dh), 0, 2, 1, 3)
        k = jnp.repeat(k_cache[:, :, Sk - W:, :], rep, axis=1)
        v = jnp.repeat(v_cache[:, :, Sk - W:, :], rep, axis=1)
        scores = jnp.einsum("bhqd,bhkd->bhqk", q, k) * (Dh ** -0.5)
        p = _softmax(scores, axis=-1)
        o = jnp.einsum("bhqk,bhkd->bhqd", p, v)
        return (lambda x, *d: x.transpose(*d))(o, 0, 2, 1, 3).reshape(B, Sq, Hq * Dh) @ wo

    def _B_ref(x, w_gate, w_up, w_down):
        g = jnp.einsum("bsd,df->bsf", x, w_gate)
        u = jnp.einsum("bsd,df->bsf", x, w_up)
        h = _sigmoid(g) * u
        return jnp.einsum("bsf,fd->bsd", h, w_down)

    x = A_x
    x = x + _A_ref(_layernorm(x, axis=-1), A_k_cache, A_v_cache, A_wq, A_wo)
    x = x + _B_ref(_layernorm(x, axis=-1), B_w_gate, B_w_up, B_w_down)
    x = x + _A_ref(_layernorm(x, axis=-1), A_k_cache, A_v_cache, A_wq, A_wo)
    x = x + _B_ref(_layernorm(x, axis=-1), B_w_gate, B_w_up, B_w_down)
    return x
```

```python
import jax
import jax.numpy as jnp
from jax import lax
import jax.experimental.pallas as pl
import jax.experimental.pallas.tpu as pltpu

D = 640
H = 32
DH = 192
F = 1536
SK = 32768
WIN = min(4096, max(256, SK // 4))
EPS = 1e-5

NC = D // 128
RT = DH // 8
NRT = H * RT
NJ = WIN // 256
NQB = H * DH // 256
NFB = F // 256
V_SPLIT = 24

RS = 2
LAG = 3
LEAD = 3

f32, bf16, u32 = jnp.float32, jnp.bfloat16, jnp.uint32


def _iota(axis):
    return lax.broadcasted_iota(jnp.int32, (8, 128), axis)


def _dot(a, b):
    return jnp.dot(a, b, preferred_element_type=f32)


def _packed(words):
    return pltpu.bitcast(words.reshape(words.shape[0] * 8, 128), bf16)


def _row(x, r):
    return jnp.broadcast_to(x[r:r + 1, :], (8, 128))


def _spread(x, half):
    lane = _iota(1)
    return jnp.take_along_axis(x, (lane // 16) * 8 + lane % 8 + 64 * half, axis=1)


def _split_parity(x):
    keep = (_iota(0) % 2) == ((_iota(1) // 8) % 2)
    return jnp.where(keep, x, 0.0).astype(bf16)


def _layernorm_lhs(x):
    valid = _iota(0) < NC
    mean = jnp.sum(x, keepdims=True) * (1.0 / D)
    xc = jnp.where(valid, x - mean, 0.0)
    var = jnp.sum(xc * xc, keepdims=True) * (1.0 / D)
    xn = xc * lax.rsqrt(var + EPS)
    halves = (_spread(xn, 0), _spread(xn, 1))
    return jnp.concatenate(
        [_split_parity(_row(halves[u % 2], u // 2)) for u in range(2 * NC)], axis=1)


def _stack_rows(rows):
    out = jnp.zeros((8, 128), f32)
    for c, r in enumerate(rows):
        out = jnp.where(_iota(0) == c, r, out)
    return out


def _kernel(x_hbm, k_hbm, v_hbm, wq_hbm, wo_hbm, wg_hbm, wu_hbm, wd_hbm, out_ref,
            x_buf, k_buf, v_buf, wq_buf, wo_buf, wg_buf, wu_buf, wd_buf,
            xl_buf, q_buf, ql_buf, p_buf, inv_buf, y_buf, sems):
    k32, v32 = k_buf.bitcast(u32), v_buf.bitcast(u32)
    wq32, wg32, wu32 = wq_buf.bitcast(u32), wg_buf.bitcast(u32), wu_buf.bitcast(u32)

    win = pl.ds((SK - WIN) // 16, WIN // 16)
    vs = V_SPLIT * RT
    cols = [pl.ds(c * 128, 128) for c in range(NC)]
    copies = {}

    def copy(name, src, dst):
        copies[name] = pltpu.make_async_copy(src, dst, sems.at[len(copies)])

    copy("x", x_hbm, x_buf)
    copy("wq", wq_hbm, wq_buf)
    for c in range(NC):
        copy(("wo", c), wo_hbm.at[:, cols[c]], wo_buf.at[c])
    copy("k", k_hbm.at[:, win, :], k_buf.at[pl.ds(0, NRT)])
    copy("v0", v_hbm.at[pl.ds(0, vs), win, :], v_buf.at[pl.ds(0, vs)])
    copy("v1", v_hbm.at[pl.ds(vs, NRT - vs), win, :], v_buf.at[pl.ds(vs, NRT - vs)])
    copy("wg", wg_hbm, wg_buf)
    copy("wu", wu_hbm, wu_buf)
    for c in range(NC):
        copy(("wd", c), wd_hbm.at[:, cols[c]], wd_buf.at[c])
    for cp in copies.values():
        cp.start()

    def wait(cond, *names):
        @pl.when(cond)
        def _():
            for name in names:
                copies[name].wait()


    def q_jobs(b):
        def job():
            r = _dot(xl_buf[...], _packed(wq32[:, pl.ds(pl.multiple_of(8 * b, 8), 8), :]))

            def drain():
                q_buf[b] = r
            return drain
        return [(2 * NC, job)]

    def q_lhs(h):
        for t in range(3):
            g = 3 * h + t
            q = jnp.broadcast_to(q_buf[g // 4, pl.ds((g // 2) % 2, 1), :], (8, 128))
            ql_buf[h % 2, t] = _split_parity(_spread(q, g % 2))

    def qk_jobs(h):
        def make(j, t):
            def job():
                w = _packed(k32[pl.ds(h * RT + 8 * t, 8), pl.ds(8 * j, 8), :])
                r = pltpu.bitcast(_dot(ql_buf[h % 2, t], w), u32)

                def drain():
                    lo = 2 * (j % 4)
                    v32[NRT + h % 2, pl.ds(32 * t + 2 * j, 2), :] = r[lo:lo + 2, :]
                return drain
            return (1, job)
        return [make(j, t) for j in range(NJ) for t in range(3)]

    def softmax(h):
        parts = [pltpu.bitcast(v32[NRT + h % 2, pl.ds(32 * t, 32), :], f32) for t in range(3)]
        s = (parts[0] + parts[1] + parts[2]) * (DH ** -0.5)
        p = jnp.exp(s - jnp.max(s, keepdims=True))
        inv_buf[h % 4] = jnp.broadcast_to(1.0 / jnp.sum(p, keepdims=True), (8, 128))
        for c in range(2 * NJ):
            p_buf[h % 2, c] = _row(p, c)

    def pv_step(h, g):
        acc = [None] * RS
        for j in range(NJ):
            p0, p1 = p_buf[h % 2, 2 * j], p_buf[h % 2, 2 * j + 1]
            for r in range(RS):
                v = v_buf[h * RT + g * RS + r, pl.ds(16 * j, 16), :].astype(f32)
                t = v[0:8] * p0 + v[8:16] * p1
                acc[r] = t if acc[r] is None else acc[r] + t
        for r in range(RS):
            rt = g * RS + r
            k32[NRT + 2 * (h % 2) + rt // 16, pl.ds(8 * (rt % 16), 8), :] = (
                pltpu.bitcast(acc[r], u32))

    def head_out(h):
        out = []
        for part, n in ((0, 128), (1, DH - 128)):
            a = pltpu.bitcast(k32[NRT + 2 * (h % 2) + part, pl.ds(0, n), :], f32).T
            a = a.reshape(16, 8, n).sum(axis=0) * inv_buf[h % 4][:, :n]
            out.append(a.astype(bf16))
        return jnp.concatenate(out, axis=1)

    def wo_jobs(h, o, first):
        def make(c):
            def job():
                r = _dot(o, wo_buf[c, pl.ds(pl.multiple_of(h * DH, DH), DH), :])

                def drain():
                    y_buf[c] = r if first else y_buf[c] + r
                return drain
            return (2, job)
        return [make(c) for c in range(NC)]

    def stage(qb=None, lhs=None, qk=None, sm=None, pv=None, wo=None, first=False):
        jobs = []
        if qb is not None:
            jobs += q_jobs(qb)
        if qk is not None:
            jobs += qk_jobs(qk)
        if wo is not None:
            jobs += wo_jobs(wo, head_out(wo), first)
        if sm is not None:
            softmax(sm)
        if pv is None:
            for drain in [job() for _, job in jobs]:
                drain()
        else:
            steps = RT // RS
            total = sum(n for n, _ in jobs)
            groups, seen = [[] for _ in range(steps)], 0
            for n, job in jobs:
                groups[seen * steps // total].append(job)
                seen += n
            pending = {}

            def issue(g):
                pending[g] = [job() for job in groups[g]]

            def flush(g):
                for drain in pending.pop(g):
                    drain()

            for g in range(LEAD):
                issue(g)
            for g in range(steps):
                if g >= LAG:
                    flush(g - LAG)
                pv_step(pv, g)
                if g + LEAD < steps:
                    issue(g + LEAD)
            for g in range(steps - LAG, steps):
                flush(g)
        if lhs is not None:
            q_lhs(lhs)

    def attention(x, cold):
        xl_buf[...] = _layernorm_lhs(x)
        wait(cold, "wq", *[("wo", c) for c in range(NC)], "k")
        stage(qb=0, lhs=0)
        stage(qb=1, lhs=1, qk=0)
        stage(qb=2, lhs=2, qk=1, sm=0)
        wait(cold, "v0")
        stage(qb=3, lhs=3, qk=2, sm=1, pv=0)
        y_buf[...] = jnp.zeros(y_buf.shape, f32)

        def body(i, carry):
            wait(jnp.logical_and(cold, i == V_SPLIT), "v1")
            stage(qb=jnp.minimum(i + 3, NQB - 1), lhs=jnp.minimum(i + 3, H - 1),
                  qk=i + 2, sm=i + 1, pv=i, wo=i - 1)
            return carry

        lax.fori_loop(1, H - 2, body, 0)
        stage(sm=H - 1, pv=H - 2, wo=H - 3)
        stage(pv=H - 1, wo=H - 2)
        stage(wo=H - 1)
        return x + _stack_rows(
            [jnp.broadcast_to(jnp.sum(y_buf[c], axis=0, keepdims=True), (8, 128))
             for c in range(NC)])

    def glu(x, cold):
        xl = _layernorm_lhs(x)
        wait(cold, "wg", "wu")
        hid = []
        for b in range(NFB):
            g = _dot(xl, _packed(wg32[:, pl.ds(8 * b, 8), :]))
            u = _dot(xl, _packed(wu32[:, pl.ds(8 * b, 8), :]))
            hid.append((jax.nn.sigmoid(g) * u).astype(bf16))
        hid = jnp.concatenate(hid, axis=1)
        pending = {}
        for c in range(NC):
            wait(cold, ("wd", c))
            even, odd = [
                _dot(hid, jnp.concatenate(
                    [wd_buf[c, pl.ds(256 * b + 128 * par, 128), :] for b in range(NFB)], axis=0))
                for par in range(2)]
            pending[c] = _row(even, 0) + _row(odd, 1)
        return x + _stack_rows([pending[c] for c in range(NC)])

    copies["x"].wait()
    x_in = x_buf[...].astype(f32)
    x0 = _stack_rows([jnp.broadcast_to(x_in[:, c * 128:(c + 1) * 128], (8, 128))
                      for c in range(NC)])

    def layer(i, x):
        return glu(attention(x, i == 0), i == 0)

    x_out = lax.fori_loop(0, 2, layer, x0)
    out_ref[...] = jnp.concatenate(
        [x_out[c:c + 1, :] for c in range(NC)], axis=1).astype(out_ref.dtype)


def _tile_order(w):
    r, c = w.shape
    w = w.reshape(r // 8, 8, c // 128, 128)
    return jnp.transpose(w, (0, 2, 1, 3)).reshape(r // 8, c // 16, 128)


@jax.jit
def pallas_interleave_layers__sliding_block_cached__glu_gated_glu__decode_kernel(
    A_x: jax.Array,
    A_k_cache: jax.Array,
    A_v_cache: jax.Array,
    A_wq: jax.Array,
    A_wo: jax.Array,
    B_x: jax.Array,
    B_w_gate: jax.Array,
    B_w_up: jax.Array,
    B_w_down: jax.Array,
):
    del B_x
    k = _tile_order(jnp.swapaxes(A_k_cache, 2, 3).reshape(H * DH, SK))
    v = _tile_order(jnp.swapaxes(A_v_cache, 2, 3).reshape(H * DH, SK))
    out = pl.pallas_call(
        _kernel,
        out_shape=jax.ShapeDtypeStruct((1, D), A_x.dtype),
        in_specs=[pl.BlockSpec(memory_space=pltpu.HBM)] * 8,
        out_specs=pl.BlockSpec(memory_space=pltpu.VMEM),
        scratch_shapes=[
            pltpu.VMEM((1, D), bf16),
            pltpu.VMEM((NRT + 4, WIN // 16, 128), bf16),
            pltpu.VMEM((NRT + 2, WIN // 16, 128), bf16),
            pltpu.VMEM((D // 8, H * DH // 16, 128), bf16),
            pltpu.VMEM((NC, H * DH, 128), bf16),
            pltpu.VMEM((D // 8, F // 16, 128), bf16),
            pltpu.VMEM((D // 8, F // 16, 128), bf16),
            pltpu.VMEM((NC, F, 128), bf16),
            pltpu.VMEM((8, 2 * D), bf16),
            pltpu.VMEM((NQB, 8, 128), f32),
            pltpu.VMEM((2, 3, 8, 128), bf16),
            pltpu.VMEM((2, 2 * NJ, 8, 128), f32),
            pltpu.VMEM((4, 8, 128), f32),
            pltpu.VMEM((NC, 8, 128), f32),
            pltpu.SemaphoreType.DMA((7 + 2 * NC,)),
        ],
        compiler_params=pltpu.CompilerParams(vmem_limit_bytes=124 * 1024 * 1024),
    )(A_x.reshape(1, D), k, v, _tile_order(A_wq), A_wo,
      _tile_order(B_w_gate), _tile_order(B_w_up), B_w_down)
    return out.reshape(A_x.shape)
```

```python
import jax
import jax.numpy as jnp
from jax import lax
import jax.experimental.pallas as pl
import jax.experimental.pallas.tpu as pltpu

D = 640
H = 32
DH = 192
F = 1536
SK = 32768
WIN = min(4096, max(256, SK // 4))
EPS = 1e-5

NC = D // 128
RT = DH // 8
NRT = H * RT
NJ = WIN // 256
NQB = H * DH // 256
NFB = F // 256
W_ROWS = D * H * DH // (256 * 128)
WQ_ROW = NRT
WO_ROW = WQ_ROW + W_ROWS
A_ROW = WO_ROW + W_ROWS
P_ROW = A_ROW + 3
S_ROW = NRT
Q_ROW = S_ROW + 2
Y_ROW = Q_ROW + 2
V_SPLIT = 24

RS = 4
JS = 8
SM = 3
EX0 = 3
OUT0, OUTS = 0, 2
QS = 5
DELAY = 0
LAG = 4
LEAD = 3

f32, bf16, u32 = jnp.float32, jnp.bfloat16, jnp.uint32


def _iota(axis):
    return lax.broadcasted_iota(jnp.int32, (8, 128), axis)


def _operand(x):
    return jnp.concatenate([x, x], axis=0).astype(bf16)


def _dot(a, b):
    return jnp.dot(a, b, preferred_element_type=f32)[0:8]


def _packed(words):
    return pltpu.bitcast(words.reshape(words.shape[0] * 8, 128), bf16)


def _row(x, r):
    return jnp.broadcast_to(x[r:r + 1, :], (8, 128))


def _spread(x, half):
    lane = _iota(1)
    return jnp.take_along_axis(x, (lane // 16) * 8 + lane % 8 + 64 * half, axis=1)


def _split_parity(x):
    keep = (_iota(0) % 2) == ((_iota(1) // 8) % 2)
    return _operand(jnp.where(keep, x, 0.0))


def _layernorm_lhs(x):
    valid = _iota(0) < NC
    mean = jnp.sum(x, keepdims=True) * (1.0 / D)
    xc = jnp.where(valid, x - mean, 0.0)
    var = jnp.sum(xc * xc, keepdims=True) * (1.0 / D)
    xn = xc * lax.rsqrt(var + EPS)
    halves = (_spread(xn, 0), _spread(xn, 1))
    return [_split_parity(_row(halves[u % 2], u // 2)) for u in range(2 * NC)]


def _stack_rows(rows):
    out = jnp.zeros((8, 128), f32)
    for c, r in enumerate(rows):
        out = jnp.where(_iota(0) == c, r, out)
    return out


def _kernel(x_hbm, k_hbm, v_hbm, wq_hbm, wo_hbm, wg_hbm, wu_hbm, wd_hbm, out_ref,
            x_buf, k_buf, v_buf, wg_buf, wu_buf, wd_buf,
            xl_buf, q_buf, ql_buf, ol_buf, inv_buf, sems):
    k32, v32 = k_buf.bitcast(u32), v_buf.bitcast(u32)
    wg32, wu32 = wg_buf.bitcast(u32), wu_buf.bitcast(u32)

    win = pl.ds((SK - WIN) // 16, WIN // 16)
    vs = V_SPLIT * RT
    cols = [pl.ds(c * 128, 128) for c in range(NC)]
    copies = {}

    def copy(name, src, dst):
        copies[name] = pltpu.make_async_copy(src, dst, sems.at[len(copies)])

    copy("x", x_hbm, x_buf)
    copy("wq", wq_hbm, k_buf.at[pl.ds(WQ_ROW, W_ROWS)])
    for c in range(NC):
        copy(("wo", c), wo_hbm.at[:, :, cols[c]],
             k_buf.at[pl.ds(WO_ROW + c * W_ROWS // NC, W_ROWS // NC)])
    copy("k", k_hbm.at[:, win, :], k_buf.at[pl.ds(0, NRT)])
    copy("v0", v_hbm.at[pl.ds(0, vs), win, :], v_buf.at[pl.ds(0, vs)])
    copy("v1", v_hbm.at[pl.ds(vs, NRT - vs), win, :], v_buf.at[pl.ds(vs, NRT - vs)])
    copy("wg", wg_hbm, wg_buf)
    copy("wu", wu_hbm, wu_buf)
    for c in range(NC):
        copy(("wd", c), wd_hbm.at[:, cols[c]], wd_buf.at[c])
    for cp in copies.values():
        cp.start()

    def wait(cond, *names):
        @pl.when(cond)
        def _():
            for name in names:
                copies[name].wait()


    def put(ref, row, i, x):
        ref[row + i // 16, pl.ds(8 * (i % 16), 8), :] = pltpu.bitcast(x, u32)

    def get(ref, row, i):
        return pltpu.bitcast(ref[row + i // 16, pl.ds(8 * (i % 16), 8), :], f32)

    def q_jobs(b, slot):
        at = [(WQ_ROW + (i >> 4), pl.ds(pl.multiple_of(8 * (i & 15), 8), 8)) for i in (b, b + NQB)]

        def make(u):
            def job():
                w = [k32[at[a % 2][0] + 3 * (a // 2), at[a % 2][1], :]
                     for a in range(8 * u, 8 * u + 8)]
                r = _dot(xl_buf[u], pltpu.bitcast(jnp.concatenate(w, axis=0), bf16))

                def drain():
                    put(v32, Q_ROW + slot, u, r)
                return drain
            return job
        return [make(u) for u in range(2 * NC)]

    def q_sum(b, slot, zero):
        parts = pltpu.bitcast(v32[zero + Q_ROW + slot, pl.ds(0, 16 * NC), :], f32)
        q_buf[b] = parts.reshape(2 * NC, 8, 128).sum(axis=0)

    def q_lhs(n, e):
        for t in range(3):
            m = 3 * n + (3 * e + t) // 2
            q = jnp.broadcast_to(q_buf[m >> 1, pl.ds(m & 1, 1), :], (8, 128))
            ql_buf[e, t] = _split_parity(_spread(q, (3 * e + t) % 2))

    def qk_jobs(n, e):
        def make(j, t):
            def job():
                w = _packed(k32[pl.ds(n * 2 * RT + e * RT + 8 * t, 8), pl.ds(8 * j, 8), :])
                r = pltpu.bitcast(_dot(ql_buf[e, t], w), u32)

                def drain():
                    lo = 2 * (j % 4)
                    v32[S_ROW + e, pl.ds(32 * t + 2 * j, 2), :] = r[lo:lo + 2, :]
                return drain
            return job
        return [make(j, t) for j in range(NJ) for t in range(3)]

    dense = {}

    def softmax(e, slot, zero):
        parts = [pltpu.bitcast(v32[zero + S_ROW + e, pl.ds(32 * t, 32), :], f32)
                 for t in range(3)]
        s = (parts[0] + parts[1] + parts[2]) * (DH ** -0.5)
        p = jnp.exp(s - jnp.max(s, keepdims=True))
        inv_buf[slot] = jnp.broadcast_to(1.0 / jnp.sum(p, keepdims=True), (8, 128))
        dense[e] = p

    def expand(e, part, zero):
        p = dense[e][8 * part:8 * part + 8]
        for c in range(8):
            put(k32, P_ROW + 2 * e, 8 * part + c, _row(p, c))

    def pv_steps(n, e):
        acc = [None] * RS

        def make(r0, j0):
            def step():
                for j in range(j0, j0 + JS):
                    p0, p1 = get(k32, P_ROW + 2 * e, 2 * j), get(k32, P_ROW + 2 * e, 2 * j + 1)
                    for r in range(RS):
                        row = n * 2 * RT + e * RT + r0 + r
                        v = v_buf[row, pl.ds(16 * j, 16), :].astype(f32)
                        t = v[0:8] * p0 + v[8:16] * p1
                        acc[r] = t if j == 0 else acc[r] + t
                done = list(acc)

                def drain():
                    for r in range(RS):
                        put(k32, A_ROW, e * RT + r0 + r, done[r])
                return drain
            return step
        return [make(r0, j0) for r0 in range(0, RT, RS) for j0 in range(0, NJ, JS)]

    def pair_out(t, zero):
        inv = (inv_buf[0] if t == 0 else inv_buf[1] if t == 2 else
               jnp.where(_iota(1) < DH - 128, inv_buf[0], inv_buf[1]))
        a = pltpu.bitcast(k32[zero + A_ROW + t], f32).T
        ol_buf[t] = _operand(a.reshape(16, 8, 128).sum(axis=0) * inv)

    def wo_jobs(n):
        def make(t, c):
            def job():
                i = 3 * n + t
                w = k32[WO_ROW + c * W_ROWS // NC + (i >> 1),
                         pl.ds(pl.multiple_of(64 * (i & 1), 64), 64), :]
                r = _dot(ol_buf[t], pltpu.bitcast(w, bf16))

                def drain():
                    put(v32, Y_ROW, c, get(v32, Y_ROW, c) + r)
                return drain
            return job
        return [make(t, c) for t in range(3) for c in range(NC)]

    def run(jobs):
        for drain in [job() for job in jobs]:
            drain()

    def interleave(jobs, steps, hooks):
        ns = len(steps)
        groups = [[job for job in jobs[g * len(jobs) // ns:(g + 1) * len(jobs) // ns] if job]
                  for g in range(ns)]
        pending = {g: [job() for job in groups[g]] for g in range(LEAD)}
        previous = None
        for g, step in enumerate(steps):
            for drain in pending.pop(g - LAG, ()):
                drain()
            for hook in hooks.get(g, ()):
                hook()
            current = step()
            if DELAY:
                current, previous = previous, current
            if current is not None:
                current()
            if g + LEAD < ns:
                pending[g + LEAD] = [job() for job in groups[g + LEAD]]
        if previous is not None:
            previous()
        for g in sorted(pending):
            for drain in pending[g]:
                drain()

    def pair(n, first=False, last=False):
        zero = n >> 8
        half = (RT // RS) * (NJ // JS)
        jobs, hooks = [], {}

        def at(g, fn, *args):
            hooks.setdefault(g, []).append(lambda: fn(*args))

        if not first:
            for t in range(3):
                at(OUT0 + t * OUTS, pair_out, t, zero)
        at(SM, softmax, 1, 2, zero)
        for part in range(4):
            at(SM + EX0 + part, expand, 1, part, zero)

        def rotate():
            inv_buf[0] = inv_buf[3]
            inv_buf[1] = inv_buf[2]
        at(half, rotate)
        if not last:
            blocks = [jnp.minimum(2 * n + 3 + i, NQB - 1) for i in range(2)]
            q_lhs(n + 1, 1)
            jobs += qk_jobs(n + 1, 0) + q_jobs(blocks[0], 0) + q_jobs(blocks[1], 1)
            jobs += qk_jobs(n + 1, 1)
            at(half + SM, softmax, 0, 3, zero)
            for part in range(4):
                at(half + SM + EX0 + part, expand, 0, part, zero)
            for i in range(2):
                at(2 * half - QS + i, q_sum, blocks[i], i, zero)
            at(2 * half - QS + 2, q_lhs, jnp.minimum(n + 2, H // 2 - 1), 0)
        else:
            jobs += [None] * (3 * NC)
        if not first:
            jobs += wo_jobs(n - 1)
        interleave(jobs, pv_steps(n, 0) + pv_steps(n, 1), hooks)

    def attention(x, cold, zero):
        for u, tile in enumerate(_layernorm_lhs(x)):
            xl_buf[u] = tile
        for c in range(NC):
            put(v32, Y_ROW, c, jnp.zeros((8, 128), f32))
        wait(cold, "wq", *[("wo", c) for c in range(NC)], "k")
        run(q_jobs(0, 0) + q_jobs(1, 1))
        q_sum(0, 0, 0)
        q_lhs(0, 0)
        q_sum(1, 1, 0)
        q_lhs(0, 1)
        run(qk_jobs(0, 0))
        softmax(0, 3, 0)
        for part in range(4):
            expand(0, part, 0)
        run(q_jobs(2, 0) + qk_jobs(0, 1))
        q_sum(2, 0, 0)
        q_lhs(1, 0)
        wait(cold, "v0")
        pair(zero, first=True)

        def body(n, carry):
            wait(jnp.logical_and(cold, n == V_SPLIT // 2), "v1")
            pair(n)
            return carry

        lax.fori_loop(1, H // 2 - 1, body, 0)
        pair(zero + (H // 2 - 1), last=True)
        for t in range(3):
            pair_out(t, 0)
        run(wo_jobs(H // 2 - 1))
        return x + _stack_rows(
            [jnp.broadcast_to(jnp.sum(get(v32, Y_ROW, c), axis=0, keepdims=True), (8, 128))
             for c in range(NC)])

    def glu(x, cold):
        xl = jnp.concatenate(_layernorm_lhs(x), axis=1)
        wait(cold, "wg", "wu")
        hid = []
        for b in range(NFB):
            g = _dot(xl, _packed(wg32[:, pl.ds(8 * b, 8), :]))
            u = _dot(xl, _packed(wu32[:, pl.ds(8 * b, 8), :]))
            hid.append(_operand(jax.nn.sigmoid(g) * u))
        hid = jnp.concatenate(hid, axis=1)
        pending = {}
        for c in range(NC):
            wait(cold, ("wd", c))
            even, odd = [
                _dot(hid, jnp.concatenate(
                    [wd_buf[c, pl.ds(256 * b + 128 * par, 128), :] for b in range(NFB)], axis=0))
                for par in range(2)]
            pending[c] = _row(even, 0) + _row(odd, 1)
        return x + _stack_rows([pending[c] for c in range(NC)])

    copies["x"].wait()
    x_in = x_buf[...].astype(f32)
    x0 = _stack_rows([jnp.broadcast_to(x_in[:, c * 128:(c + 1) * 128], (8, 128))
                      for c in range(NC)])

    def layer(i, x):
        return glu(attention(x, i == 0, i >> 1), i == 0)

    x_out = lax.fori_loop(0, 2, layer, x0)
    out_ref[...] = jnp.concatenate(
        [x_out[c:c + 1, :] for c in range(NC)], axis=1).astype(out_ref.dtype)


def _tile_order(w):
    r, c = w.shape
    w = w.reshape(r // 8, 8, c // 128, 128)
    return jnp.transpose(w, (0, 2, 1, 3)).reshape(r // 8, c // 16, 128)


@jax.jit
def pallas_interleave_layers__sliding_block_cached__glu_gated_glu__decode_kernel(
    A_x: jax.Array,
    A_k_cache: jax.Array,
    A_v_cache: jax.Array,
    A_wq: jax.Array,
    A_wo: jax.Array,
    B_x: jax.Array,
    B_w_gate: jax.Array,
    B_w_up: jax.Array,
    B_w_down: jax.Array,
):
    del B_x
    k = _tile_order(jnp.swapaxes(A_k_cache, 2, 3).reshape(H * DH, SK))
    v = _tile_order(jnp.swapaxes(A_v_cache, 2, 3).reshape(H * DH, SK))
    out = pl.pallas_call(
        _kernel,
        out_shape=jax.ShapeDtypeStruct((1, D), A_x.dtype),
        in_specs=[pl.BlockSpec(memory_space=pltpu.HBM)] * 8,
        out_specs=pl.BlockSpec(memory_space=pltpu.VMEM),
        scratch_shapes=[
            pltpu.VMEM((1, D), bf16),
            pltpu.VMEM((P_ROW + 4, 256, 128), bf16),
            pltpu.VMEM((Y_ROW + 1, 256, 128), bf16),
            pltpu.VMEM((D // 8, F // 16, 128), bf16),
            pltpu.VMEM((D // 8, F // 16, 128), bf16),
            pltpu.VMEM((NC, F, 128), bf16),
            pltpu.VMEM((2 * NC, 16, 128), bf16),
            pltpu.VMEM((NQB, 8, 128), f32),
            pltpu.VMEM((2, 3, 16, 128), bf16),
            pltpu.VMEM((3, 16, 128), bf16),
            pltpu.VMEM((4, 8, 128), f32),
            pltpu.SemaphoreType.DMA((7 + 2 * NC,)),
        ],
        compiler_params=pltpu.CompilerParams(vmem_limit_bytes=124 * 1024 * 1024),
    )(A_x.reshape(1, D), k, v,
      _tile_order(A_wq).reshape(W_ROWS, 256, 128), A_wo.reshape(H * DH // 256, 256, D),
      _tile_order(B_w_gate), _tile_order(B_w_up), B_w_down)
    return out.reshape(A_x.shape)
```

```python
import jax
import jax.numpy as jnp
from jax import lax
import jax.experimental.pallas as pl
import jax.experimental.pallas.tpu as pltpu

D = 640
H = 32
DH = 192
F = 1536
SK = 32768
WIN = min(4096, max(256, SK // 4))
EPS = 1e-5

NC = D // 128
NP = H // 2
RT = DH // 8
NRT = H * RT
NJ = WIN // 256
NFB = F // 256
V_SPLIT = 24

WO_ROWS = H * DH // 256
WQ2_ROW = NRT
WQ1_ROW = WQ2_ROW + D // 8
WO_ROW = WQ1_ROW + D // 16
A_ROW = WO_ROW + NC * WO_ROWS
P_ROW = A_ROW + 2
S_ROW = NRT
Q_ROW = S_ROW + 2
Y_ROW = Q_ROW + 1

RS = 3
JS = 8
LAG = 4
LEAD = 3
SM = 1
PS = 7
EXN = 4
OUT0 = 6
QS = 22

f32, bf16, u32 = jnp.float32, jnp.bfloat16, jnp.uint32


def _iota(axis):
    return lax.broadcasted_iota(jnp.int32, (8, 128), axis)


def _operand(x):
    return jnp.concatenate([x, x], axis=0).astype(bf16)


def _dot(a, b):
    return jnp.dot(a, b, preferred_element_type=f32)[0:8]


def _packed(words):
    return pltpu.bitcast(words.reshape(words.shape[0] * 8, 128), bf16)


def _row(x, r):
    return jnp.broadcast_to(x[r:r + 1, :], (8, 128))


def _spread(x, half):
    lane = _iota(1)
    return jnp.take_along_axis(x, (lane // 16) * 8 + lane % 8 + 64 * half, axis=1)


def _split_parity(x):
    keep = (_iota(0) % 2) == ((_iota(1) // 8) % 2)
    return _operand(jnp.where(keep, x, 0.0))


def _layernorm(x):
    mean = jnp.sum(x, keepdims=True) * (1.0 / D)
    xc = jnp.where(_iota(0) < NC, x - mean, 0.0)
    var = jnp.sum(xc * xc, keepdims=True) * (1.0 / D)
    return xc * lax.rsqrt(var + EPS)


def _paired_operands(x):
    halves = (_spread(x, 0), _spread(x, 1))
    return [_split_parity(_row(halves[u % 2], u // 2)) for u in range(2 * NC)]


def _stack_rows(rows):
    out = jnp.zeros((8, 128), f32)
    for c, r in enumerate(rows):
        out = jnp.where(_iota(0) == c, r, out)
    return out


def _kernel(x_hbm, k_hbm, v_hbm, wq_hbm, wo_hbm, wg_hbm, wu_hbm, wd_hbm, out_ref,
            x_buf, k_buf, v_buf, wg_buf, wu_buf, wd_buf,
            xl_buf, q_buf, ql_buf, ol_buf, inv_buf, sems):
    k32, v32 = k_buf.bitcast(u32), v_buf.bitcast(u32)
    wg32, wu32 = wg_buf.bitcast(u32), wu_buf.bitcast(u32)

    win = pl.ds((SK - WIN) // 256, NJ)
    vs = V_SPLIT * RT
    cols = [pl.ds(c * 128, 128) for c in range(NC)]
    copies = {}

    def copy(name, src, dst):
        copies[name] = pltpu.make_async_copy(src, dst, sems.at[len(copies)])

    copy("x", x_hbm, x_buf)
    for i in range(2):
        copy(("wq", i), wq_hbm.at[:, i, :, pl.ds(0, 16), :],
             k_buf.at[pl.ds(WQ2_ROW + i * D // 16, D // 16)])
        copy(("wq", 2 + i), wq_hbm.at[:, i, :, pl.ds(16, 8), :],
             k_buf.at[pl.ds(WQ1_ROW, D // 16), :, pl.ds(8 * i, 8), :])
    for c in range(NC):
        copy(("wo", c), wo_hbm.at[:, :, :, cols[c]],
             k_buf.at[pl.ds(WO_ROW + c * WO_ROWS, WO_ROWS)])
    copy("k", k_hbm.at[:, win], k_buf.at[pl.ds(0, NRT)])
    copy("v0", v_hbm.at[pl.ds(0, vs), win], v_buf.at[pl.ds(0, vs)])
    copy("v1", v_hbm.at[pl.ds(vs, NRT - vs), win], v_buf.at[pl.ds(vs, NRT - vs)])
    copy("wg", wg_hbm, wg_buf)
    copy("wu", wu_hbm, wu_buf)
    for c in range(NC):
        copy(("wd", c), wd_hbm.at[:, cols[c]], wd_buf.at[c])
    for cp in copies.values():
        cp.start()

    def wait(cond, *names):
        @pl.when(cond)
        def _():
            for name in names:
                copies[name].wait()


    def put(ref, row, i, x):
        ref[row + i // 16, i % 16] = pltpu.bitcast(x, u32)

    def get(ref, row, i):
        return pltpu.bitcast(ref[row + i // 16, i % 16], f32)

    def q_jobs(n):
        def make(u):
            def job():
                if u < 2 * NC:
                    w = [k32[WQ2_ROW + (a % 2) * (D // 16) + a // 2, n]
                         for a in range(8 * u, 8 * u + 8)]
                    w = pltpu.bitcast(jnp.concatenate(w, axis=0), bf16)
                else:
                    w = _packed(k32[pl.ds(WQ1_ROW + 8 * (u - 2 * NC), 8), n])
                r = _dot(xl_buf[u], w)
                return lambda: put(v32, Q_ROW, u, r)
            return job
        return [make(u) for u in range(3 * NC)]

    def q_sum(zero):
        parts = pltpu.bitcast(v32[zero + Q_ROW, pl.ds(0, 3 * NC)], f32)
        q_buf[0] = parts[:2 * NC].sum(axis=0)
        q_buf[1] = parts[2 * NC:].sum(axis=0)

    def q_lhs(e):
        for t in range(3):
            m = (3 * e + t) // 2
            q = _row(q_buf[0], m) if m < 2 else q_buf[1]
            ql_buf[e, t] = _split_parity(_spread(q, (3 * e + t) % 2))

    def qk_jobs(n, e):
        def make(j, t):
            def job():
                w = _packed(k32[pl.ds(n * 2 * RT + e * RT + 8 * t, 8), j])
                r = pltpu.bitcast(_dot(ql_buf[e, t], w), u32)

                def drain():
                    lo = 2 * (j % 4)
                    v32[S_ROW + e, 4 * t + j // 4, pl.ds(lo, 2), :] = r[lo:lo + 2, :]
                return drain
            return job
        return [make(j, t) for j in range(NJ) for t in range(3)]

    def softmax(e, slot, zero):
        parts = pltpu.bitcast(v32[zero + S_ROW + e, pl.ds(0, 12)], f32)
        s = (parts[0:4] + parts[4:8] + parts[8:12]).reshape(32, 128) * (DH ** -0.5)
        p = jnp.exp(s - jnp.max(s, keepdims=True))
        inv_buf[slot] = jnp.broadcast_to(1.0 / jnp.sum(p, keepdims=True), (8, 128))

        def publish():
            for i in range(4):
                put(v32, S_ROW + e, 12 + i, p[8 * i:8 * i + 8])
        return publish

    def expand(e, part, zero):
        for c in range(32 * part // EXN, 32 * (part + 1) // EXN):
            row = pltpu.bitcast(v32[zero + S_ROW + e, 12 + c // 8, pl.ds(c % 8, 1), :], f32)
            put(k32, P_ROW + 2 * e, c, jnp.broadcast_to(row, (8, 128)))

    def pv_steps(n, e):
        acc = [None] * RS

        def make(r0, j0):
            def step():
                for j in range(j0, j0 + JS):
                    p0, p1 = get(k32, P_ROW + 2 * e, 2 * j), get(k32, P_ROW + 2 * e, 2 * j + 1)
                    for r in range(RS):
                        v = v_buf[n * 2 * RT + e * RT + r0 + r, j].astype(f32)
                        t = v[0:8] * p0 + v[8:16] * p1
                        acc[r] = t if j == 0 else acc[r] + t
                for r in range(RS):
                    rt = e * RT + r0 + r
                    k_buf[A_ROW + rt // 32, (rt // 2) % 16, pl.ds(8 * (rt % 2), 8), :] = (
                        acc[r].astype(bf16))
            return step
        return [make(r0, j0) for r0 in range(0, RT, RS) for j0 in range(0, NJ, JS)]

    def out_job(t, zero):
        def job():
            w = _packed(k32[zero + A_ROW + t // 2, pl.ds(8 * (t % 2), 8)])
            r = lax.dot_general(jnp.ones((16, 128), bf16), w, (((1,), (1,)), ((), ())),
                                preferred_element_type=f32)[0:8]
            return lambda: put(v32, Y_ROW, 8 + t, r)
        return job

    def normalise(t):
        inv = (inv_buf[0] if t == 0 else inv_buf[1] if t == 2 else
               jnp.where(_iota(1) < DH - 128, inv_buf[0], inv_buf[1]))
        ol_buf[t] = _operand(get(v32, Y_ROW, 8 + t) * inv)

    def wo_jobs(n):
        def make(t, c):
            def job():
                i = 3 * n + t
                w = _packed(k32[WO_ROW + c * WO_ROWS + (i >> 1), pl.ds(8 * (i & 1), 8)])
                r = _dot(ol_buf[t], w)
                return lambda: put(v32, Y_ROW, c, get(v32, Y_ROW, c) + r)
            return job
        return [make(t, c) for t in range(3) for c in range(NC)]

    def run(jobs):
        for drain in [job() for job in jobs]:
            drain()

    def interleave(jobs, steps, hooks):
        ns = len(steps)
        extra = len(jobs) - 4 * ns
        assert max(hooks) < ns and extra >= 0
        groups = [[job for job in jobs[4 * g + extra * (g > 0):4 * g + 4 + extra] if job]
                  for g in range(ns)]
        pending = {g: [job() for job in groups[g]] for g in range(LEAD)}
        for g, step in enumerate(steps):
            for drain in pending.pop(g - LAG, ()):
                drain()
            for hook in hooks.get(g, ()):
                hook()
            step()
            if g + LEAD < ns:
                pending[g + LEAD] = [job() for job in groups[g + LEAD]]
        for g in sorted(pending):
            for drain in pending[g]:
                drain()

    def pair(n, first=False, last=False):
        zero = n >> 8
        steps = pv_steps(n, 0) + pv_steps(n, 1)
        half = len(steps) // 2
        hooks = {}

        def at(g, fn, *args):
            hooks.setdefault(g, []).append(lambda: fn(*args))

        def softmax_at(g, e):
            result = []
            at(g, lambda: result.append(softmax(e, 3 - e, zero)))
            at(g + PS, lambda: result[0]())
            for part in range(EXN):
                at(g + PS + 1 + part, expand, e, part, zero)

        def rotate():
            inv_buf[0] = inv_buf[3]
            inv_buf[1] = inv_buf[2]

        softmax_at(SM, 1)
        at(half, rotate)
        head, tail = [None] * 3, [None] * (3 * NC)
        if not first:
            head, tail = [out_job(t, zero) for t in range(3)], wo_jobs(n - 1)
            for t in range(3):
                at(OUT0 + t, normalise, t)
        middle = [None] * (6 * NJ + 3 * NC)
        if not last:
            q_lhs(1)
            middle = qk_jobs(n + 1, 0) + q_jobs(jnp.minimum(n + 2, NP - 1)) + qk_jobs(n + 1, 1)
            softmax_at(half + SM, 0)
            at(QS, q_sum, zero)
            at(QS + 2, q_lhs, 0)
        interleave(head + middle + tail, steps, hooks)

    def attention(x, cold, zero):
        xn = _layernorm(x)
        for u, tile in enumerate(_paired_operands(xn)):
            xl_buf[u] = tile
        for c in range(NC):
            xl_buf[2 * NC + c] = _operand(_row(xn, c))
            put(v32, Y_ROW, c, jnp.zeros((8, 128), f32))
        wait(cold, *[("wq", i) for i in range(4)], *[("wo", c) for c in range(NC)], "k")
        run(q_jobs(0))
        q_sum(0)
        q_lhs(0)
        q_lhs(1)
        run(q_jobs(1) + qk_jobs(0, 0))
        softmax(0, 3, 0)()
        for part in range(EXN):
            expand(0, part, 0)
        run(qk_jobs(0, 1))
        q_sum(0)
        q_lhs(0)
        wait(cold, "v0")
        pair(zero, first=True)

        def body(n, carry):
            wait(jnp.logical_and(cold, n == V_SPLIT // 2), "v1")
            pair(n)
            return carry

        lax.fori_loop(1, NP - 1, body, 0)
        pair(zero + (NP - 1), last=True)
        run([out_job(t, 0) for t in range(3)])
        for t in range(3):
            normalise(t)
        run(wo_jobs(NP - 1))
        return x + _stack_rows([get(v32, Y_ROW, c) for c in range(NC)])

    def glu(x, cold):
        xl = jnp.concatenate(_paired_operands(_layernorm(x)), axis=1)
        wait(cold, "wg", "wu")
        hid = []
        for b in range(NFB):
            g = _dot(xl, _packed(wg32[:, pl.ds(8 * b, 8), :]))
            u = _dot(xl, _packed(wu32[:, pl.ds(8 * b, 8), :]))
            hid.append(_operand(jax.nn.sigmoid(g) * u))
        hid = jnp.concatenate(hid, axis=1)
        out = []
        for c in range(NC):
            wait(cold, ("wd", c))
            even, odd = [
                _dot(hid, jnp.concatenate(
                    [wd_buf[c, pl.ds(256 * b + 128 * par, 128), :] for b in range(NFB)], axis=0))
                for par in range(2)]
            out.append(_row(even, 0) + _row(odd, 1))
        return x + _stack_rows(out)

    copies["x"].wait()
    x_in = x_buf[...].astype(f32)
    x0 = _stack_rows([jnp.broadcast_to(x_in[:, c * 128:(c + 1) * 128], (8, 128))
                      for c in range(NC)])

    def layer(i, x):
        return glu(attention(x, i == 0, i >> 1), i == 0)

    x_out = lax.fori_loop(0, 2, layer, x0)
    out_ref[...] = jnp.concatenate(
        [x_out[c:c + 1, :] for c in range(NC)], axis=1).astype(out_ref.dtype)


def _tile_order(w, *shape):
    r, c = w.shape
    w = w.reshape(r // 8, 8, c // 128, 128)
    return jnp.transpose(w, (0, 2, 1, 3)).reshape(*shape, 128)


@jax.jit
def pallas_interleave_layers__sliding_block_cached__glu_gated_glu__decode_kernel(
    A_x: jax.Array,
    A_k_cache: jax.Array,
    A_v_cache: jax.Array,
    A_wq: jax.Array,
    A_wo: jax.Array,
    B_x: jax.Array,
    B_w_gate: jax.Array,
    B_w_up: jax.Array,
    B_w_down: jax.Array,
):
    del B_x
    k, v = [_tile_order(jnp.swapaxes(a, 2, 3).reshape(H * DH, SK), NRT, SK // 256, 16)
            for a in (A_k_cache, A_v_cache)]
    out = pl.pallas_call(
        _kernel,
        out_shape=jax.ShapeDtypeStruct((1, D), A_x.dtype),
        in_specs=[pl.BlockSpec(memory_space=pltpu.HBM)] * 8,
        out_specs=pl.BlockSpec(memory_space=pltpu.VMEM),
        scratch_shapes=[
            pltpu.VMEM((1, D), bf16),
            pltpu.VMEM((P_ROW + 4, 16, 16, 128), bf16),
            pltpu.VMEM((Y_ROW + 1, 16, 16, 128), bf16),
            pltpu.VMEM((D // 8, F // 16, 128), bf16),
            pltpu.VMEM((D // 8, F // 16, 128), bf16),
            pltpu.VMEM((NC, F, 128), bf16),
            pltpu.VMEM((3 * NC, 16, 128), bf16),
            pltpu.VMEM((2, 8, 128), f32),
            pltpu.VMEM((2, 3, 16, 128), bf16),
            pltpu.VMEM((3, 16, 128), bf16),
            pltpu.VMEM((4, 8, 128), f32),
            pltpu.SemaphoreType.DMA((10 + 2 * NC,)),
        ],
        compiler_params=pltpu.CompilerParams(vmem_limit_bytes=124 * 1024 * 1024),
    )(A_x.reshape(1, D), k, v,
      _tile_order(A_wq, D // 16, 2, NP, 24), A_wo.reshape(WO_ROWS, 16, 16, D),
      _tile_order(B_w_gate, D // 8, F // 16), _tile_order(B_w_up, D // 8, F // 16), B_w_down)
    return out.reshape(A_x.shape)
```

```python
import jax
import jax.numpy as jnp
from jax import lax
import jax.experimental.pallas as pl
import jax.experimental.pallas.tpu as pltpu

D = 640
H = 32
DH = 192
F = 1536
SK = 32768
WIN = min(4096, max(256, SK // 4))
EPS = 1e-5
LAYERS = 2
XP = 1

NC = D // 128
NP = H // 2
RT = DH // 8
NRT = H * RT
NJ = WIN // 256
NFB = F // 256
V_SPLIT = 24

WO_ROWS = H * DH * D // (256 * 128)
WQ2_ROW = NRT
WQ1_ROW = WQ2_ROW + D // 8
WO_ROW = WQ1_ROW + D // 16
A_ROW = WO_ROW + WO_ROWS
P_ROW = A_ROW + 2
S_ROW = NRT
Q_ROW = S_ROW + 2
Y_ROW = Q_ROW + 1

RS = 3
JS = 8
LAG = 4
LEAD = 3
SM = 1
PS = 7
EXN = 4
OUT0 = 6
QS = 22

f32, bf16, u32 = jnp.float32, jnp.bfloat16, jnp.uint32


def _iota(axis):
    return lax.broadcasted_iota(jnp.int32, (8, 128), axis)


def _operand(x):
    return jnp.concatenate([x, x], axis=0).astype(bf16)


def _dot(a, b):
    return jnp.dot(a, b, preferred_element_type=f32)[0:8]


def _packed(words):
    return pltpu.bitcast(words.reshape(words.shape[0] * 8, 128), bf16)


def _row(x, r):
    return jnp.broadcast_to(x[r:r + 1, :], (8, 128))


def _spread(x, half):
    lane = _iota(1)
    return jnp.take_along_axis(x, (lane // 16) * 8 + lane % 8 + 64 * half, axis=1)


def _split_parity(x):
    keep = (_iota(0) % 2) == ((_iota(1) // 8) % 2)
    return _operand(jnp.where(keep, x, 0.0))


def _layernorm(x):
    mean = jnp.sum(x, keepdims=True) * (1.0 / D)
    xc = jnp.where(_iota(0) < NC, x - mean, 0.0)
    var = jnp.sum(xc * xc, keepdims=True) * (1.0 / D)
    return xc * lax.rsqrt(var + EPS)


def _paired_operands(x):
    halves = (_spread(x, 0), _spread(x, 1))
    return [_split_parity(_row(halves[u % 2], u // 2)) for u in range(2 * NC)]


def _stack_rows(rows):
    out = jnp.zeros((8, 128), f32)
    for c, r in enumerate(rows):
        out = jnp.where(_iota(0) == c, r, out)
    return out


RAGGED = (0, 0, 1, 2, 2)


def _ragged_operands(x):
    lane = _iota(1)
    first = (lane // 16) * 16 + lane % 8
    return [_split_parity(jnp.take_along_axis(x, first, axis=1)), _split_parity(x),
            _split_parity(jnp.take_along_axis(x, first + 8, axis=1))]


def _ragged_result(parts):
    tiles = [_row(parts[i // 2], i % 2) for i in range(2 * NC)]
    return _stack_rows([tiles[c] + tiles[NC + c] for c in range(NC)])


def _kernel(x_hbm, k_hbm, v_hbm, wq_hbm, wo_hbm, wg_hbm, wu_hbm, wd_hbm, out_ref,
            x_buf, k_buf, v_buf, wg_buf, wu_buf, wd_buf,
            xl_buf, q_buf, ql_buf, ol_buf, inv_buf, sems):
    k32, v32 = k_buf.bitcast(u32), v_buf.bitcast(u32)
    wg32, wu32, wd32 = wg_buf.bitcast(u32), wu_buf.bitcast(u32), wd_buf.bitcast(u32)

    win = pl.ds((SK - WIN) // 256, NJ)
    vs = V_SPLIT * RT
    copies = {}

    def copy(name, src, dst):
        copies[name] = pltpu.make_async_copy(src, dst, sems.at[len(copies)])

    copy("x", x_hbm, x_buf)
    for i in range(2):
        copy(("wq", i), wq_hbm.at[:, i, :, pl.ds(0, 16), :],
             k_buf.at[pl.ds(WQ2_ROW + i * D // 16, D // 16)])
        copy(("wq", 2 + i), wq_hbm.at[:, i, :, pl.ds(16, 8), :],
             k_buf.at[pl.ds(WQ1_ROW, D // 16), :, pl.ds(8 * i, 8), :])
    copy("wo", wo_hbm, k_buf.at[pl.ds(WO_ROW, WO_ROWS)])
    copy("k", k_hbm.at[:, win], k_buf.at[pl.ds(0, NRT)])
    copy("v0", v_hbm.at[pl.ds(0, vs), win], v_buf.at[pl.ds(0, vs)])
    copy("v1", v_hbm.at[pl.ds(vs, NRT - vs), win], v_buf.at[pl.ds(vs, NRT - vs)])
    copy("wg", wg_hbm, wg_buf)
    copy("wu", wu_hbm, wu_buf)
    for i in range(2):
        rows = pl.ds(i * F // 32, F // 32)
        copy(("wd", i), wd_hbm.at[rows], wd_buf.at[rows])
    for cp in copies.values():
        cp.start()

    def wait(cond, *names):
        @pl.when(cond)
        def _():
            for name in names:
                copies[name].wait()


    def put(ref, row, i, x):
        ref[row + i // 16, i % 16] = pltpu.bitcast(x, u32)

    def get(ref, row, i):
        return pltpu.bitcast(ref[row + i // 16, i % 16], f32)

    def q_jobs(n):
        def make(u):
            def job():
                if u < 2 * NC:
                    w = [k32[WQ2_ROW + (a % 2) * (D // 16) + a // 2, n]
                         for a in range(8 * u, 8 * u + 8)]
                    w = pltpu.bitcast(jnp.concatenate(w, axis=0), bf16)
                else:
                    w = _packed(k32[pl.ds(WQ1_ROW + 8 * (u - 2 * NC), 8), n])
                r = _dot(xl_buf[u], w)
                return lambda: put(v32, Q_ROW, u, r)
            return job
        return [make(u) for u in range(3 * NC)]

    def q_sum(zero):
        parts = pltpu.bitcast(v32[zero + Q_ROW, pl.ds(0, 3 * NC)], f32)
        q_buf[0] = parts[:2 * NC].sum(axis=0)
        q_buf[1] = parts[2 * NC:].sum(axis=0)

    def q_lhs(e):
        for t in range(3):
            m = (3 * e + t) // 2
            q = _row(q_buf[0], m) if m < 2 else q_buf[1]
            ql_buf[e, t] = _split_parity(_spread(q, (3 * e + t) % 2))

    def qk_jobs(n, e):
        def make(j, t):
            def job():
                w = _packed(k32[pl.ds(n * 2 * RT + e * RT + 8 * t, 8), j])
                r = pltpu.bitcast(_dot(ql_buf[e, t], w), u32)

                def drain():
                    lo = 2 * (j % 4)
                    v32[S_ROW + e, 4 * t + j // 4, pl.ds(lo, 2), :] = r[lo:lo + 2, :]
                return drain
            return job
        return [make(j, t) for j in range(NJ) for t in range(3)]

    def softmax(e, slot, zero):
        parts = pltpu.bitcast(v32[zero + S_ROW + e, pl.ds(0, 12)], f32)
        s = (parts[0:4] + parts[4:8] + parts[8:12]).reshape(32, 128) * (DH ** -0.5)
        p = jnp.exp(s - jnp.max(s, keepdims=True))
        inv_buf[slot] = jnp.broadcast_to(1.0 / jnp.sum(p, keepdims=True), (8, 128))

        def publish():
            for i in range(4):
                put(v32, S_ROW + e, 12 + i, p[8 * i:8 * i + 8])
        return publish

    def expand(e, part, zero):
        for c in range(32 * part // EXN, 32 * (part + 1) // EXN):
            row = pltpu.bitcast(v32[zero + S_ROW + e, 12 + c // 8, pl.ds(c % 8, 1), :], f32)
            put(k32, P_ROW + 2 * e, c, jnp.broadcast_to(row, (8, 128)))

    def pv_steps(n, e):
        acc = [None] * RS

        def make(r0, j0):
            def step():
                for j in range(j0, j0 + JS):
                    p0, p1 = get(k32, P_ROW + 2 * e, 2 * j), get(k32, P_ROW + 2 * e, 2 * j + 1)
                    for r in range(RS):
                        v = v_buf[n * 2 * RT + e * RT + r0 + r, j].astype(f32)
                        t = v[0:8] * p0 + v[8:16] * p1
                        acc[r] = t if j == 0 else acc[r] + t
                for r in range(RS):
                    rt = e * RT + r0 + r
                    k_buf[A_ROW + rt // 32, (rt // 2) % 16, pl.ds(8 * (rt % 2), 8), :] = (
                        acc[r].astype(bf16))
            return step
        return [make(r0, j0) for r0 in range(0, RT, RS) for j0 in range(0, NJ, JS)]

    def out_job(t, zero):
        def job():
            w = _packed(k32[zero + A_ROW + t // 2, pl.ds(8 * (t % 2), 8)])
            r = lax.dot_general(jnp.ones((16, 128), bf16), w, (((1,), (XP,)), ((), ())),
                                preferred_element_type=f32)[0:8]
            return lambda: put(v32, Y_ROW, 8 + t, r)
        return job

    def normalise(t):
        inv = (inv_buf[0] if t == 0 else inv_buf[1] if t == 2 else
               jnp.where(_iota(1) < DH - 128, inv_buf[0], inv_buf[1]))
        for i, tile in enumerate(_ragged_operands(get(v32, Y_ROW, 8 + t) * inv)):
            ol_buf[t, i] = tile

    def wo_jobs(n):
        at = [(WO_ROW + (i >> 1), 8 * (i & 1)) for i in (3 * NC * n, 3 * NC * n + 1)]

        def make(t, m):
            def job():
                w = [k32[at[i // 8 % 2][0] + i // 16, at[i // 8 % 2][1] + i % 8]
                     for i in range(8 * NC * t + m, 8 * NC * (t + 1), NC)]
                r = _dot(ol_buf[t, RAGGED[m]], pltpu.bitcast(jnp.concatenate(w, axis=0), bf16))
                return lambda: put(v32, Y_ROW, m, get(v32, Y_ROW, m) + r)
            return job
        return [make(t, m) for t in range(3) for m in range(NC)]

    def run(jobs):
        for drain in [job() for job in jobs]:
            drain()

    def interleave(jobs, steps, hooks):
        ns = len(steps)
        extra = len(jobs) - 4 * ns
        assert max(hooks) < ns and extra >= 0
        groups = [[job for job in jobs[4 * g + extra * (g > 0):4 * g + 4 + extra] if job]
                  for g in range(ns)]
        pending = {g: [job() for job in groups[g]] for g in range(LEAD)}
        for g, step in enumerate(steps):
            for drain in pending.pop(g - LAG, ()):
                drain()
            for hook in hooks.get(g, ()):
                hook()
            step()
            if g + LEAD < ns:
                pending[g + LEAD] = [job() for job in groups[g + LEAD]]
        for g in sorted(pending):
            for drain in pending[g]:
                drain()

    def pair(n, first=False, last=False):
        zero = n >> 8
        steps = pv_steps(n, 0) + pv_steps(n, 1)
        half = len(steps) // 2
        hooks = {}

        def at(g, fn, *args):
            hooks.setdefault(g, []).append(lambda: fn(*args))

        def softmax_at(g, e):
            result = []
            at(g, lambda: result.append(softmax(e, 3 - e, zero)))
            at(g + PS, lambda: result[0]())
            for part in range(EXN):
                at(g + PS + 1 + part, expand, e, part, zero)

        def rotate():
            inv_buf[0] = inv_buf[3]
            inv_buf[1] = inv_buf[2]

        softmax_at(SM, 1)
        at(half, rotate)
        head, tail = [None] * 3, [None] * (3 * NC)
        if not first:
            head, tail = [out_job(t, zero) for t in range(3)], wo_jobs(n - 1)
            for t in range(3):
                at(OUT0 + t, normalise, t)
        middle = [None] * (6 * NJ + 3 * NC)
        if not last:
            q_lhs(1)
            middle = qk_jobs(n + 1, 0) + q_jobs(jnp.minimum(n + 2, NP - 1)) + qk_jobs(n + 1, 1)
            softmax_at(half + SM, 0)
            at(QS, q_sum, zero)
            at(QS + 2, q_lhs, 0)
        interleave(head + middle + tail, steps, hooks)

    def attention(x, cold, zero):
        xn = _layernorm(x)
        for u, tile in enumerate(_paired_operands(xn)):
            xl_buf[u] = tile
        for c in range(NC):
            xl_buf[2 * NC + c] = _operand(_row(xn, c))
            put(v32, Y_ROW, c, jnp.zeros((8, 128), f32))
        wait(cold, *[("wq", i) for i in range(4)], "wo", "k")
        run(q_jobs(0))
        q_sum(0)
        q_lhs(0)
        q_lhs(1)
        run(q_jobs(1) + qk_jobs(0, 0))
        softmax(0, 3, 0)()
        for part in range(EXN):
            expand(0, part, 0)
        run(qk_jobs(0, 1))
        q_sum(0)
        q_lhs(0)
        wait(cold, "v0")
        pair(zero, first=True)

        def body(n, carry):
            wait(jnp.logical_and(cold, n == V_SPLIT // 2), "v1")
            pair(n)
            return carry

        lax.fori_loop(1, NP - 1, body, 0)
        pair(zero + (NP - 1), last=True)
        run([out_job(t, 0) for t in range(3)])
        for t in range(3):
            normalise(t)
        run(wo_jobs(NP - 1))
        return x + _ragged_result([get(v32, Y_ROW, m) for m in range(NC)])

    def glu(x, cold):
        xl = jnp.concatenate(_paired_operands(_layernorm(x)), axis=1)
        wait(cold, "wg", "wu")
        hid = []
        for b in range(NFB):
            g = _dot(xl, _packed(wg32[:, pl.ds(8 * b, 8), :]))
            u = _dot(xl, _packed(wu32[:, pl.ds(8 * b, 8), :]))
            h = jax.nn.sigmoid(g) * u
            hid += [_ragged_operands(_row(h, par)) for par in range(2)]
        out = [0.0] * NC
        for i in range(2):
            wait(cold, ("wd", i))
            for m in range(NC):
                lhs = jnp.concatenate([h[RAGGED[m]] for h in hid[i * NFB:(i + 1) * NFB]], axis=1)
                out[m] += _dot(lhs, _packed(wd32[pl.ds(i * F // 32, F // 32), m]))
        return x + _ragged_result(out)

    copies["x"].wait()
    x_in = x_buf[...].astype(f32)
    x0 = _stack_rows([jnp.broadcast_to(x_in[:, c * 128:(c + 1) * 128], (8, 128))
                      for c in range(NC)])

    def layer(i, x):
        return glu(attention(x, i == 0, i >> 8), i == 0)

    x_out = lax.fori_loop(0, LAYERS, layer, x0)
    out_ref[...] = jnp.concatenate(
        [x_out[c:c + 1, :] for c in range(NC)], axis=1).astype(out_ref.dtype)


def _tile_order(w, *shape):
    r, c = w.shape
    w = w.reshape(r // 8, 8, c // 128, 128)
    return jnp.transpose(w, (0, 2, 1, 3)).reshape(*shape, 128)


@jax.jit
def pallas_interleave_layers__sliding_block_cached__glu_gated_glu__decode_kernel(
    A_x: jax.Array,
    A_k_cache: jax.Array,
    A_v_cache: jax.Array,
    A_wq: jax.Array,
    A_wo: jax.Array,
    B_x: jax.Array,
    B_w_gate: jax.Array,
    B_w_up: jax.Array,
    B_w_down: jax.Array,
):
    del B_x
    k, v = [_tile_order(jnp.swapaxes(a, 2, 3).reshape(H * DH, SK), NRT, SK // 256, 16)
            for a in (A_k_cache, A_v_cache)]
    out = pl.pallas_call(
        _kernel,
        out_shape=jax.ShapeDtypeStruct((1, D), A_x.dtype),
        in_specs=[pl.BlockSpec(memory_space=pltpu.HBM)] * 8,
        out_specs=pl.BlockSpec(memory_space=pltpu.VMEM),
        scratch_shapes=[
            pltpu.VMEM((1, D), bf16),
            pltpu.VMEM((P_ROW + 4, 16, 16, 128), bf16),
            pltpu.VMEM((Y_ROW + 1, 16, 16, 128), bf16),
            pltpu.VMEM((D // 8, F // 16, 128), bf16),
            pltpu.VMEM((D // 8, F // 16, 128), bf16),
            pltpu.VMEM((F // 16, NC, 16, 128), bf16),
            pltpu.VMEM((3 * NC, 16, 128), bf16),
            pltpu.VMEM((2, 8, 128), f32),
            pltpu.VMEM((2, 3, 16, 128), bf16),
            pltpu.VMEM((3, 3, 16, 128), bf16),
            pltpu.VMEM((4, 8, 128), f32),
            pltpu.SemaphoreType.DMA((13,)),
        ],
        compiler_params=pltpu.CompilerParams(vmem_limit_bytes=124 * 1024 * 1024),
    )(A_x.reshape(1, D), k, v,
      _tile_order(A_wq, D // 16, 2, NP, 24), _tile_order(A_wo, WO_ROWS, 16, 16),
      _tile_order(B_w_gate, D // 8, F // 16), _tile_order(B_w_up, D // 8, F // 16),
      _tile_order(B_w_down, F // 16, NC, 16))
    return out.reshape(A_x.shape)
```

```python
import jax
import jax.numpy as jnp
from jax import lax
import jax.experimental.pallas as pl
import jax.experimental.pallas.tpu as pltpu

D = 640
H = 32
DH = 192
F = 1536
SK = 32768
WIN = min(4096, max(256, SK // 4))
EPS = 1e-5
LAYERS = 2
SN = 0
U0, U, U1 = 1, 1, 1
XP = 1

NC = D // 128
NP = H // 2
RT = DH // 8
NRT = H * RT
NJ = WIN // 256
NFB = F // 256
V_SPLIT = 24

WO_ROWS = H * DH * D // (256 * 128)
WQ2_ROW = NRT
WQ1_ROW = WQ2_ROW + D // 8
WO_ROW = WQ1_ROW + D // 16
A_ROW = WO_ROW + WO_ROWS
P_ROW = A_ROW + 2
S_ROW = NRT
Q_ROW = S_ROW + 2
O_ROW = Q_ROW + 1
Y_ROW = O_ROW + 1

RS = 3
JS = 8
LAG = 4
LEAD = 3
SM = 1
PS = 7
EXN = 4
OUT0 = 6
YS = 14
QS = 22

f32, bf16, u32 = jnp.float32, jnp.bfloat16, jnp.uint32


def _iota(axis):
    return lax.broadcasted_iota(jnp.int32, (8, 128), axis)


def _operand(x):
    return jnp.concatenate([x, x], axis=0).astype(bf16)


def _dot(a, b):
    return jnp.dot(a, b, preferred_element_type=f32)[0:8]


def _packed(words):
    return pltpu.bitcast(words.reshape(words.shape[0] * 8, 128), bf16)


def _row(x, r):
    return jnp.broadcast_to(x[r:r + 1, :], (8, 128))


def _spread(x, half):
    lane = _iota(1)
    return jnp.take_along_axis(x, (lane // 16) * 8 + lane % 8 + 64 * half, axis=1)


def _split_parity(x):
    keep = (_iota(0) % 2) == ((_iota(1) // 8) % 2)
    return _operand(jnp.where(keep, x, 0.0))


def _reduce(fn, x):
    x = fn(x.reshape(-1, 8, 128), axis=0)
    return jnp.broadcast_to(fn(fn(x, axis=0, keepdims=True), axis=1, keepdims=True), (8, 128))


def _layernorm(x):
    mean = _reduce(jnp.sum, x) * (1.0 / D)
    xc = jnp.where(_iota(0) < NC, x - mean, 0.0)
    rstd = lax.rsqrt(_reduce(jnp.sum, xc * xc) * (1.0 / D) + EPS)
    halves = [_spread(x, half) - mean for half in range(2)]
    return xc, [_split_parity(_row(halves[u % 2], u // 2)) for u in range(2 * NC)], rstd


def _stack_rows(rows):
    out = jnp.zeros((8, 128), f32)
    for c, r in enumerate(rows):
        out = jnp.where(_iota(0) == c, r, out)
    return out


RAGGED = (0, 0, 1, 2, 2)


def _ragged_operands(x):
    lane = _iota(1)
    first = (lane // 16) * 16 + lane % 8
    return [_split_parity(jnp.take_along_axis(x, first, axis=1)), _split_parity(x),
            _split_parity(jnp.take_along_axis(x, first + 8, axis=1))]


def _ragged_result(parts):
    tiles = [_row(parts[i // 2], i % 2) for i in range(2 * NC)]
    return _stack_rows([tiles[c] + tiles[NC + c] for c in range(NC)])


def _kernel(x_hbm, k_hbm, v_hbm, wq_hbm, wo_hbm, wg_hbm, wu_hbm, wd_hbm, out_ref,
            x_buf, k_buf, v_buf, wg_buf, wu_buf, wd_buf,
            xl_buf, q_buf, ql_buf, ol_buf, inv_buf, y_buf, sems):
    k32, v32 = k_buf.bitcast(u32), v_buf.bitcast(u32)
    wg32, wu32, wd32 = wg_buf.bitcast(u32), wu_buf.bitcast(u32), wd_buf.bitcast(u32)

    win = pl.ds((SK - WIN) // 256, NJ)
    vs = V_SPLIT * RT
    copies = {}

    def copy(name, src, dst):
        copies[name] = pltpu.make_async_copy(src, dst, sems.at[len(copies)])

    copy("x", x_hbm, x_buf)
    for i in range(2):
        copy(("wq", i), wq_hbm.at[:, i, :, pl.ds(0, 16), :],
             k_buf.at[pl.ds(WQ2_ROW + i * D // 16, D // 16)])
        copy(("wq", 2 + i), wq_hbm.at[:, i, :, pl.ds(16, 8), :],
             k_buf.at[pl.ds(WQ1_ROW, D // 16), :, pl.ds(8 * i, 8), :])
    copy("wo", wo_hbm, k_buf.at[pl.ds(WO_ROW, WO_ROWS)])
    copy("k", k_hbm.at[:, win], k_buf.at[pl.ds(0, NRT)])
    copy("v0", v_hbm.at[pl.ds(0, vs), win], v_buf.at[pl.ds(0, vs)])
    copy("v1", v_hbm.at[pl.ds(vs, NRT - vs), win], v_buf.at[pl.ds(vs, NRT - vs)])
    copy("wg", wg_hbm, wg_buf)
    copy("wu", wu_hbm, wu_buf)
    for i in range(2):
        rows = pl.ds(i * F // 32, F // 32)
        copy(("wd", i), wd_hbm.at[rows], wd_buf.at[rows])
    for cp in copies.values():
        cp.start()

    def wait(cond, *names):
        @pl.when(cond)
        def _():
            for name in names:
                copies[name].wait()


    def put(ref, row, i, x):
        ref[row + i // 16, i % 16] = pltpu.bitcast(x, u32)

    def get(ref, row, i):
        return pltpu.bitcast(ref[row + i // 16, i % 16], f32)

    def q_jobs(n):
        def make(u):
            def job():
                if u < 2 * NC:
                    w = [k32[WQ2_ROW + (a % 2) * (D // 16) + a // 2, n]
                         for a in range(8 * u, 8 * u + 8)]
                    w = pltpu.bitcast(jnp.concatenate(w, axis=0), bf16)
                else:
                    w = _packed(k32[pl.ds(WQ1_ROW + 8 * (u - 2 * NC), 8), n])
                r = _dot(xl_buf[u], w)
                return lambda: put(v32, Q_ROW, u, r)
            return job
        return [make(u) for u in range(3 * NC)]

    def q_sum(zero):
        parts = pltpu.bitcast(v32[zero + Q_ROW, pl.ds(0, 3 * NC)], f32)
        q_buf[0] = parts[:2 * NC].sum(axis=0) * q_buf[2]
        q_buf[1] = parts[2 * NC:].sum(axis=0) * q_buf[2]

    def q_lhs(e):
        for t in range(3):
            m = (3 * e + t) // 2
            q = _row(q_buf[0], m) if m < 2 else q_buf[1]
            ql_buf[e, t] = _split_parity(_spread(q, (3 * e + t) % 2))

    def qk_jobs(n, e):
        def make(j, t):
            def job():
                w = _packed(k32[pl.ds(n * 2 * RT + e * RT + 8 * t, 8), j])
                r = pltpu.bitcast(_dot(ql_buf[e, t], w), u32)

                def drain():
                    lo = 2 * (j % 4)
                    v32[S_ROW + e, 4 * t + j // 4, pl.ds(lo, 2), :] = r[lo:lo + 2, :]
                return drain
            return job
        return [make(j, t) for j in range(NJ) for t in range(3)]

    def softmax(e, slot, zero):
        parts = pltpu.bitcast(v32[zero + S_ROW + e, pl.ds(0, 12)], f32)
        s = (parts[0:4] + parts[4:8] + parts[8:12]).reshape(32, 128) * (DH ** -0.5)
        p = jnp.exp(s - jnp.concatenate([_reduce(jnp.max, s)] * 4, axis=0))
        inv_buf[slot] = 1.0 / _reduce(jnp.sum, p)

        def publish():
            for i in range(4):
                put(v32, S_ROW + e, 12 + i, p[8 * i:8 * i + 8])
        return publish

    def expand(e, part, zero):
        for c in range(32 * part // EXN, 32 * (part + 1) // EXN):
            row = pltpu.bitcast(v32[zero + S_ROW + e, 12 + c // 8, pl.ds(c % 8, 1), :], f32)
            put(k32, P_ROW + 2 * e, c, jnp.broadcast_to(row, (8, 128)))

    def pv_steps(n, e):
        acc = [None] * RS

        def make(r0, j0):
            def step():
                for j in range(j0, j0 + JS):
                    p0, p1 = get(k32, P_ROW + 2 * e, 2 * j), get(k32, P_ROW + 2 * e, 2 * j + 1)
                    for r in range(RS):
                        v = v_buf[n * 2 * RT + e * RT + r0 + r, j].astype(f32)
                        t = v[0:8] * p0 + v[8:16] * p1
                        acc[r] = t if j == 0 else acc[r] + t
                for r in range(SN if j0 + JS < NJ else 0, RS):
                    rt = e * RT + r0 + r
                    k_buf[A_ROW + rt // 32, (rt // 2) % 16, pl.ds(8 * (rt % 2), 8), :] = (
                        acc[r].astype(bf16))
            return step
        return [make(r0, j0) for r0 in range(0, RT, RS) for j0 in range(0, NJ, JS)]

    def out_job(t, zero):
        def job():
            w = _packed(k32[zero + A_ROW + t // 2, pl.ds(8 * (t % 2), 8)])
            r = lax.dot_general(jnp.ones((16, 128), bf16), w, (((1,), (XP,)), ((), ())),
                                preferred_element_type=f32)[0:8]
            return lambda: put(v32, O_ROW, t, r)
        return job

    def normalise(t):
        inv = (inv_buf[0] if t == 0 else inv_buf[1] if t == 2 else
               jnp.where(_iota(1) < DH - 128, inv_buf[0], inv_buf[1]))
        for i, tile in enumerate(_ragged_operands(get(v32, O_ROW, t) * inv)):
            ol_buf[t, i] = tile

    def wo_jobs(n):
        at = [(WO_ROW + (i >> 1), 8 * (i & 1)) for i in (3 * NC * n, 3 * NC * n + 1)]

        def make(t, m):
            def job():
                w = [k32[at[i // 8 % 2][0] + i // 16, at[i // 8 % 2][1] + i % 8]
                     for i in range(8 * NC * t + m, 8 * NC * (t + 1), NC)]
                r = _dot(ol_buf[t, RAGGED[m]], pltpu.bitcast(jnp.concatenate(w, axis=0), bf16))
                return lambda: put(v32, Y_ROW, NC * t + m, r)
            return job
        return [make(t, m) for t in range(3) for m in range(NC)]

    def y_sum(m, zero):
        parts = [get(v32, zero + Y_ROW, NC * t + m) for t in range(3)]
        y_buf[m] += parts[0] + parts[1] + parts[2]

    def run(jobs):
        for drain in [job() for job in jobs]:
            drain()

    def interleave(*plans):
        hooks, steps, groups = zip(*[slot for plan in plans for slot in plan])
        ns = len(steps)
        pending = {g: [job() for job in groups[g]] for g in range(LEAD)}
        for g, step in enumerate(steps):
            for drain in pending.pop(g - LAG, ()):
                drain()
            for hook in hooks[g]:
                hook()
            step()
            if g + LEAD < ns:
                pending[g + LEAD] = [job() for job in groups[g + LEAD]]
        for g in sorted(pending):
            for drain in pending[g]:
                drain()

    def pair(n, first=False, last=False):
        zero = n >> 8
        steps = pv_steps(n, 0) + pv_steps(n, 1)
        half = len(steps) // 2
        hooks = {}

        def at(g, fn, *args):
            hooks.setdefault(g, []).append(lambda: fn(*args))

        def softmax_at(g, e):
            result = []
            at(g, lambda: result.append(softmax(e, 3 - e, zero)))
            at(g + PS, lambda: result[0]())
            for part in range(EXN):
                at(g + PS + 1 + part, expand, e, part, zero)

        def rotate():
            inv_buf[0] = inv_buf[3]
            inv_buf[1] = inv_buf[2]

        softmax_at(SM, 1)
        at(half, rotate)
        head, tail = [None] * 3, [None] * (3 * NC)
        if not first:
            head, tail = [out_job(t, zero) for t in range(3)], wo_jobs(n - 1)
            for t in range(3):
                at(OUT0 + t, normalise, t)
            for m in range(NC):
                at(YS + m, y_sum, m, zero)
        middle = [None] * (6 * NJ + 3 * NC)
        if not last:
            at(0, q_lhs, 1)
            middle = qk_jobs(n + 1, 0) + q_jobs(jnp.minimum(n + 2, NP - 1)) + qk_jobs(n + 1, 1)
            softmax_at(half + SM, 0)
            at(QS, q_sum, zero)
            at(QS + 2, q_lhs, 0)
        jobs = head + middle + tail
        extra = len(jobs) - 4 * len(steps)

        return [(hooks.get(g, ()), step,
                 [job for job in jobs[4 * g + extra * (g > 0):4 * g + 4 + extra] if job])
                for g, step in enumerate(steps)]

    def attention(x, cold, zero):
        wait(cold, *[("wq", i) for i in range(4)], "wo", "k")
        xc, tiles, q_buf[2] = _layernorm(x)
        for u, tile in enumerate(tiles):
            xl_buf[u] = tile
        for c in range(NC):
            xl_buf[2 * NC + c] = _operand(_row(xc, c))
            y_buf[c] = jnp.zeros((8, 128), f32)
        for i in range(3 * NC):
            put(v32, Y_ROW, i, jnp.zeros((8, 128), f32))
        run(q_jobs(0))
        q_sum(0)
        q_lhs(0)
        q_lhs(1)
        run(q_jobs(1) + qk_jobs(0, 0))
        softmax(0, 3, 0)()
        for part in range(EXN):
            expand(0, part, 0)
        run(qk_jobs(0, 1))
        q_sum(0)
        q_lhs(0)
        wait(cold, "v0")
        interleave(pair(zero, first=True), *[pair(zero + i) for i in range(1, U0)])

        def body(i, carry):
            n = U0 + i * U
            wait(jnp.logical_and(cold, n == V_SPLIT // 2), "v1")
            interleave(*[pair(n + i) for i in range(U)])
            return carry

        trips = (NP - U0 - U1) // U
        assert U0 + trips * U + U1 == NP
        if trips:
            lax.fori_loop(0, trips, body, 0)
        interleave(*[pair(zero + i) for i in range(NP - U1, NP - 1)],
                   pair(zero + (NP - 1), last=True))
        run([out_job(t, 0) for t in range(3)])
        for t in range(3):
            normalise(t)
        for m in range(NC):
            y_sum(m, 0)
        run(wo_jobs(NP - 1))
        for m in range(NC):
            y_sum(m, 0)
        return x + _ragged_result([y_buf[m] for m in range(NC)])

    def glu(x, cold):
        def arrive(name):
            if cold:
                copies[name].wait()

        arrive("wg")
        arrive("wu")
        _, tiles, rstd = _layernorm(x)
        xl = jnp.concatenate(tiles, axis=1)
        hid = []
        for b in range(NFB):
            g = _dot(xl, _packed(wg32[:, pl.ds(8 * b, 8), :])) * rstd
            u = _dot(xl, _packed(wu32[:, pl.ds(8 * b, 8), :])) * rstd
            h = jax.nn.sigmoid(g) * u
            hid += [_ragged_operands(_row(h, par)) for par in range(2)]
        out = [0.0] * NC
        for i, chunk in enumerate(hid):
            if i % NFB == 0:
                arrive(("wd", i // NFB))
            for m in range(NC):
                out[m] += _dot(chunk[RAGGED[m]], _packed(wd32[pl.ds(8 * i, 8), m]))
        return x + _ragged_result(out)

    copies["x"].wait()
    x_in = x_buf[...].astype(f32)
    x0 = _stack_rows([jnp.broadcast_to(x_in[:, c * 128:(c + 1) * 128], (8, 128))
                      for c in range(NC)])

    def layer(i, x):
        x = attention(x, i == 0, i >> 8)
        x = lax.cond(i == 0, lambda: glu(x, True), lambda: glu(x, False))
        return x

    x_out = lax.fori_loop(0, LAYERS, layer, x0)
    out_ref[...] = jnp.concatenate(
        [x_out[c:c + 1, :] for c in range(NC)], axis=1).astype(out_ref.dtype)


def _tile_order(w, *shape):
    r, c = w.shape
    w = w.reshape(r // 8, 8, c // 128, 128)
    return jnp.transpose(w, (0, 2, 1, 3)).reshape(*shape, 128)


@jax.jit
def pallas_interleave_layers__sliding_block_cached__glu_gated_glu__decode_kernel(
    A_x: jax.Array,
    A_k_cache: jax.Array,
    A_v_cache: jax.Array,
    A_wq: jax.Array,
    A_wo: jax.Array,
    B_x: jax.Array,
    B_w_gate: jax.Array,
    B_w_up: jax.Array,
    B_w_down: jax.Array,
):
    del B_x
    k, v = [_tile_order(jnp.swapaxes(a, 2, 3).reshape(H * DH, SK), NRT, SK // 256, 16)
            for a in (A_k_cache, A_v_cache)]
    out = pl.pallas_call(
        _kernel,
        out_shape=jax.ShapeDtypeStruct((1, D), A_x.dtype),
        in_specs=[pl.BlockSpec(memory_space=pltpu.HBM)] * 8,
        out_specs=pl.BlockSpec(memory_space=pltpu.VMEM),
        scratch_shapes=[
            pltpu.VMEM((1, D), bf16),
            pltpu.VMEM((P_ROW + 4, 16, 16, 128), bf16),
            pltpu.VMEM((Y_ROW + 1, 16, 16, 128), bf16),
            pltpu.VMEM((D // 8, F // 16, 128), bf16),
            pltpu.VMEM((D // 8, F // 16, 128), bf16),
            pltpu.VMEM((F // 16, NC, 16, 128), bf16),
            pltpu.VMEM((3 * NC, 16, 128), bf16),
            pltpu.VMEM((3, 8, 128), f32),
            pltpu.VMEM((2, 3, 16, 128), bf16),
            pltpu.VMEM((3, 3, 16, 128), bf16),
            pltpu.VMEM((4, 8, 128), f32),
            pltpu.VMEM((NC, 8, 128), f32),
            pltpu.SemaphoreType.DMA((13,)),
        ],
        compiler_params=pltpu.CompilerParams(vmem_limit_bytes=124 * 1024 * 1024),
    )(A_x.reshape(1, D), k, v,
      _tile_order(A_wq, D // 16, 2, NP, 24), _tile_order(A_wo, WO_ROWS, 16, 16),
      _tile_order(B_w_gate, D // 8, F // 16), _tile_order(B_w_up, D // 8, F // 16),
      _tile_order(B_w_down, F // 16, NC, 16))
    return out.reshape(A_x.shape)
```

```python
import jax
import jax.numpy as jnp
from jax import lax
import jax.experimental.pallas as pl
import jax.experimental.pallas.tpu as pltpu

D = 640
H = 32
DH = 192
F = 1536
SK = 32768
WIN = min(4096, max(256, SK // 4))
EPS = 1e-5
LAYERS = 2
SN = 2
LPS = 3
LJ = 8
QL0 = 30
QL1 = 27
SM0 = 1
PS0 = 7
EXS = 2
OS = 1
YSS = 1
RO = 16
EXTRA = 1
ONLY = 0
U0, U, U1 = 1, 1, 1
XP = 1

NC = D // 128
NP = H // 2
RT = DH // 8
NRT = H * RT
NJ = WIN // 256
NFB = F // 256
V_SPLIT = 24

WO_ROWS = H * DH * D // (256 * 128)
WQ2_ROW = NRT
WQ1_ROW = WQ2_ROW + D // 8
WO_ROW = WQ1_ROW + D // 16
VT_ROW = WO_ROW + WO_ROWS
A_ROW = VT_ROW + 16
P_ROW = A_ROW + 2
S_ROW = NRT - 16
Q_ROW = S_ROW + 2
O_ROW = Q_ROW + 1
Z_ROW = O_ROW + 1
Y_ROW = Z_ROW + 1

RS = 3
JS = 8
LAG = 4
LEAD = 3
SM = 1
PS = 5
EXN = 4
OUT0 = 8
YS = 14
QS = 23

f32, bf16, u32 = jnp.float32, jnp.bfloat16, jnp.uint32


def _iota(axis):
    return lax.broadcasted_iota(jnp.int32, (8, 128), axis)


def _operand(x):
    return jnp.concatenate([x, x], axis=0).astype(bf16)


def _dot(a, b):
    return jnp.dot(a, b, preferred_element_type=f32)[0:8]


def _packed(words):
    return pltpu.bitcast(words.reshape(words.shape[0] * 8, 128), bf16)


def _row(x, r):
    return jnp.broadcast_to(x[r:r + 1, :], (8, 128))


def _spread(x, half):
    lane = _iota(1)
    return jnp.take_along_axis(x, (lane // 16) * 8 + lane % 8 + 64 * half, axis=1)


def _split_parity(x):
    keep = (_iota(0) % 2) == ((_iota(1) // 8) % 2)
    return _operand(jnp.where(keep, x, 0.0))


def _reduce(fn, x):
    x = fn(x.reshape(-1, 8, 128), axis=0)
    return jnp.broadcast_to(fn(fn(x, axis=0, keepdims=True), axis=1, keepdims=True), (8, 128))


def _layernorm(x):
    mean = _reduce(jnp.sum, x) * (1.0 / D)
    xc = jnp.where(_iota(0) < NC, x - mean, 0.0)
    rstd = lax.rsqrt(_reduce(jnp.sum, xc * xc) * (1.0 / D) + EPS)
    halves = [_spread(x, half) - mean for half in range(2)]
    return xc, [_split_parity(_row(halves[u % 2], u // 2)) for u in range(2 * NC)], rstd


def _stack_rows(rows):
    out = jnp.zeros((8, 128), f32)
    for c, r in enumerate(rows):
        out = jnp.where(_iota(0) == c, r, out)
    return out


RAGGED = (0, 0, 1, 2, 2)


def _ragged_operands(x):
    lane = _iota(1)
    first = (lane // 16) * 16 + lane % 8
    return [_split_parity(jnp.take_along_axis(x, first, axis=1)), _split_parity(x),
            _split_parity(jnp.take_along_axis(x, first + 8, axis=1))]


def _ragged_result(parts):
    tiles = [_row(parts[i // 2], i % 2) for i in range(2 * NC)]
    return _stack_rows([tiles[c] + tiles[NC + c] for c in range(NC)])


def _kernel(x_hbm, k_hbm, v_hbm, wq_hbm, wo_hbm, wg_hbm, wu_hbm, wd_hbm, out_ref,
            x_buf, k_buf, v_buf, wg_buf, wu_buf, wd_buf,
            xl_buf, q_buf, ql_buf, ol_buf, inv_buf, y_buf, sems):
    k32, v32 = k_buf.bitcast(u32), v_buf.bitcast(u32)
    wg32, wu32, wd32 = wg_buf.bitcast(u32), wu_buf.bitcast(u32), wd_buf.bitcast(u32)

    win = pl.ds((SK - WIN) // 256, NJ)
    vs = V_SPLIT * RT
    copies = {}

    def copy(name, src, dst):
        copies[name] = pltpu.make_async_copy(src, dst, sems.at[len(copies)])

    copy("x", x_hbm, x_buf)
    for i in range(2):
        copy(("wq", i), wq_hbm.at[:, i, :, pl.ds(0, 16), :],
             k_buf.at[pl.ds(WQ2_ROW + i * D // 16, D // 16)])
        copy(("wq", 2 + i), wq_hbm.at[:, i, :, pl.ds(16, 8), :],
             k_buf.at[pl.ds(WQ1_ROW, D // 16), :, pl.ds(8 * i, 8), :])
    copy("wo", wo_hbm, k_buf.at[pl.ds(WO_ROW, WO_ROWS)])
    copy("k", k_hbm.at[:, win], k_buf.at[pl.ds(0, NRT)])
    copy("v0", v_hbm.at[pl.ds(0, vs), win], v_buf.at[pl.ds(0, vs)])
    copy("v1", v_hbm.at[pl.ds(vs, NRT - 16 - vs), win], v_buf.at[pl.ds(vs, NRT - 16 - vs)])
    copy("v2", v_hbm.at[pl.ds(NRT - 16, 16), win], k_buf.at[pl.ds(VT_ROW, 16)])
    copy("wg", wg_hbm, wg_buf)
    copy("wu", wu_hbm, wu_buf)
    for i in range(2):
        rows = pl.ds(i * F // 32, F // 32)
        copy(("wd", i), wd_hbm.at[rows], wd_buf.at[rows])
    for cp in copies.values():
        cp.start()

    def wait(cond, *names):
        @pl.when(cond)
        def _():
            for name in names:
                copies[name].wait()


    def put(ref, row, i, x):
        ref[row + i // 16, i % 16] = pltpu.bitcast(x, u32)

    def get(ref, row, i):
        return pltpu.bitcast(ref[row + i // 16, i % 16], f32)

    def q_jobs(n):
        def make(u):
            def job():
                if u < 2 * NC:
                    w = [k32[WQ2_ROW + (a % 2) * (D // 16) + a // 2, n]
                         for a in range(8 * u, 8 * u + 8)]
                    w = pltpu.bitcast(jnp.concatenate(w, axis=0), bf16)
                else:
                    w = _packed(k32[pl.ds(WQ1_ROW + 8 * (u - 2 * NC), 8), n])
                r = _dot(xl_buf[u], w)
                return lambda: put(v32, Q_ROW, u, r)
            return job
        return [make(u) for u in range(3 * NC)]

    def q_sum(zero):
        parts = pltpu.bitcast(v32[zero + Q_ROW, pl.ds(0, 3 * NC)], f32)
        q_buf[0] = parts[:2 * NC].sum(axis=0) * q_buf[2]
        q_buf[1] = parts[2 * NC:].sum(axis=0) * q_buf[2]

    def q_lhs(e):
        for t in range(3):
            m = (3 * e + t) // 2
            q = _row(q_buf[0], m) if m < 2 else q_buf[1]
            ql_buf[e, t] = _split_parity(_spread(q, (3 * e + t) % 2))

    def qk_jobs(n, e):
        def make(j, t):
            def job():
                w = _packed(k32[pl.ds(n * 2 * RT + e * RT + 8 * t, 8), j])
                r = pltpu.bitcast(_dot(ql_buf[e, t], w), u32)

                def drain():
                    lo = 2 * (j % 4)
                    v32[S_ROW + e, 4 * t + j // 4, pl.ds(lo, 2), :] = r[lo:lo + 2, :]
                return drain
            return job
        return [make(j, t) for j in range(NJ) for t in range(3)]

    def softmax(e, slot, zero):
        parts = pltpu.bitcast(v32[zero + S_ROW + e, pl.ds(0, 12)], f32)
        s = (parts[0:4] + parts[4:8] + parts[8:12]).reshape(32, 128) * (DH ** -0.5)
        p = jnp.exp(s - jnp.concatenate([_reduce(jnp.max, s)] * 4, axis=0))
        inv_buf[slot] = 1.0 / _reduce(jnp.sum, p)

        def publish():
            for i in range(4):
                put(v32, S_ROW + e, 12 + i, p[8 * i:8 * i + 8])
        return publish

    def expand(e, part, zero):
        for c in range(32 * part // EXN, 32 * (part + 1) // EXN):
            row = pltpu.bitcast(v32[zero + S_ROW + e, 12 + c // 8, pl.ds(c % 8, 1), :], f32)
            put(k32, P_ROW + 2 * e, c, jnp.broadcast_to(row, (8, 128)))

    def pv_steps(n, e, tiles=RT):
        acc = [None] * RS

        def make(r0, j0):
            def step():
                for j in range(j0, j0 + JS):
                    p0, p1 = get(k32, P_ROW + 2 * e, 2 * j), get(k32, P_ROW + 2 * e, 2 * j + 1)
                    for r in range(min(RS, tiles - r0)):
                        v = v_buf[n * 2 * RT + e * RT + r0 + r, j].astype(f32)
                        t = v[0:8] * p0 + v[8:16] * p1
                        acc[r] = t if j == 0 else acc[r] + t
                for r in range(min(RS, tiles - r0)):
                    if j0 + JS < NJ:
                        if r >= SN:
                            put(k32, A_ROW + 1, 8 + r, acc[r])
                        continue
                    rt = e * RT + r0 + r
                    k_buf[A_ROW + rt // 32, (rt // 2) % 16, pl.ds(8 * (rt % 2), 8), :] = (
                        acc[r].astype(bf16))
            return step
        return [make(r0, j0) for r0 in range(0, tiles, RS) for j0 in range(0, NJ, JS)]

    def out_job(t, zero):
        def job():
            w = _packed(k32[zero + A_ROW + t // 2, pl.ds(8 * (t % 2), 8)])
            r = lax.dot_general(jnp.ones((16, 128), bf16), w, (((1,), (XP,)), ((), ())),
                                preferred_element_type=f32)[0:8]
            return lambda: put(v32, O_ROW, t, r)
        return job

    def pv_jobs(zero):
        def make(j, odd):
            def job():
                w = [k32[zero + VT_ROW + r, j] for r in range(odd, 16, 2)]
                r = lax.dot_general(xl_buf[j], pltpu.bitcast(jnp.concatenate(w, axis=0), bf16),
                                    (((1,), (1,)), ((), ())), preferred_element_type=f32)[0:8]
                return lambda: put(v32, Q_ROW, j, r) if odd else put(v32, Z_ROW, j, r)
            return job
        return [make(j, odd) for j in range(NJ) for odd in range(2)]

    def pv_lhs():
        for j in range(NJ):
            p = get(v32, S_ROW + 1, 12 + j // 4)
            xl_buf[j] = _operand(jnp.where(_iota(0) // 2 == j % 4, p, 0.0))

    def pv_finish():
        lane, halves = _iota(1), []
        for row in (Z_ROW, Q_ROW):
            a = pltpu.bitcast(v32[row], f32).sum(axis=0)
            a = jnp.where(_iota(0) % 2 == (lane // 8) % 2, a, 0.0).sum(axis=0, keepdims=True)
            a = jnp.broadcast_to(a, (8, 128))
            halves.append((a + jnp.take_along_axis(a, lane ^ 8, axis=1)) * inv_buf[1])
        ol_buf[2, 0] = _split_parity(halves[0])
        ol_buf[2, 1] = _split_parity(jnp.where((lane // 8) % 2 == 0, *halves))
        ol_buf[2, 2] = _split_parity(halves[1])

    def normalise(t):
        inv = (inv_buf[0] if t == 0 else inv_buf[1] if t == 2 else
               jnp.where(_iota(1) < DH - 128, inv_buf[0], inv_buf[1]))
        for i, tile in enumerate(_ragged_operands(get(v32, O_ROW, t) * inv)):
            ol_buf[t, i] = tile

    def wo_jobs(n, direct=False):
        at = [(WO_ROW + (i >> 1), 8 * (i & 1)) for i in (3 * NC * n, 3 * NC * n + 1)]

        def make(t, m):
            def job():
                w = [k32[at[i // 8 % 2][0] + i // 16, at[i // 8 % 2][1] + i % 8]
                     for i in range(8 * NC * t + m, 8 * NC * (t + 1), NC)]
                r = _dot(ol_buf[t, RAGGED[m]], pltpu.bitcast(jnp.concatenate(w, axis=0), bf16))
                return r if direct else lambda: put(v32, Y_ROW, NC * t + m, r)
            return job
        return [make(t, m) for t in range(3) for m in range(NC)]

    def y_sum(m, zero):
        parts = [get(v32, zero + Y_ROW, NC * t + m) for t in range(3)]
        y_buf[m] += parts[0] + parts[1] + parts[2]

    def run(jobs):
        for drain in [job() for job in jobs]:
            drain()

    def interleave(*plans):
        hooks, steps, groups = zip(*[slot for plan in plans for slot in plan])
        ns = len(steps)
        pending = {g: [job() for job in groups[g]] for g in range(LEAD)}
        for g, step in enumerate(steps):
            for drain in pending.pop(g - LAG, ()):
                drain()
            for hook in hooks[g]:
                hook()
            step()
            if g + LEAD < ns:
                pending[g + LEAD] = [job() for job in groups[g + LEAD]]
        for g in sorted(pending):
            for drain in pending[g]:
                drain()

    def pair(n, first=False, last=False):
        zero = n >> 8
        steps = pv_steps(n, 0)
        half = len(steps)
        steps += pv_steps(n, 1, RT - 16 if last else RT)
        hooks = {}

        def at(g, fn, *args):
            hooks.setdefault(g, []).append(lambda: fn(*args))

        def softmax_at(g, e, ps=PS):
            result = []
            at(g, lambda: result.append(softmax(e, 3 - e, zero)))
            at(g + ps, lambda: result[0]())
            for part in range(EXN):
                at(g + ps + 1 + part * EXS, expand, e, part, zero)

        def rotate():
            inv_buf[0] = inv_buf[3]
            inv_buf[1] = inv_buf[2]

        softmax_at(0 if last else SM, 1, LPS if last else PS)
        at(RO, rotate)
        head, tail = [None] * 3, [None] * (3 * NC)
        if not first:
            head, tail = [out_job(t, zero) for t in range(3)], wo_jobs(n - 1)
            for t in range(3):
                at(OUT0 + t * OS, normalise, t)
            for m in range(NC):
                at(YS + m * YSS, y_sum, m, zero)
        if last:
            groups = [[] for _ in steps]
            groups[0] = head
            at(LPS, pv_lhs)
            for i, job in enumerate(pv_jobs(zero)):
                groups[LPS + LEAD + i * LJ // 16].append(job)
        else:
            middle = qk_jobs(n + 1, 0) + q_jobs(jnp.minimum(n + 2, NP - 1)) + qk_jobs(n + 1, 1)
            softmax_at(half + SM0, 0, PS0)
            at(QS, q_sum, zero)
            at(QL0, q_lhs, 0)
            at(QL1, q_lhs, 1)
            jobs = head + middle + tail
            extra = len(jobs) - 4 * len(steps)
            groups = [[job for job in jobs[4 * g + extra * (g > EXTRA):4 * g + 4 + extra * (g >= EXTRA)] if job]
                      for g in range(len(steps))]
        assert max(hooks) < len(steps)
        return [(hooks.get(g, ()), step, groups[g]) for g, step in enumerate(steps)]

    def attention(x, cold, zero):
        wait(cold, *[("wq", i) for i in range(4)], "wo", "k")
        xc, tiles, q_buf[2] = _layernorm(x)
        for u, tile in enumerate(tiles):
            xl_buf[u] = tile
        for c in range(NC):
            xl_buf[2 * NC + c] = _operand(_row(xc, c))
            y_buf[c] = jnp.zeros((8, 128), f32)
        for i in range(3 * NC):
            put(v32, Y_ROW, i, jnp.zeros((8, 128), f32))
        run(q_jobs(0))
        q_sum(0)
        q_lhs(0)
        q_lhs(1)
        run(q_jobs(1) + qk_jobs(0, 0))
        softmax(0, 3, 0)()
        for part in range(EXN):
            expand(0, part, 0)
        run(qk_jobs(0, 1))
        q_sum(0)
        q_lhs(0)
        q_lhs(1)
        wait(cold, "v0")
        if not ONLY:
            interleave(pair(zero, first=True), *[pair(zero + i) for i in range(1, U0)])

        def body(i, carry):
            n = U0 + i * U
            wait(jnp.logical_and(cold, n == V_SPLIT // 2), "v1", "v2")
            interleave(*[pair(n + i) for i in range(U)])
            return carry

        trips = (NP - U0 - U1) // U
        assert U0 + trips * U + U1 == NP
        if trips:
            lax.fori_loop(0, trips, body, 0)
        if ONLY:
            return x + y_buf[0]
        interleave(*[pair(zero + i) for i in range(NP - U1, NP - 1)],
                   pair(zero + (NP - 1), last=True))
        drains = [out_job(t, 0)() for t in range(2)]
        parts = [job() for job in wo_jobs(NP - 2, True)]
        pv_finish()
        for t, drain in enumerate(drains):
            drain()
            normalise(t)
        jobs = wo_jobs(NP - 1, True)
        parts += [job() for job in jobs[2 * NC:] + jobs[:2 * NC]]
        return x + _ragged_result([sum(parts[m::NC], y_buf[m]) for m in range(NC)])

    def glu(x, cold):
        def arrive(name):
            if cold:
                copies[name].wait()

        arrive("wg")
        arrive("wu")
        _, tiles, rstd = _layernorm(x)
        xl = jnp.concatenate(tiles, axis=1)
        hid = []
        for b in range(NFB):
            g = _dot(xl, _packed(wg32[:, pl.ds(8 * b, 8), :])) * rstd
            u = _dot(xl, _packed(wu32[:, pl.ds(8 * b, 8), :])) * rstd
            h = jax.nn.sigmoid(g) * u
            hid += [_ragged_operands(_row(h, par)) for par in range(2)]
        out = [0.0] * NC
        for i, chunk in enumerate(hid):
            if i % NFB == 0:
                arrive(("wd", i // NFB))
            for m in range(NC):
                out[m] += _dot(chunk[RAGGED[m]], _packed(wd32[pl.ds(8 * i, 8), m]))
        return x + _ragged_result(out)

    copies["x"].wait()
    x_in = x_buf[...].astype(f32)
    x0 = _stack_rows([jnp.broadcast_to(x_in[:, c * 128:(c + 1) * 128], (8, 128))
                      for c in range(NC)])

    def layer(i, x):
        x = attention(x, i == 0, i >> 8)
        if ONLY:
            return x
        x = lax.cond(i == 0, lambda: glu(x, True), lambda: glu(x, False))
        return x

    x_out = lax.fori_loop(0, LAYERS, layer, x0)
    out_ref[...] = jnp.concatenate(
        [x_out[c:c + 1, :] for c in range(NC)], axis=1).astype(out_ref.dtype)


def _tile_order(w, *shape):
    r, c = w.shape
    w = w.reshape(r // 8, 8, c // 128, 128)
    return jnp.transpose(w, (0, 2, 1, 3)).reshape(*shape, 128)


@jax.jit
def pallas_interleave_layers__sliding_block_cached__glu_gated_glu__decode_kernel(
    A_x: jax.Array,
    A_k_cache: jax.Array,
    A_v_cache: jax.Array,
    A_wq: jax.Array,
    A_wo: jax.Array,
    B_x: jax.Array,
    B_w_gate: jax.Array,
    B_w_up: jax.Array,
    B_w_down: jax.Array,
):
    del B_x
    k, v = [_tile_order(jnp.swapaxes(a, 2, 3).reshape(H * DH, SK), NRT, SK // 256, 16)
            for a in (A_k_cache, A_v_cache)]
    out = pl.pallas_call(
        _kernel,
        out_shape=jax.ShapeDtypeStruct((1, D), A_x.dtype),
        in_specs=[pl.BlockSpec(memory_space=pltpu.HBM)] * 8,
        out_specs=pl.BlockSpec(memory_space=pltpu.VMEM),
        scratch_shapes=[
            pltpu.VMEM((1, D), bf16),
            pltpu.VMEM((P_ROW + 4, 16, 16, 128), bf16),
            pltpu.VMEM((Y_ROW + 1, 16, 16, 128), bf16),
            pltpu.VMEM((D // 8, F // 16, 128), bf16),
            pltpu.VMEM((D // 8, F // 16, 128), bf16),
            pltpu.VMEM((F // 16, NC, 16, 128), bf16),
            pltpu.VMEM((NJ, 16, 128), bf16),
            pltpu.VMEM((3, 8, 128), f32),
            pltpu.VMEM((2, 3, 16, 128), bf16),
            pltpu.VMEM((3, 3, 16, 128), bf16),
            pltpu.VMEM((4, 8, 128), f32),
            pltpu.VMEM((NC, 8, 128), f32),
            pltpu.SemaphoreType.DMA((14,)),
        ],
        compiler_params=pltpu.CompilerParams(vmem_limit_bytes=124 * 1024 * 1024),
    )(A_x.reshape(1, D), k, v,
      _tile_order(A_wq, D // 16, 2, NP, 24), _tile_order(A_wo, WO_ROWS, 16, 16),
      _tile_order(B_w_gate, D // 8, F // 16), _tile_order(B_w_up, D // 8, F // 16),
      _tile_order(B_w_down, F // 16, NC, 16))
    return out.reshape(A_x.shape)
```

```python
import jax
import jax.numpy as jnp
from jax import lax
import jax.experimental.pallas as pl
import jax.experimental.pallas.tpu as pltpu

D = 640
H = 32
DH = 192
F = 1536
SK = 32768
WIN = min(4096, max(256, SK // 4))
EPS = 1e-5
LAYERS = 2
KO = 4
SB = 0
JM = 1
JA = 0
AO = 0
PB = 0
AB = 0
QF = 0
WF = 0
SN = 2
LPS = 3
LJ = 8
QL0 = 30
QL1 = 27
SM0 = 1
PS0 = 7
EXS = 2
OS = 1
YSS = 1
RO = 16
EXTRA = 1
ONLY = 0
U0, U, U1 = 1, 1, 1
XP = 1

NC = D // 128
NP = H // 2
RT = DH // 8
NRT = H * RT
NJ = WIN // 256
NFB = F // 256
V_SPLIT = 24

WO_ROWS = H * DH * D // (256 * 128)
WQ2_ROW = NRT
WQ1_ROW = WQ2_ROW + D // 8
WO_ROW = WQ1_ROW + D // 16
VT_ROW = WO_ROW + WO_ROWS
A_ROW = VT_ROW + 16
P_ROW = A_ROW + 2
S_ROW = NRT - 16
Q_ROW = S_ROW + 2
O_ROW = Q_ROW + 1
Z_ROW = O_ROW + 1
Y_ROW = Z_ROW + 1

RS = 3
JS = 8
LAG = 4
LEAD = 3
SM = 1
PS = 5
EXN = 4
OUT0 = 8
YS = 14
QS = 23

f32, bf16, u32 = jnp.float32, jnp.bfloat16, jnp.uint32


def _iota(axis):
    return lax.broadcasted_iota(jnp.int32, (8, 128), axis)


def _operand(x):
    return jnp.concatenate([x, x], axis=0).astype(bf16)


def _dot(a, b):
    return jnp.dot(a, b, preferred_element_type=f32)[0:8]


def _packed(words):
    return pltpu.bitcast(words.reshape(words.shape[0] * 8, 128), bf16)


def _row(x, r):
    return jnp.broadcast_to(x[r:r + 1, :], (8, 128))


def _spread(x, half):
    lane = _iota(1)
    return jnp.take_along_axis(x, (lane // 16) * 8 + lane % 8 + 64 * half, axis=1)


def _split_parity(x):
    keep = (_iota(0) % 2) == ((_iota(1) // 8) % 2)
    return _operand(jnp.where(keep, x, 0.0))


def _reduce(fn, x):
    x = fn(x.reshape(-1, 8, 128), axis=0)
    return jnp.broadcast_to(fn(fn(x, axis=0, keepdims=True), axis=1, keepdims=True), (8, 128))


def _layernorm(x):
    mean = _reduce(jnp.sum, x) * (1.0 / D)
    xc = jnp.where(_iota(0) < NC, x - mean, 0.0)
    rstd = lax.rsqrt(_reduce(jnp.sum, xc * xc) * (1.0 / D) + EPS)
    halves = [_spread(x, half) - mean for half in range(2)]
    return xc, [_split_parity(_row(halves[u % 2], u // 2)) for u in range(2 * NC)], rstd


def _stack_rows(rows):
    out = jnp.zeros((8, 128), f32)
    for c, r in enumerate(rows):
        out = jnp.where(_iota(0) == c, r, out)
    return out


RAGGED = (0, 0, 1, 2, 2)


def _ragged_operands(x):
    lane = _iota(1)
    first = (lane // 16) * 16 + lane % 8
    return [_split_parity(jnp.take_along_axis(x, first, axis=1)), _split_parity(x),
            _split_parity(jnp.take_along_axis(x, first + 8, axis=1))]


def _ragged_result(parts):
    tiles = [_row(parts[i // 2], i % 2) for i in range(2 * NC)]
    return _stack_rows([tiles[c] + tiles[NC + c] for c in range(NC)])


def _kernel(x_hbm, k_hbm, v_hbm, wq_hbm, wo_hbm, wg_hbm, wu_hbm, wd_hbm, out_ref,
            x_buf, k_buf, v_buf, wg_buf, wu_buf, wd_buf,
            xl_buf, q_buf, ql_buf, ol_buf, inv_buf, y_buf, sems):
    k32, v32 = k_buf.bitcast(u32), v_buf.bitcast(u32)
    wg32, wu32, wd32 = wg_buf.bitcast(u32), wu_buf.bitcast(u32), wd_buf.bitcast(u32)

    win = pl.ds((SK - WIN) // 256, NJ)
    vs = V_SPLIT * RT
    copies = {}

    def copy(name, src, dst):
        copies[name] = pltpu.make_async_copy(src, dst, sems.at[len(copies)])

    copy("x", x_hbm, x_buf)
    for i in range(2):
        copy(("wq", i), wq_hbm.at[:, i, :, pl.ds(0, 16), :],
             k_buf.at[pl.ds(WQ2_ROW + i * D // 16, D // 16)])
        copy(("wq", 2 + i), wq_hbm.at[:, i, :, pl.ds(16, 8), :],
             k_buf.at[pl.ds(WQ1_ROW, D // 16), :, pl.ds(8 * i, 8), :])
    copy("wo", wo_hbm, k_buf.at[pl.ds(WO_ROW, WO_ROWS)])
    copy("k", k_hbm.at[:, win], k_buf.at[pl.ds(0, NRT)])
    copy("v0", v_hbm.at[pl.ds(0, vs), win], v_buf.at[pl.ds(0, vs)])
    copy("v1", v_hbm.at[pl.ds(vs, NRT - 16 - vs), win], v_buf.at[pl.ds(vs, NRT - 16 - vs)])
    copy("v2", v_hbm.at[pl.ds(NRT - 16, 16), win], k_buf.at[pl.ds(VT_ROW, 16)])
    copy("wg", wg_hbm, wg_buf)
    copy("wu", wu_hbm, wu_buf)
    for i in range(2):
        rows = pl.ds(i * F // 32, F // 32)
        copy(("wd", i), wd_hbm.at[rows], wd_buf.at[rows])
    for cp in copies.values():
        cp.start()

    def wait(cond, *names):
        @pl.when(cond)
        def _():
            for name in names:
                copies[name].wait()


    def put(ref, row, i, x):
        ref[row + i // 16, i % 16] = pltpu.bitcast(x, u32)

    def get(ref, row, i):
        return pltpu.bitcast(ref[row + i // 16, i % 16], f32)

    def q_jobs(n):
        def make(u):
            def job():
                if u < 2 * NC:
                    w = [k32[WQ2_ROW + (a % 2) * (D // 16) + a // 2, n]
                         for a in range(8 * u, 8 * u + 8)]
                    w = pltpu.bitcast(jnp.concatenate(w, axis=0), bf16)
                else:
                    w = _packed(k32[pl.ds(WQ1_ROW + 8 * (u - 2 * NC), 8), n])
                r = _dot(xl_buf[u], w)
                return lambda: put(v32, Q_ROW, u, r)
            return job
        return [make(u) for u in range(3 * NC)]

    def q_sum(zero):
        parts = pltpu.bitcast(v32[zero + Q_ROW, pl.ds(0, 3 * NC)], f32)
        q_buf[0] = parts[:2 * NC].sum(axis=0) * q_buf[2]
        q_buf[1] = parts[2 * NC:].sum(axis=0) * q_buf[2]

    def q_lhs(e):
        for t in range(3):
            m = (3 * e + t) // 2
            q = _row(q_buf[0], m) if m < 2 else q_buf[1]
            ql_buf[e, t] = _split_parity(_spread(q, (3 * e + t) % 2))

    def qk_jobs(n, e):
        def make(j, t):
            def job():
                w = _packed(k32[pl.ds(n * 2 * RT + e * RT + 8 * t, 8), j])
                r = pltpu.bitcast(_dot(ql_buf[e, t], w), u32)

                def drain():
                    lo = 2 * (j % 4)
                    v32[S_ROW + e, 4 * t + (j // 4 + SB * t) % 4, pl.ds(lo, 2), :] = r[lo:lo + 2, :]
                return drain
            return job
        return [make(j0 + j, t) for j0 in range(0, NJ, KO) for t in range(3) for j in range(KO)]

    def softmax(e, slot, zero):
        parts = pltpu.bitcast(v32[zero + S_ROW + e, pl.ds(0, 12)], f32)
        s = jnp.concatenate(
            [parts[i] + parts[4 + (i + SB) % 4] + parts[8 + (i + 2 * SB) % 4] for i in range(4)],
            axis=0) * (DH ** -0.5)
        p = jnp.exp(s - jnp.concatenate([_reduce(jnp.max, s)] * 4, axis=0))
        inv_buf[slot] = 1.0 / _reduce(jnp.sum, p)

        def publish():
            for i in range(4):
                put(v32, S_ROW + e, 12 + i, p[8 * i:8 * i + 8])
        return publish

    def expand(e, part, zero):
        for c in range(32 * part // EXN, 32 * (part + 1) // EXN):
            row = pltpu.bitcast(v32[zero + S_ROW + e, 12 + c // 8, pl.ds(c % 8, 1), :], f32)
            put(k32, P_ROW + 2 * e, (c + PB) % 32, jnp.broadcast_to(row, (8, 128)))

    def pv_steps(n, e, tiles=RT):
        acc = [None] * RS

        def make(r0, j0):
            def step():
                for j in range(j0, j0 + JS):
                    start = j == 0
                    j = (j * JM + JA) % NJ
                    p0, p1 = [get(k32, P_ROW + 2 * e, (2 * j + i + PB) % 32) for i in range(2)]
                    for r in range(min(RS, tiles - r0)):
                        v = v_buf[n * 2 * RT + e * RT + r0 + r, j].astype(f32)
                        if AO and not start:
                            acc[r] = acc[r] + v[0:8] * p0 + v[8:16] * p1
                            continue
                        t = v[0:8] * p0 + v[8:16] * p1
                        acc[r] = t if start else acc[r] + t
                for r in range(min(RS, tiles - r0)):
                    if j0 + JS < NJ:
                        if r >= SN:
                            put(k32, A_ROW + 1, 8 + r + AB, acc[r])
                        continue
                    rt = e * RT + r0 + r
                    k_buf[A_ROW + rt // 32, (rt // 2) % 16, pl.ds(8 * (rt % 2), 8), :] = (
                        acc[r].astype(bf16))
            return step
        return [make(r0, j0) for r0 in range(0, tiles, RS) for j0 in range(0, NJ, JS)]

    def out_job(t, zero):
        def job():
            w = _packed(k32[zero + A_ROW + t // 2, pl.ds(8 * (t % 2), 8)])
            r = lax.dot_general(jnp.ones((16, 128), bf16), w, (((1,), (XP,)), ((), ())),
                                preferred_element_type=f32)[0:8]
            return lambda: put(v32, O_ROW, t, r)
        return job

    def pv_jobs(zero):
        def make(j, odd):
            def job():
                w = [k32[zero + VT_ROW + r, j] for r in range(odd, 16, 2)]
                r = lax.dot_general(xl_buf[j], pltpu.bitcast(jnp.concatenate(w, axis=0), bf16),
                                    (((1,), (1,)), ((), ())), preferred_element_type=f32)[0:8]
                return lambda: put(v32, Q_ROW, j, r) if odd else put(v32, Z_ROW, j, r)
            return job
        return [make(j, odd) for j in range(NJ) for odd in range(2)]

    def pv_lhs():
        for j in range(NJ):
            p = get(v32, S_ROW + 1, 12 + j // 4)
            xl_buf[j] = _operand(jnp.where(_iota(0) // 2 == j % 4, p, 0.0))

    def pv_finish():
        lane, halves = _iota(1), []
        for row in (Z_ROW, Q_ROW):
            a = pltpu.bitcast(v32[row], f32).sum(axis=0)
            a = jnp.where(_iota(0) % 2 == (lane // 8) % 2, a, 0.0).sum(axis=0, keepdims=True)
            a = jnp.broadcast_to(a, (8, 128))
            halves.append((a + jnp.take_along_axis(a, lane ^ 8, axis=1)) * inv_buf[1])
        ol_buf[2, 0] = _split_parity(halves[0])
        ol_buf[2, 1] = _split_parity(jnp.where((lane // 8) % 2 == 0, *halves))
        ol_buf[2, 2] = _split_parity(halves[1])

    def normalise(t):
        inv = (inv_buf[0] if t == 0 else inv_buf[1] if t == 2 else
               jnp.where(_iota(1) < DH - 128, inv_buf[0], inv_buf[1]))
        for i, tile in enumerate(_ragged_operands(get(v32, O_ROW, t) * inv)):
            ol_buf[t, i] = tile

    def wo_jobs(n, direct=False):
        at = [(WO_ROW + (i >> 1), 8 * (i & 1)) for i in (3 * NC * n, 3 * NC * n + 1)]

        def make(t, m):
            def job():
                w = [k32[at[i // 8 % 2][0] + i // 16, at[i // 8 % 2][1] + i % 8]
                     for i in range(8 * NC * t + m, 8 * NC * (t + 1), NC)]
                r = _dot(ol_buf[t, RAGGED[m]], pltpu.bitcast(jnp.concatenate(w, axis=0), bf16))
                return r if direct else lambda: put(v32, Y_ROW, NC * t + m, r)
            return job
        return [make(t, m) for t in range(3) for m in range(NC)]

    def y_sum(m, zero):
        parts = [get(v32, zero + Y_ROW, NC * t + m) for t in range(3)]
        y_buf[m] += parts[0] + parts[1] + parts[2]

    def run(jobs):
        for drain in [job() for job in jobs]:
            drain()

    def interleave(*plans):
        hooks, steps, groups = zip(*[slot for plan in plans for slot in plan])
        ns = len(steps)
        pending = {g: [job() for job in groups[g]] for g in range(LEAD)}
        for g, step in enumerate(steps):
            for drain in pending.pop(g - LAG, ()):
                drain()
            for hook in hooks[g]:
                hook()
            step()
            if g + LEAD < ns:
                pending[g + LEAD] = [job() for job in groups[g + LEAD]]
        for g in sorted(pending):
            for drain in pending[g]:
                drain()

    def pair(n, first=False, last=False):
        zero = n >> 8
        steps = pv_steps(n, 0)
        half = len(steps)
        steps += pv_steps(n, 1, RT - 16 if last else RT)
        hooks = {}

        def at(g, fn, *args):
            hooks.setdefault(g, []).append(lambda: fn(*args))

        def softmax_at(g, e, ps=PS):
            result = []
            at(g, lambda: result.append(softmax(e, 3 - e, zero)))
            at(g + ps, lambda: result[0]())
            for part in range(EXN):
                at(g + ps + 1 + part * EXS, expand, e, part, zero)

        def rotate():
            inv_buf[0] = inv_buf[3]
            inv_buf[1] = inv_buf[2]

        softmax_at(0 if last else SM, 1, LPS if last else PS)
        at(RO, rotate)
        head, tail = [None] * 3, [None] * (3 * NC)
        if not first:
            head, tail = [out_job(t, zero) for t in range(3)], wo_jobs(n - 1)
            for t in range(3):
                at(OUT0 + t * OS, normalise, t)
            for m in range(NC):
                at(YS + m * YSS, y_sum, m, zero)
        if last:
            groups = [[] for _ in steps]
            groups[0] = head
            at(LPS, pv_lhs)
            for i, job in enumerate(pv_jobs(zero)):
                groups[LPS + LEAD + i * LJ // 16].append(job)
        else:
            q = q_jobs(jnp.minimum(n + 2, NP - 1))
            middle = q[:QF] + qk_jobs(n + 1, 0) + q[QF:] + tail[:WF] + qk_jobs(n + 1, 1)
            tail = tail[WF:]
            softmax_at(half + SM0, 0, PS0)
            at(QS, q_sum, zero)
            at(QL0, q_lhs, 0)
            at(QL1, q_lhs, 1)
            jobs = head + middle + tail
            extra = len(jobs) - 4 * len(steps)
            groups = [[job for job in jobs[4 * g + extra * (g > EXTRA):4 * g + 4 + extra * (g >= EXTRA)] if job]
                      for g in range(len(steps))]
        assert max(hooks) < len(steps)
        return [(hooks.get(g, ()), step, groups[g]) for g, step in enumerate(steps)]

    def attention(x, cold, zero):
        wait(cold, *[("wq", i) for i in range(4)], "wo", "k")
        xc, tiles, q_buf[2] = _layernorm(x)
        for u, tile in enumerate(tiles):
            xl_buf[u] = tile
        for c in range(NC):
            xl_buf[2 * NC + c] = _operand(_row(xc, c))
            y_buf[c] = jnp.zeros((8, 128), f32)
        for i in range(3 * NC):
            put(v32, Y_ROW, i, jnp.zeros((8, 128), f32))
        run(q_jobs(0))
        q_sum(0)
        q_lhs(0)
        q_lhs(1)
        run(q_jobs(1) + qk_jobs(0, 0))
        softmax(0, 3, 0)()
        for part in range(EXN):
            expand(0, part, 0)
        run(qk_jobs(0, 1))
        q_sum(0)
        q_lhs(0)
        q_lhs(1)
        wait(cold, "v0")
        if not ONLY:
            interleave(pair(zero, first=True), *[pair(zero + i) for i in range(1, U0)])

        def body(i, carry):
            n = U0 + i * U
            wait(jnp.logical_and(cold, n == V_SPLIT // 2), "v1", "v2")
            interleave(*[pair(n + i) for i in range(U)])
            return carry

        trips = (NP - U0 - U1) // U
        assert U0 + trips * U + U1 == NP
        if trips:
            lax.fori_loop(0, trips, body, 0)
        if ONLY:
            return x + y_buf[0]
        interleave(*[pair(zero + i) for i in range(NP - U1, NP - 1)],
                   pair(zero + (NP - 1), last=True))
        drains = [out_job(t, 0)() for t in range(2)]
        parts = [job() for job in wo_jobs(NP - 2, True)]
        pv_finish()
        for t, drain in enumerate(drains):
            drain()
            normalise(t)
        jobs = wo_jobs(NP - 1, True)
        parts += [job() for job in jobs[2 * NC:] + jobs[:2 * NC]]
        return x + _ragged_result([sum(parts[m::NC], y_buf[m]) for m in range(NC)])

    def glu(x, cold):
        def arrive(name):
            if cold:
                copies[name].wait()

        arrive("wg")
        arrive("wu")
        _, tiles, rstd = _layernorm(x)
        xl = jnp.concatenate(tiles, axis=1)
        hid = []
        for b in range(NFB):
            g = _dot(xl, _packed(wg32[:, pl.ds(8 * b, 8), :])) * rstd
            u = _dot(xl, _packed(wu32[:, pl.ds(8 * b, 8), :])) * rstd
            h = jax.nn.sigmoid(g) * u
            hid += [_ragged_operands(_row(h, par)) for par in range(2)]
        out = [0.0] * NC
        for i, chunk in enumerate(hid):
            if i % NFB == 0:
                arrive(("wd", i // NFB))
            for m in range(NC):
                out[m] += _dot(chunk[RAGGED[m]], _packed(wd32[pl.ds(8 * i, 8), m]))
        return x + _ragged_result(out)

    copies["x"].wait()
    x_in = x_buf[...].astype(f32)
    x0 = _stack_rows([jnp.broadcast_to(x_in[:, c * 128:(c + 1) * 128], (8, 128))
                      for c in range(NC)])

    def layer(i, x):
        x = attention(x, i == 0, i >> 8)
        if ONLY:
            return x
        x = lax.cond(i == 0, lambda: glu(x, True), lambda: glu(x, False))
        return x

    x_out = lax.fori_loop(0, LAYERS, layer, x0)
    out_ref[...] = jnp.concatenate(
        [x_out[c:c + 1, :] for c in range(NC)], axis=1).astype(out_ref.dtype)


def _tile_order(w, *shape):
    r, c = w.shape
    w = w.reshape(r // 8, 8, c // 128, 128)
    return jnp.transpose(w, (0, 2, 1, 3)).reshape(*shape, 128)


@jax.jit
def pallas_interleave_layers__sliding_block_cached__glu_gated_glu__decode_kernel(
    A_x: jax.Array,
    A_k_cache: jax.Array,
    A_v_cache: jax.Array,
    A_wq: jax.Array,
    A_wo: jax.Array,
    B_x: jax.Array,
    B_w_gate: jax.Array,
    B_w_up: jax.Array,
    B_w_down: jax.Array,
):
    del B_x
    k, v = [_tile_order(jnp.swapaxes(a, 2, 3).reshape(H * DH, SK), NRT, SK // 256, 16)
            for a in (A_k_cache, A_v_cache)]
    out = pl.pallas_call(
        _kernel,
        out_shape=jax.ShapeDtypeStruct((1, D), A_x.dtype),
        in_specs=[pl.BlockSpec(memory_space=pltpu.HBM)] * 8,
        out_specs=pl.BlockSpec(memory_space=pltpu.VMEM),
        scratch_shapes=[
            pltpu.VMEM((1, D), bf16),
            pltpu.VMEM((P_ROW + 4, 16, 16, 128), bf16),
            pltpu.VMEM((Y_ROW + 1, 16, 16, 128), bf16),
            pltpu.VMEM((D // 8, F // 16, 128), bf16),
            pltpu.VMEM((D // 8, F // 16, 128), bf16),
            pltpu.VMEM((F // 16, NC, 16, 128), bf16),
            pltpu.VMEM((NJ, 16, 128), bf16),
            pltpu.VMEM((3, 8, 128), f32),
            pltpu.VMEM((2, 3, 16, 128), bf16),
            pltpu.VMEM((3, 3, 16, 128), bf16),
            pltpu.VMEM((4, 8, 128), f32),
            pltpu.VMEM((NC, 8, 128), f32),
            pltpu.SemaphoreType.DMA((14,)),
        ],
        compiler_params=pltpu.CompilerParams(vmem_limit_bytes=124 * 1024 * 1024),
    )(A_x.reshape(1, D), k, v,
      _tile_order(A_wq, D // 16, 2, NP, 24), _tile_order(A_wo, WO_ROWS, 16, 16),
      _tile_order(B_w_gate, D // 8, F // 16), _tile_order(B_w_up, D // 8, F // 16),
      _tile_order(B_w_down, F // 16, NC, 16))
    return out.reshape(A_x.shape)
```

```python
import jax
import jax.numpy as jnp
from jax import lax
import jax.experimental.pallas as pl
import jax.experimental.pallas.tpu as pltpu

D = 640
H = 32
DH = 192
F = 1536
SK = 32768
WIN = min(4096, max(256, SK // 4))
EPS = 1e-5
LAYERS = 2
KO = 4
SB = 0
JM = 3
JA = 0
AO = 0
PB = 0
AB = 0
QF = 0
WF = 0
SN = 2
LPS = 1
LJ = 8
QL0 = 30
QL1 = 29
SM0 = 1
PS0 = 7
EXS = 2
OS = 1
YSS = 1
RO = 16
EXTRA = 1
ONLY = 0
U0, U, U1 = 1, 1, 1
XP = 1

NC = D // 128
NP = H // 2
RT = DH // 8
NRT = H * RT
NJ = WIN // 256
NFB = F // 256
V_SPLIT = 24

WO_ROWS = H * DH * D // (256 * 128)
WQ2_ROW = NRT
WQ1_ROW = WQ2_ROW + D // 8
WO_ROW = WQ1_ROW + D // 16
VT_ROW = WO_ROW + WO_ROWS
A_ROW = VT_ROW + 16
P_ROW = A_ROW + 2
S_ROW = NRT - 16
Q_ROW = S_ROW + 2
O_ROW = Q_ROW + 1
Z_ROW = O_ROW + 1
Y_ROW = Z_ROW + 1

RS = 3
JS = 8
LAG = 4
LEAD = 3
SM = 1
PS = 5
EXN = 4
OUT0 = 8
YS = 14
QS = 26

f32, bf16, u32 = jnp.float32, jnp.bfloat16, jnp.uint32


def _iota(axis):
    return lax.broadcasted_iota(jnp.int32, (8, 128), axis)


def _operand(x):
    return jnp.concatenate([x, x], axis=0).astype(bf16)


def _dot(a, b):
    return jnp.dot(a, b, preferred_element_type=f32)[0:8]


def _packed(words):
    return pltpu.bitcast(words.reshape(words.shape[0] * 8, 128), bf16)


def _row(x, r):
    return jnp.broadcast_to(x[r:r + 1, :], (8, 128))


def _spread(x, half):
    lane = _iota(1)
    return jnp.take_along_axis(x, (lane // 16) * 8 + lane % 8 + 64 * half, axis=1)


def _split_parity(x):
    keep = (_iota(0) % 2) == ((_iota(1) // 8) % 2)
    return _operand(jnp.where(keep, x, 0.0))


def _reduce(fn, x):
    x = fn(x.reshape(-1, 8, 128), axis=0)
    return jnp.broadcast_to(fn(fn(x, axis=0, keepdims=True), axis=1, keepdims=True), (8, 128))


def _layernorm(x):
    mean = _reduce(jnp.sum, x) * (1.0 / D)
    xc = jnp.where(_iota(0) < NC, x - mean, 0.0)
    rstd = lax.rsqrt(_reduce(jnp.sum, xc * xc) * (1.0 / D) + EPS)
    halves = [_spread(x, half) - mean for half in range(2)]
    return xc, [_split_parity(_row(halves[u % 2], u // 2)) for u in range(2 * NC)], rstd


def _stack_rows(rows):
    out = jnp.zeros((8, 128), f32)
    for c, r in enumerate(rows):
        out = jnp.where(_iota(0) == c, r, out)
    return out


RAGGED = (0, 0, 1, 2, 2)


def _ragged_operands(x):
    lane = _iota(1)
    first = (lane // 16) * 16 + lane % 8
    return [_split_parity(jnp.take_along_axis(x, first, axis=1)), _split_parity(x),
            _split_parity(jnp.take_along_axis(x, first + 8, axis=1))]


def _ragged_result(parts):
    tiles = [_row(parts[i // 2], i % 2) for i in range(2 * NC)]
    return _stack_rows([tiles[c] + tiles[NC + c] for c in range(NC)])


def _kernel(x_hbm, k_hbm, v_hbm, wq_hbm, wo_hbm, wg_hbm, wu_hbm, wd_hbm, out_ref,
            x_buf, k_buf, v_buf, wg_buf, wu_buf, wd_buf,
            xl_buf, q_buf, ql_buf, ol_buf, inv_buf, y_buf, sems):
    k32, v32 = k_buf.bitcast(u32), v_buf.bitcast(u32)
    wg32, wu32, wd32 = wg_buf.bitcast(u32), wu_buf.bitcast(u32), wd_buf.bitcast(u32)

    win = pl.ds((SK - WIN) // 256, NJ)
    vs = V_SPLIT * RT
    copies = {}

    def copy(name, src, dst):
        copies[name] = pltpu.make_async_copy(src, dst, sems.at[len(copies)])

    copy("x", x_hbm, x_buf)
    for i in range(2):
        copy(("wq", i), wq_hbm.at[:, i, :, pl.ds(0, 16), :],
             k_buf.at[pl.ds(WQ2_ROW + i * D // 16, D // 16)])
        copy(("wq", 2 + i), wq_hbm.at[:, i, :, pl.ds(16, 8), :],
             k_buf.at[pl.ds(WQ1_ROW, D // 16), :, pl.ds(8 * i, 8), :])
    copy("wo", wo_hbm, k_buf.at[pl.ds(WO_ROW, WO_ROWS)])
    copy("k", k_hbm.at[:, win], k_buf.at[pl.ds(0, NRT)])
    copy("v0", v_hbm.at[pl.ds(0, vs), win], v_buf.at[pl.ds(0, vs)])
    copy("v1", v_hbm.at[pl.ds(vs, NRT - 16 - vs), win], v_buf.at[pl.ds(vs, NRT - 16 - vs)])
    copy("v2", v_hbm.at[pl.ds(NRT - 16, 16), win], k_buf.at[pl.ds(VT_ROW, 16)])
    copy("wg", wg_hbm, wg_buf)
    copy("wu", wu_hbm, wu_buf)
    for i in range(2):
        rows = pl.ds(i * F // 32, F // 32)
        copy(("wd", i), wd_hbm.at[rows], wd_buf.at[rows])
    for cp in copies.values():
        cp.start()

    def wait(cond, *names):
        @pl.when(cond)
        def _():
            for name in names:
                copies[name].wait()


    def put(ref, row, i, x):
        ref[row + i // 16, i % 16] = pltpu.bitcast(x, u32)

    def get(ref, row, i):
        return pltpu.bitcast(ref[row + i // 16, i % 16], f32)

    def q_jobs(n):
        def make(u):
            def job():
                if u < 2 * NC:
                    w = [k32[WQ2_ROW + (a % 2) * (D // 16) + a // 2, n]
                         for a in range(8 * u, 8 * u + 8)]
                    w = pltpu.bitcast(jnp.concatenate(w, axis=0), bf16)
                else:
                    w = _packed(k32[pl.ds(WQ1_ROW + 8 * (u - 2 * NC), 8), n])
                r = _dot(xl_buf[u], w)
                return lambda: put(v32, Q_ROW, u, r)
            return job
        return [make(u) for u in range(3 * NC)]

    def q_sum(zero):
        parts = pltpu.bitcast(v32[zero + Q_ROW, pl.ds(0, 3 * NC)], f32)
        q_buf[0] = parts[:2 * NC].sum(axis=0) * q_buf[2]
        q_buf[1] = parts[2 * NC:].sum(axis=0) * q_buf[2]

    def q_lhs(e):
        for t in range(3):
            m = (3 * e + t) // 2
            q = _row(q_buf[0], m) if m < 2 else q_buf[1]
            ql_buf[e, t] = _split_parity(_spread(q, (3 * e + t) % 2))

    def qk_jobs(n, e):
        def make(j, t):
            def job():
                w = _packed(k32[pl.ds(n * 2 * RT + e * RT + 8 * t, 8), j])
                r = pltpu.bitcast(_dot(ql_buf[e, t], w), u32)

                def drain():
                    lo = 2 * (j % 4)
                    v32[S_ROW + e, 4 * t + (j // 4 + SB * t) % 4, pl.ds(lo, 2), :] = r[lo:lo + 2, :]
                return drain
            return job
        return [make(j0 + j, t) for j0 in range(0, NJ, KO) for t in range(3) for j in range(KO)]

    def softmax(e, slot, zero):
        parts = pltpu.bitcast(v32[zero + S_ROW + e, pl.ds(0, 12)], f32)
        s = jnp.concatenate(
            [parts[i] + parts[4 + (i + SB) % 4] + parts[8 + (i + 2 * SB) % 4] for i in range(4)],
            axis=0) * (DH ** -0.5)
        p = jnp.exp(s - jnp.concatenate([_reduce(jnp.max, s)] * 4, axis=0))
        inv_buf[slot] = 1.0 / _reduce(jnp.sum, p)

        def publish():
            for i in range(4):
                put(v32, S_ROW + e, 12 + i, p[8 * i:8 * i + 8])
        return publish

    def expand(e, part, zero):
        for c in range(32 * part // EXN, 32 * (part + 1) // EXN):
            row = pltpu.bitcast(v32[zero + S_ROW + e, 12 + c // 8, pl.ds(c % 8, 1), :], f32)
            put(k32, P_ROW + 2 * e, (c + PB) % 32, jnp.broadcast_to(row, (8, 128)))

    def pv_steps(n, e, tiles=RT):
        acc = [None] * RS

        def make(r0, j0):
            def step():
                for j in range(j0, j0 + JS):
                    start = j == 0
                    j = (j * JM + JA) % NJ
                    p0, p1 = [get(k32, P_ROW + 2 * e, (2 * j + i + PB) % 32) for i in range(2)]
                    for r in range(min(RS, tiles - r0)):
                        v = v_buf[n * 2 * RT + e * RT + r0 + r, j].astype(f32)
                        if AO and not start:
                            acc[r] = acc[r] + v[0:8] * p0 + v[8:16] * p1
                            continue
                        t = v[0:8] * p0 + v[8:16] * p1
                        acc[r] = t if start else acc[r] + t
                for r in range(min(RS, tiles - r0)):
                    if j0 + JS < NJ:
                        if r >= SN:
                            put(k32, A_ROW + 1, 8 + r + AB, acc[r])
                        continue
                    rt = e * RT + r0 + r
                    k_buf[A_ROW + rt // 32, (rt // 2) % 16, pl.ds(8 * (rt % 2), 8), :] = (
                        acc[r].astype(bf16))
            return step
        return [make(r0, j0) for r0 in range(0, tiles, RS) for j0 in range(0, NJ, JS)]

    def out_job(t, zero):
        def job():
            w = _packed(k32[zero + A_ROW + t // 2, pl.ds(8 * (t % 2), 8)])
            r = lax.dot_general(jnp.ones((16, 128), bf16), w, (((1,), (XP,)), ((), ())),
                                preferred_element_type=f32)[0:8]
            return lambda: put(v32, O_ROW, t, r)
        return job

    def pv_jobs(zero):
        def make(j, odd):
            def job():
                w = [k32[zero + VT_ROW + r, j] for r in range(odd, 16, 2)]
                r = lax.dot_general(xl_buf[j], pltpu.bitcast(jnp.concatenate(w, axis=0), bf16),
                                    (((1,), (1,)), ((), ())), preferred_element_type=f32)[0:8]
                return lambda: put(v32, Q_ROW, j, r) if odd else put(v32, Z_ROW, j, r)
            return job
        return [make(j, odd) for j in range(NJ) for odd in range(2)]

    def pv_lhs():
        for j in range(NJ):
            p = get(v32, S_ROW + 1, 12 + j // 4)
            xl_buf[j] = _operand(jnp.where(_iota(0) // 2 == j % 4, p, 0.0))

    def pv_finish():
        lane, halves = _iota(1), []
        for row in (Z_ROW, Q_ROW):
            a = pltpu.bitcast(v32[row], f32).sum(axis=0)
            a = jnp.where(_iota(0) % 2 == (lane // 8) % 2, a, 0.0).sum(axis=0, keepdims=True)
            a = jnp.broadcast_to(a, (8, 128))
            halves.append((a + jnp.take_along_axis(a, lane ^ 8, axis=1)) * inv_buf[1])
        ol_buf[2, 0] = _split_parity(halves[0])
        ol_buf[2, 1] = _split_parity(jnp.where((lane // 8) % 2 == 0, *halves))
        ol_buf[2, 2] = _split_parity(halves[1])

    def normalise(t):
        inv = (inv_buf[0] if t == 0 else inv_buf[1] if t == 2 else
               jnp.where(_iota(1) < DH - 128, inv_buf[0], inv_buf[1]))
        for i, tile in enumerate(_ragged_operands(get(v32, O_ROW, t) * inv)):
            ol_buf[t, i] = tile

    def wo_jobs(n, direct=False):
        at = [(WO_ROW + (i >> 1), 8 * (i & 1)) for i in (3 * NC * n, 3 * NC * n + 1)]

        def make(t, m):
            def job():
                w = [k32[at[i // 8 % 2][0] + i // 16, at[i // 8 % 2][1] + i % 8]
                     for i in range(8 * NC * t + m, 8 * NC * (t + 1), NC)]
                r = _dot(ol_buf[t, RAGGED[m]], pltpu.bitcast(jnp.concatenate(w, axis=0), bf16))
                return r if direct else lambda: put(v32, Y_ROW, NC * t + m, r)
            return job
        return [make(t, m) for t in range(3) for m in range(NC)]

    def y_sum(m, zero):
        parts = [get(v32, zero + Y_ROW, NC * t + m) for t in range(3)]
        y_buf[m] += parts[0] + parts[1] + parts[2]

    def run(jobs):
        for drain in [job() for job in jobs]:
            drain()

    def interleave(*plans):
        hooks, steps, groups = zip(*[slot for plan in plans for slot in plan])
        ns = len(steps)
        pending = {g: [job() for job in groups[g]] for g in range(LEAD)}
        for g, step in enumerate(steps):
            for drain in pending.pop(g - LAG, ()):
                drain()
            for hook in hooks[g]:
                hook()
            step()
            if g + LEAD < ns:
                pending[g + LEAD] = [job() for job in groups[g + LEAD]]
        for g in sorted(pending):
            for drain in pending[g]:
                drain()

    def pair(n, first=False, last=False):
        zero = n >> 8
        steps = pv_steps(n, 0)
        half = len(steps)
        steps += pv_steps(n, 1, RT - 16 if last else RT)
        hooks = {}

        def at(g, fn, *args):
            hooks.setdefault(g, []).append(lambda: fn(*args))

        def softmax_at(g, e, ps=PS):
            result = []
            at(g, lambda: result.append(softmax(e, 3 - e, zero)))
            at(g + ps, lambda: result[0]())
            for part in range(EXN):
                at(g + ps + 1 + part * EXS, expand, e, part, zero)

        def rotate():
            inv_buf[0] = inv_buf[3]
            inv_buf[1] = inv_buf[2]

        softmax_at(0 if last else SM, 1, LPS if last else PS)
        at(RO, rotate)
        head, tail = [None] * 3, [None] * (3 * NC)
        if not first:
            head, tail = [out_job(t, zero) for t in range(3)], wo_jobs(n - 1)
            for t in range(3):
                at(OUT0 + t * OS, normalise, t)
            for m in range(NC):
                at(YS + m * YSS, y_sum, m, zero)
        if last:
            groups = [[] for _ in steps]
            groups[0] = head
            at(LPS, pv_lhs)
            for i, job in enumerate(pv_jobs(zero)):
                groups[LPS + LEAD + i * LJ // 16].append(job)
        else:
            q = q_jobs(jnp.minimum(n + 2, NP - 1))
            middle = q[:QF] + qk_jobs(n + 1, 0) + q[QF:] + tail[:WF] + qk_jobs(n + 1, 1)
            tail = tail[WF:]
            softmax_at(half + SM0, 0, PS0)
            at(QS, q_sum, zero)
            at(QL0, q_lhs, 0)
            at(QL1, q_lhs, 1)
            jobs = head + middle + tail
            extra = len(jobs) - 4 * len(steps)
            groups = [[job for job in jobs[4 * g + extra * (g > EXTRA):4 * g + 4 + extra * (g >= EXTRA)] if job]
                      for g in range(len(steps))]
        assert max(hooks) < len(steps)
        return [(hooks.get(g, ()), step, groups[g]) for g, step in enumerate(steps)]

    def attention(x, cold, zero):
        wait(cold, *[("wq", i) for i in range(4)], "wo", "k")
        xc, tiles, q_buf[2] = _layernorm(x)
        for u, tile in enumerate(tiles):
            xl_buf[u] = tile
        for c in range(NC):
            xl_buf[2 * NC + c] = _operand(_row(xc, c))
            y_buf[c] = jnp.zeros((8, 128), f32)
        for i in range(3 * NC):
            put(v32, Y_ROW, i, jnp.zeros((8, 128), f32))
        run(q_jobs(0))
        q_sum(0)
        q_lhs(0)
        q_lhs(1)
        run(q_jobs(1) + qk_jobs(0, 0))
        softmax(0, 3, 0)()
        for part in range(EXN):
            expand(0, part, 0)
        run(qk_jobs(0, 1))
        q_sum(0)
        q_lhs(0)
        q_lhs(1)
        wait(cold, "v0")
        if not ONLY:
            interleave(pair(zero, first=True), *[pair(zero + i) for i in range(1, U0)])

        def body(i, carry):
            n = U0 + i * U
            wait(jnp.logical_and(cold, n == V_SPLIT // 2), "v1", "v2")
            interleave(*[pair(n + i) for i in range(U)])
            return carry

        trips = (NP - U0 - U1) // U
        assert U0 + trips * U + U1 == NP
        if trips:
            lax.fori_loop(0, trips, body, 0)
        if ONLY:
            return x + y_buf[0]
        interleave(*[pair(zero + i) for i in range(NP - U1, NP - 1)],
                   pair(zero + (NP - 1), last=True))
        drains = [out_job(t, 0)() for t in range(2)]
        parts = [job() for job in wo_jobs(NP - 2, True)]
        pv_finish()
        for t, drain in enumerate(drains):
            drain()
            normalise(t)
        jobs = wo_jobs(NP - 1, True)
        parts += [job() for job in jobs[2 * NC:] + jobs[:2 * NC]]
        return x + _ragged_result([sum(parts[m::NC], y_buf[m]) for m in range(NC)])

    def glu(x, cold):
        def arrive(name):
            if cold:
                copies[name].wait()

        arrive("wg")
        arrive("wu")
        _, tiles, rstd = _layernorm(x)
        xl = jnp.concatenate(tiles, axis=1)
        hid = []
        for b in range(NFB):
            g = _dot(xl, _packed(wg32[:, pl.ds(8 * b, 8), :])) * rstd
            u = _dot(xl, _packed(wu32[:, pl.ds(8 * b, 8), :])) * rstd
            h = jax.nn.sigmoid(g) * u
            hid += [_ragged_operands(_row(h, par)) for par in range(2)]
        out = [0.0] * NC
        for i, chunk in enumerate(hid):
            if i % NFB == 0:
                arrive(("wd", i // NFB))
            for m in range(NC):
                out[m] += _dot(chunk[RAGGED[m]], _packed(wd32[pl.ds(8 * i, 8), m]))
        return x + _ragged_result(out)

    copies["x"].wait()
    x_in = x_buf[...].astype(f32)
    x0 = _stack_rows([jnp.broadcast_to(x_in[:, c * 128:(c + 1) * 128], (8, 128))
                      for c in range(NC)])

    def layer(i, x):
        x = attention(x, i == 0, i >> 8)
        if ONLY:
            return x
        x = lax.cond(i == 0, lambda: glu(x, True), lambda: glu(x, False))
        return x

    x_out = lax.fori_loop(0, LAYERS, layer, x0)
    out_ref[...] = jnp.concatenate(
        [x_out[c:c + 1, :] for c in range(NC)], axis=1).astype(out_ref.dtype)


def _tile_order(w, *shape):
    r, c = w.shape
    w = w.reshape(r // 8, 8, c // 128, 128)
    return jnp.transpose(w, (0, 2, 1, 3)).reshape(*shape, 128)


@jax.jit
def pallas_interleave_layers__sliding_block_cached__glu_gated_glu__decode_kernel(
    A_x: jax.Array,
    A_k_cache: jax.Array,
    A_v_cache: jax.Array,
    A_wq: jax.Array,
    A_wo: jax.Array,
    B_x: jax.Array,
    B_w_gate: jax.Array,
    B_w_up: jax.Array,
    B_w_down: jax.Array,
):
    del B_x
    k, v = [_tile_order(jnp.swapaxes(a, 2, 3).reshape(H * DH, SK), NRT, SK // 256, 16)
            for a in (A_k_cache, A_v_cache)]
    out = pl.pallas_call(
        _kernel,
        out_shape=jax.ShapeDtypeStruct((1, D), A_x.dtype),
        in_specs=[pl.BlockSpec(memory_space=pltpu.HBM)] * 8,
        out_specs=pl.BlockSpec(memory_space=pltpu.VMEM),
        scratch_shapes=[
            pltpu.VMEM((1, D), bf16),
            pltpu.VMEM((P_ROW + 4, 16, 16, 128), bf16),
            pltpu.VMEM((Y_ROW + 1, 16, 16, 128), bf16),
            pltpu.VMEM((D // 8, F // 16, 128), bf16),
            pltpu.VMEM((D // 8, F // 16, 128), bf16),
            pltpu.VMEM((F // 16, NC, 16, 128), bf16),
            pltpu.VMEM((NJ, 16, 128), bf16),
            pltpu.VMEM((3, 8, 128), f32),
            pltpu.VMEM((2, 3, 16, 128), bf16),
            pltpu.VMEM((3, 3, 16, 128), bf16),
            pltpu.VMEM((4, 8, 128), f32),
            pltpu.VMEM((NC, 8, 128), f32),
            pltpu.SemaphoreType.DMA((14,)),
        ],
        compiler_params=pltpu.CompilerParams(vmem_limit_bytes=124 * 1024 * 1024),
    )(A_x.reshape(1, D), k, v,
      _tile_order(A_wq, D // 16, 2, NP, 24), _tile_order(A_wo, WO_ROWS, 16, 16),
      _tile_order(B_w_gate, D // 8, F // 16), _tile_order(B_w_up, D // 8, F // 16),
      _tile_order(B_w_down, F // 16, NC, 16))
    return out.reshape(A_x.shape)
```

```python
import jax
import jax.numpy as jnp
from jax import lax
import jax.experimental.pallas as pl
import jax.experimental.pallas.tpu as pltpu

D = 640
H = 32
DH = 192
F = 1536
SK = 32768
WIN = min(4096, max(256, SK // 4))
EPS = 1e-5
LAYERS = 2

NC = D // 128
NP = H // 2
RT = DH // 8
NRT = H * RT
NJ = WIN // 256
NF = F // 128
V_SPLIT = 12
WD_SPLIT = 9
MXU_RT = 16

WO_ROWS = H * DH * D // (256 * 128)
WQ2_ROW = NRT
WQ1_ROW = WQ2_ROW + D // 8
WO_ROW = WQ1_ROW + D // 16
VT_ROW = WO_ROW + WO_ROWS
A_ROW = VT_ROW + MXU_RT
P_ROW = A_ROW + 2
S_ROW = NRT - MXU_RT
Q_ROW = S_ROW + 2
O_ROW = Q_ROW + 1
T_ROW = O_ROW + 1
Y_ROW = T_ROW + 2

RS, JS = 3, 8
LEAD = 3
LAG = 4

f32, bf16, u32 = jnp.float32, jnp.bfloat16, jnp.uint32


def _iota(axis):
    return lax.broadcasted_iota(jnp.int32, (8, 128), axis)


def _operand(x):
    return jnp.concatenate([x, x], axis=0).astype(bf16)


def _dot(a, b, axis=0):
    return lax.dot_general(a, b, (((1,), (axis,)), ((), ())), preferred_element_type=f32)[0:8]


def _packed(words):
    if isinstance(words, list):
        return pltpu.bitcast(jnp.concatenate(words, axis=0), bf16)
    return pltpu.bitcast(words.reshape(words.shape[0] * 8, 128), bf16)


def _row(x, r):
    return jnp.broadcast_to(x[r:r + 1, :], (8, 128))


def _spread(x, half):
    lane = _iota(1)
    return jnp.take_along_axis(x, (lane // 16) * 8 + lane % 8 + 64 * half, axis=1)


def _own_tile():
    return (_iota(0) % 2) == ((_iota(1) // 8) % 2)


def _split_parity(x):
    return _operand(jnp.where(_own_tile(), x, 0.0))


def _reduce(fn, x):
    x = fn(x.reshape(-1, 8, 128), axis=0)
    return jnp.broadcast_to(fn(fn(x, axis=0, keepdims=True), axis=1, keepdims=True), (8, 128))


def _layernorm(x):
    mean = _reduce(jnp.sum, x) * (1.0 / D)
    xc = jnp.where(_iota(0) < NC, x - mean, 0.0)
    rstd = lax.rsqrt(_reduce(jnp.sum, xc * xc) * (1.0 / D) + EPS)
    halves = [_spread(x, half) - mean for half in range(2)]
    return xc, [_split_parity(_row(halves[u % 2], u // 2)) for u in range(2 * NC)], rstd


def _stack_rows(rows):
    out = jnp.zeros((8, 128), f32)
    for c, r in enumerate(rows):
        out = jnp.where(_iota(0) == c, r, out)
    return out


RAGGED = (0, 0, 1, 2, 2)


def _ragged_operands(x):
    lane = _iota(1)
    first = (lane // 16) * 16 + lane % 8
    return [_split_parity(jnp.take_along_axis(x, first, axis=1)), _split_parity(x),
            _split_parity(jnp.take_along_axis(x, first + 8, axis=1))]


def _ragged_result(parts):
    tiles = [_row(parts[i // 2], i % 2) for i in range(2 * NC)]
    return _stack_rows([tiles[c] + tiles[NC + c] for c in range(NC)])


def _kernel(x_hbm, k_hbm, v_hbm, wq_hbm, wo_hbm, wg_hbm, wu_hbm, wd_hbm, out_ref,
            x_buf, k_buf, v_buf, wg_buf, wu_buf, wd_buf,
            xl_buf, q_buf, ql_buf, ol_buf, inv_buf, y_buf, sems):
    k32, v32 = k_buf.bitcast(u32), v_buf.bitcast(u32)
    wg32, wu32, wd32 = wg_buf.bitcast(u32), wu_buf.bitcast(u32), wd_buf.bitcast(u32)

    copies = {}

    def copy(name, src, dst):
        copies[name] = pltpu.make_async_copy(src, dst, sems.at[len(copies)])

    win = pl.ds((SK - WIN) // 256, NJ)
    vs, ds = V_SPLIT * 2 * RT, WD_SPLIT * 8
    copy("x", x_hbm, x_buf)
    for i in range(2):
        copy(("wq", i), wq_hbm.at[:, i, :, pl.ds(0, 16), :],
             k_buf.at[pl.ds(WQ2_ROW + i * D // 16, D // 16)])
        copy(("wq", 2 + i), wq_hbm.at[:, i, :, pl.ds(16, 8), :],
             k_buf.at[pl.ds(WQ1_ROW, D // 16), :, pl.ds(8 * i, 8), :])
    copy("wo", wo_hbm, k_buf.at[pl.ds(WO_ROW, WO_ROWS)])
    copy("k", k_hbm.at[:, win], k_buf.at[pl.ds(0, NRT)])
    copy("v0", v_hbm.at[pl.ds(0, vs), win], v_buf.at[pl.ds(0, vs)])
    copy("v1", v_hbm.at[pl.ds(vs, S_ROW - vs), win], v_buf.at[pl.ds(vs, S_ROW - vs)])
    copy("v2", v_hbm.at[pl.ds(S_ROW, MXU_RT), win], k_buf.at[pl.ds(VT_ROW, MXU_RT)])
    copy("wg", wg_hbm, wg_buf)
    copy("wu", wu_hbm, wu_buf)
    copy(("wd", 0), wd_hbm.at[pl.ds(0, ds)], wd_buf.at[pl.ds(0, ds)])
    copy(("wd", WD_SPLIT), wd_hbm.at[pl.ds(ds, F // 16 - ds)], wd_buf.at[pl.ds(ds, F // 16 - ds)])
    for cp in copies.values():
        cp.start()

    def wait(cond, *names):
        @pl.when(cond)
        def _():
            for name in names:
                copies[name].wait()

    def put(ref, row, i, x):
        ref[row + i // 16, i % 16] = pltpu.bitcast(x, u32)

    def get(ref, row, i):
        return pltpu.bitcast(ref[row + i // 16, i % 16], f32)


    def q_jobs(n):
        def make(u):
            def job():
                if u < 2 * NC:
                    w = [k32[WQ2_ROW + (a % 2) * (D // 16) + a // 2, n]
                         for a in range(8 * u, 8 * u + 8)]
                else:
                    w = k32[pl.ds(WQ1_ROW + 8 * (u - 2 * NC), 8), n]
                r = _dot(xl_buf[u], _packed(w))
                return lambda: put(v32, Q_ROW, u, r)
            return job
        return [make(u) for u in range(3 * NC)]

    def q_sum(zero):
        parts = pltpu.bitcast(v32[zero + Q_ROW, pl.ds(0, 3 * NC)], f32)
        q_buf[0] = parts[:2 * NC].sum(axis=0) * q_buf[2]
        q_buf[1] = parts[2 * NC:].sum(axis=0) * q_buf[2]

    def q_lhs(e):
        for t in range(3):
            m = (3 * e + t) // 2
            q = _row(q_buf[0], m) if m < 2 else q_buf[1]
            ql_buf[e, t] = _split_parity(_spread(q, (3 * e + t) % 2))

    def qk_jobs(n, e):
        def make(j, t):
            def job():
                w = _packed(k32[pl.ds(n * 2 * RT + e * RT + 8 * t, 8), j])
                r = pltpu.bitcast(_dot(ql_buf[e, t], w), u32)

                def drain():
                    lo = 2 * (j % 4)
                    v32[S_ROW + e, 4 * t + j // 4, pl.ds(lo, 2), :] = r[lo:lo + 2, :]
                return drain
            return job
        return [make(j, t) for t in range(3) for j in range(NJ)]

    def softmax(e, zero):
        parts = pltpu.bitcast(v32[zero + S_ROW + e, pl.ds(0, 12)], f32)
        s = jnp.concatenate([parts[i] + parts[4 + i] + parts[8 + i] for i in range(4)],
                            axis=0) * (DH ** -0.5)
        p = jnp.exp(s - jnp.concatenate([_reduce(jnp.max, s)] * 4, axis=0))
        inv_buf[3 - e] = 1.0 / _reduce(jnp.sum, p)

        def publish():
            for i in range(4):
                put(v32, S_ROW + e, 12 + i, p[8 * i:8 * i + 8])
        return publish

    def expand(e, i, zero):
        for c in range(8):
            row = pltpu.bitcast(v32[zero + S_ROW + e, 12 + i, pl.ds(c, 1), :], f32)
            put(k32, P_ROW + 2 * e, 8 * i + c, jnp.broadcast_to(row, (8, 128)))

    def pv_steps(n, e, tiles=RT):
        acc = {}

        def make(r0, j0):
            def step():
                rows = range(e * RT + r0, e * RT + min(r0 + RS, tiles))
                for j in range(j0, j0 + JS):
                    p0, p1 = [get(k32, P_ROW + 2 * e, 2 * j + i) for i in range(2)]
                    for r in rows:
                        v = v_buf[n * 2 * RT + r, j].astype(f32)
                        t = v[0:8] * p0 + v[8:16] * p1
                        acc[r] = t if j == 0 else acc[r] + t
                if j0 + JS < NJ:
                    put(k32, A_ROW + 1, 10, acc[rows[-1]])
                else:
                    for r in rows:
                        k_buf[A_ROW + r // 32, (r // 2) % 16, pl.ds(8 * (r % 2), 8), :] = (
                            acc[r].astype(bf16))
            return step
        return [make(r0, j0) for r0 in range(0, tiles, RS) for j0 in range(0, NJ, JS)]

    def out_job(t, zero):
        def job():
            w = _packed(k32[zero + A_ROW + t // 2, pl.ds(8 * (t % 2), 8)])
            r = _dot(jnp.ones((16, 128), bf16), w, axis=1)
            return lambda: put(v32, O_ROW, t, r)
        return job

    def normalise(t):
        inv = (inv_buf[0] if t == 0 else inv_buf[1] if t == 2 else
               jnp.where(_iota(1) < DH - 128, inv_buf[0], inv_buf[1]))
        for i, tile in enumerate(_ragged_operands(get(v32, O_ROW, t) * inv)):
            ol_buf[t, i] = tile

    def tail_lhs():
        for j in range(NJ):
            p = get(v32, S_ROW + 1, 12 + j // 4)
            xl_buf[j] = _operand(jnp.where(_iota(0) // 2 == j % 4, p, 0.0))

    def tail_jobs(zero):
        def make(j, odd):
            def job():
                w = [k32[zero + VT_ROW + r, j] for r in range(odd, MXU_RT, 2)]
                r = _dot(xl_buf[j], _packed(w), axis=1)
                return lambda: put(v32, T_ROW + odd, j, r)
            return job
        return [make(j, odd) for j in range(NJ) for odd in range(2)]

    def tail_normalise():
        lane, halves = _iota(1), []
        for odd in range(2):
            a = pltpu.bitcast(v32[T_ROW + odd], f32).sum(axis=0)
            a = jnp.where(_own_tile(), a, 0.0).sum(axis=0, keepdims=True)
            a = jnp.broadcast_to(a, (8, 128))
            halves.append((a + jnp.take_along_axis(a, lane ^ 8, axis=1)) * inv_buf[1])
        ol_buf[2, 0] = _split_parity(halves[0])
        ol_buf[2, 1] = _split_parity(jnp.where((lane // 8) % 2 == 0, *halves))
        ol_buf[2, 2] = _split_parity(halves[1])

    def wo_jobs(n, keep=False):
        at = [(WO_ROW + (i >> 1), 8 * (i & 1)) for i in (3 * NC * n, 3 * NC * n + 1)]

        def make(t, m):
            def job():
                w = [k32[at[i // 8 % 2][0] + i // 16, at[i // 8 % 2][1] + i % 8]
                     for i in range(8 * NC * t + m, 8 * NC * (t + 1), NC)]
                r = _dot(ol_buf[t, RAGGED[m]], _packed(w))
                return r if keep else lambda: put(v32, Y_ROW, NC * t + m, r)
            return job
        return [make(t, m) for t in range(3) for m in range(NC)]

    def y_sum(m, zero):
        parts = [get(v32, zero + Y_ROW, NC * t + m) for t in range(3)]
        y_buf[m] += parts[0] + parts[1] + parts[2]

    def run(jobs):
        for drain in [job() for job in jobs]:
            drain()

    def pair(n, first=False, last=False):
        zero = n >> 8
        steps = pv_steps(n, 0) + pv_steps(n, 1, RT - MXU_RT if last else RT)
        hooks = [[] for _ in steps]

        def at(g, fn, *args):
            hooks[g].append(lambda: fn(*args))

        def softmax_between(g0, g1, e):
            publish = []
            at(g0, lambda: publish.append(softmax(e, zero)))
            at(g1, lambda: publish[0]())
            for i in range(4):
                at(g1 + 1 + 2 * i, expand, e, i, zero)

        def rotate():
            inv_buf[0] = inv_buf[3]
            inv_buf[1] = inv_buf[2]

        softmax_between(*((0, 1) if last else (1, 6)), 1)
        at(16, rotate)
        head, tail = [None] * 3, [None] * (3 * NC)
        if not first:
            head, tail = [out_job(t, zero) for t in range(3)], wo_jobs(n - 1)
            for t in range(3):
                at(8 + t, normalise, t)
            for m in range(NC):
                at(8 + m, y_sum, m, zero)
        if last:
            at(1, tail_lhs)
            groups = [head] + [[] for _ in steps[1:]]
            for i, job in enumerate(tail_jobs(zero)):
                groups[1 + LEAD + i // 2].append(job)
        else:
            softmax_between(17, 24, 0)
            at(26, q_sum, zero)
            at(29, q_lhs, 1)
            at(30, q_lhs, 0)
            jobs = (head + qk_jobs(n + 1, 0) + q_jobs(jnp.minimum(n + 2, NP - 1))
                    + qk_jobs(n + 1, 1) + tail)
            groups = [[job for job in jobs[4 * g + (g > 1):4 * g + 4 + (g >= 1)] if job]
                      for g in range(len(steps))]

        pending = {g: [job() for job in groups[g]] for g in range(LEAD)}
        for g, step in enumerate(steps):
            for drain in pending.pop(g - LAG, ()):
                drain()
            for hook in hooks[g]:
                hook()
            step()
            if g + LEAD < len(steps):
                pending[g + LEAD] = [job() for job in groups[g + LEAD]]
        for g in sorted(pending):
            for drain in pending[g]:
                drain()

    def attention(x, cold, zero):
        wait(cold, *[("wq", i) for i in range(4)], "wo", "k")
        xc, tiles, q_buf[2] = _layernorm(x)
        for u, tile in enumerate(tiles):
            xl_buf[u] = tile
        for c in range(NC):
            xl_buf[2 * NC + c] = _operand(_row(xc, c))
            y_buf[c] = jnp.zeros((8, 128), f32)
        for i in range(3 * NC):
            put(v32, Y_ROW, i, jnp.zeros((8, 128), f32))
        run(q_jobs(0))
        q_sum(0)
        q_lhs(0)
        q_lhs(1)
        run(q_jobs(1) + qk_jobs(0, 0))
        softmax(0, 0)()
        for i in range(4):
            expand(0, i, 0)
        run(qk_jobs(0, 1))
        q_sum(0)
        q_lhs(0)
        q_lhs(1)
        wait(cold, "v0")
        pair(zero, first=True)

        def body(n, carry):
            wait(jnp.logical_and(cold, n == V_SPLIT), "v1", "v2")
            pair(n)
            return carry

        lax.fori_loop(1, NP - 1, body, 0)
        pair(zero + (NP - 1), last=True)
        drains = [out_job(t, 0)() for t in range(2)]
        parts = [job() for job in wo_jobs(NP - 2, keep=True)]
        tail_normalise()
        for t, drain in enumerate(drains):
            drain()
            normalise(t)
        jobs = wo_jobs(NP - 1, keep=True)
        parts += [job() for job in jobs[2 * NC:] + jobs[:2 * NC]]
        return x + _ragged_result([sum(parts[m::NC], y_buf[m]) for m in range(NC)])

    def glu(x, cold):
        def arrive(name):
            if cold and name in copies:
                copies[name].wait()

        arrive("wg")
        arrive("wu")
        _, tiles, rstd = _layernorm(x)
        xl = jnp.concatenate(tiles, axis=1)
        hid = []
        for b in range(NF // 2):
            g = _dot(xl, _packed(wg32[:, pl.ds(8 * b, 8), :])) * rstd
            u = _dot(xl, _packed(wu32[:, pl.ds(8 * b, 8), :])) * rstd
            h = jax.nn.sigmoid(g) * u
            hid += [_ragged_operands(_row(h, par)) for par in range(2)]
        out = [0.0] * NC
        for i, chunk in enumerate(hid):
            arrive(("wd", i))
            for m in range(NC):
                out[m] += _dot(chunk[RAGGED[m]], _packed(wd32[pl.ds(8 * i, 8), m]))
        return x + _ragged_result(out)

    copies["x"].wait()
    x_in = x_buf[...].astype(f32)
    x0 = _stack_rows([jnp.broadcast_to(x_in[:, c * 128:(c + 1) * 128], (8, 128))
                      for c in range(NC)])

    def layer(i, x):
        x = attention(x, i == 0, i >> 8)
        x = lax.cond(i == 0, lambda: glu(x, True), lambda: glu(x, False))
        return x

    x_out = lax.fori_loop(0, LAYERS, layer, x0)
    out_ref[...] = jnp.concatenate(
        [x_out[c:c + 1, :] for c in range(NC)], axis=1).astype(out_ref.dtype)


def _tile_order(w, *shape):
    r, c = w.shape
    w = w.reshape(r // 8, 8, c // 128, 128)
    return jnp.transpose(w, (0, 2, 1, 3)).reshape(*shape, 128)


@jax.jit
def pallas_interleave_layers__sliding_block_cached__glu_gated_glu__decode_kernel(
    A_x: jax.Array,
    A_k_cache: jax.Array,
    A_v_cache: jax.Array,
    A_wq: jax.Array,
    A_wo: jax.Array,
    B_x: jax.Array,
    B_w_gate: jax.Array,
    B_w_up: jax.Array,
    B_w_down: jax.Array,
):
    del B_x
    k, v = [_tile_order(jnp.swapaxes(a, 2, 3).reshape(H * DH, SK), NRT, SK // 256, 16)
            for a in (A_k_cache, A_v_cache)]
    out = pl.pallas_call(
        _kernel,
        out_shape=jax.ShapeDtypeStruct((1, D), A_x.dtype),
        in_specs=[pl.BlockSpec(memory_space=pltpu.HBM)] * 8,
        out_specs=pl.BlockSpec(memory_space=pltpu.VMEM),
        scratch_shapes=[
            pltpu.VMEM((1, D), bf16),
            pltpu.VMEM((P_ROW + 4, 16, 16, 128), bf16),
            pltpu.VMEM((Y_ROW + 1, 16, 16, 128), bf16),
            pltpu.VMEM((D // 8, F // 16, 128), bf16),
            pltpu.VMEM((D // 8, F // 16, 128), bf16),
            pltpu.VMEM((F // 16, NC, 16, 128), bf16),
            pltpu.VMEM((NJ, 16, 128), bf16),
            pltpu.VMEM((3, 8, 128), f32),
            pltpu.VMEM((2, 3, 16, 128), bf16),
            pltpu.VMEM((3, 3, 16, 128), bf16),
            pltpu.VMEM((4, 8, 128), f32),
            pltpu.VMEM((NC, 8, 128), f32),
            pltpu.SemaphoreType.DMA((14,)),
        ],
        compiler_params=pltpu.CompilerParams(vmem_limit_bytes=124 * 1024 * 1024),
    )(A_x.reshape(1, D), k, v,
      _tile_order(A_wq, D // 16, 2, NP, 24), _tile_order(A_wo, WO_ROWS, 16, 16),
      _tile_order(B_w_gate, D // 8, F // 16), _tile_order(B_w_up, D // 8, F // 16),
      _tile_order(B_w_down, F // 16, NC, 16))
    return out.reshape(A_x.shape)
```

```python
import jax
import jax.numpy as jnp
from jax import lax
import jax.experimental.pallas as pl
import jax.experimental.pallas.tpu as pltpu

D = 640
H = 32
DH = 192
F = 1536
SK = 32768
WIN = min(4096, max(256, SK // 4))
EPS = 1e-5
LAYERS = 2

NC = D // 128
NP = H // 2
RT = DH // 8
NRT = H * RT
NJ = WIN // 256
NF = F // 128
V_SPLIT = 12
WD_SPLIT = 9
VPU_UP = 3
MXU_RT = 16

WO_ROWS = H * DH * D // (256 * 128)
WQ2_ROW = NRT
WQ1_ROW = WQ2_ROW + D // 8
WO_ROW = WQ1_ROW + D // 16
VT_ROW = WO_ROW + WO_ROWS
A_ROW = VT_ROW + MXU_RT
P_ROW = A_ROW + 2
S_ROW = NRT - MXU_RT
Q_ROW = S_ROW + 2
O_ROW = Q_ROW + 1
T_ROW = O_ROW + 1
Y_ROW = T_ROW + 2

RS, JS = 3, 8
LEAD = 3
LAG = 4

f32, bf16, u32 = jnp.float32, jnp.bfloat16, jnp.uint32


def _iota(axis):
    return lax.broadcasted_iota(jnp.int32, (8, 128), axis)


def _operand(x):
    return jnp.concatenate([x, x], axis=0).astype(bf16)


def _dot(a, b, axis=0):
    return lax.dot_general(a, b, (((1,), (axis,)), ((), ())), preferred_element_type=f32)[0:8]


def _packed(words):
    if isinstance(words, list):
        return pltpu.bitcast(jnp.concatenate(words, axis=0), bf16)
    return pltpu.bitcast(words.reshape(words.shape[0] * 8, 128), bf16)


def _row(x, r):
    return jnp.broadcast_to(x[r:r + 1, :], (8, 128))


def _spread(x, half):
    lane = _iota(1)
    return jnp.take_along_axis(x, (lane // 16) * 8 + lane % 8 + 64 * half, axis=1)


def _own_tile():
    return (_iota(0) % 2) == ((_iota(1) // 8) % 2)


def _split_parity(x):
    return _operand(jnp.where(_own_tile(), x, 0.0))


def _reduce(fn, x):
    x = fn(x.reshape(-1, 8, 128), axis=0)
    return jnp.broadcast_to(fn(fn(x, axis=0, keepdims=True), axis=1, keepdims=True), (8, 128))


def _layernorm(x):
    mean = _reduce(jnp.sum, x) * (1.0 / D)
    xc = jnp.where(_iota(0) < NC, x - mean, 0.0)
    rstd = lax.rsqrt(_reduce(jnp.sum, xc * xc) * (1.0 / D) + EPS)
    halves = [_spread(x, half) - mean for half in range(2)]
    return xc, [_split_parity(_row(halves[u % 2], u // 2)) for u in range(2 * NC)], rstd


def _columns(x):
    out = []
    for c in range(NC):
        xt = jnp.broadcast_to(x[c:c + 1, :], (128, 128)).T
        out += [xt[8 * i:8 * i + 8] for i in range(16)]
    return out


def _stack_rows(rows):
    out = jnp.zeros((8, 128), f32)
    for c, r in enumerate(rows):
        out = jnp.where(_iota(0) == c, r, out)
    return out


RAGGED = (0, 0, 1, 2, 2)


def _ragged_operands(x):
    lane = _iota(1)
    first = (lane // 16) * 16 + lane % 8
    return [_split_parity(jnp.take_along_axis(x, first, axis=1)), _split_parity(x),
            _split_parity(jnp.take_along_axis(x, first + 8, axis=1))]


def _ragged_result(parts):
    tiles = [_row(parts[i // 2], i % 2) for i in range(2 * NC)]
    return _stack_rows([tiles[c] + tiles[NC + c] for c in range(NC)])


def _kernel(x_hbm, k_hbm, v_hbm, wq_hbm, wo_hbm, wg_hbm, wu_hbm, wd_hbm, out_ref,
            x_buf, k_buf, v_buf, wg_buf, wu_buf, wd_buf,
            xl_buf, q_buf, ql_buf, ol_buf, inv_buf, y_buf, sems):
    k32, v32 = k_buf.bitcast(u32), v_buf.bitcast(u32)
    wg32, wu32, wd32 = wg_buf.bitcast(u32), wu_buf.bitcast(u32), wd_buf.bitcast(u32)

    copies = {}

    def copy(name, src, dst):
        copies[name] = pltpu.make_async_copy(src, dst, sems.at[len(copies)])

    win = pl.ds((SK - WIN) // 256, NJ)
    vs, ds = V_SPLIT * 2 * RT, WD_SPLIT * 8
    copy("x", x_hbm, x_buf)
    for i in range(2):
        copy(("wq", i), wq_hbm.at[:, i, :, pl.ds(0, 16), :],
             k_buf.at[pl.ds(WQ2_ROW + i * D // 16, D // 16)])
        copy(("wq", 2 + i), wq_hbm.at[:, i, :, pl.ds(16, 8), :],
             k_buf.at[pl.ds(WQ1_ROW, D // 16), :, pl.ds(8 * i, 8), :])
    copy("wo", wo_hbm, k_buf.at[pl.ds(WO_ROW, WO_ROWS)])
    copy("k", k_hbm.at[:, win], k_buf.at[pl.ds(0, NRT)])
    copy("v0", v_hbm.at[pl.ds(0, vs), win], v_buf.at[pl.ds(0, vs)])
    copy("v1", v_hbm.at[pl.ds(vs, S_ROW - vs), win], v_buf.at[pl.ds(vs, S_ROW - vs)])
    copy("v2", v_hbm.at[pl.ds(S_ROW, MXU_RT), win], k_buf.at[pl.ds(VT_ROW, MXU_RT)])
    copy("wg", wg_hbm, wg_buf)
    copy("wu", wu_hbm, wu_buf)
    copy(("wd", 0), wd_hbm.at[pl.ds(0, ds)], wd_buf.at[pl.ds(0, ds)])
    copy(("wd", WD_SPLIT), wd_hbm.at[pl.ds(ds, F // 16 - ds)], wd_buf.at[pl.ds(ds, F // 16 - ds)])
    for cp in copies.values():
        cp.start()

    def wait(cond, *names):
        @pl.when(cond)
        def _():
            for name in names:
                copies[name].wait()

    def put(ref, row, i, x):
        ref[row + i // 16, i % 16] = pltpu.bitcast(x, u32)

    def get(ref, row, i):
        return pltpu.bitcast(ref[row + i // 16, i % 16], f32)


    def q_jobs(n):
        def make(u):
            def job():
                if u < 2 * NC:
                    w = [k32[WQ2_ROW + (a % 2) * (D // 16) + a // 2, n]
                         for a in range(8 * u, 8 * u + 8)]
                else:
                    w = k32[pl.ds(WQ1_ROW + 8 * (u - 2 * NC), 8), n]
                r = _dot(xl_buf[u], _packed(w))
                return lambda: put(v32, Q_ROW, u, r)
            return job
        return [make(u) for u in range(3 * NC)]

    def q_sum(zero):
        parts = pltpu.bitcast(v32[zero + Q_ROW, pl.ds(0, 3 * NC)], f32)
        q_buf[0] = parts[:2 * NC].sum(axis=0) * q_buf[2]
        q_buf[1] = parts[2 * NC:].sum(axis=0) * q_buf[2]

    def q_lhs(e):
        for t in range(3):
            m = (3 * e + t) // 2
            q = _row(q_buf[0], m) if m < 2 else q_buf[1]
            ql_buf[e, t] = _split_parity(_spread(q, (3 * e + t) % 2))

    def qk_jobs(n, e):
        def make(j, t):
            def job():
                w = _packed(k32[pl.ds(n * 2 * RT + e * RT + 8 * t, 8), j])
                r = pltpu.bitcast(_dot(ql_buf[e, t], w), u32)

                def drain():
                    lo = 2 * (j % 4)
                    v32[S_ROW + e, 4 * t + j // 4, pl.ds(lo, 2), :] = r[lo:lo + 2, :]
                return drain
            return job
        return [make(j, t) for t in range(3) for j in range(NJ)]

    def softmax(e, zero):
        parts = pltpu.bitcast(v32[zero + S_ROW + e, pl.ds(0, 12)], f32)
        s = jnp.concatenate([parts[i] + parts[4 + i] + parts[8 + i] for i in range(4)],
                            axis=0) * (DH ** -0.5)
        p = jnp.exp(s - jnp.concatenate([_reduce(jnp.max, s)] * 4, axis=0))
        inv_buf[3 - e] = 1.0 / _reduce(jnp.sum, p)

        def publish():
            for i in range(4):
                put(v32, S_ROW + e, 12 + i, p[8 * i:8 * i + 8])
        return publish

    def expand(e, i, zero):
        for c in range(8):
            row = pltpu.bitcast(v32[zero + S_ROW + e, 12 + i, pl.ds(c, 1), :], f32)
            put(k32, P_ROW + 2 * e, 8 * i + c, jnp.broadcast_to(row, (8, 128)))

    def pv_steps(n, e, tiles=RT):
        acc = {}

        def make(r0, j0):
            def step():
                rows = range(e * RT + r0, e * RT + min(r0 + RS, tiles))
                for j in range(j0, j0 + JS):
                    p0, p1 = [get(k32, P_ROW + 2 * e, 2 * j + i) for i in range(2)]
                    for r in rows:
                        v = v_buf[n * 2 * RT + r, j].astype(f32)
                        t = v[0:8] * p0 + v[8:16] * p1
                        acc[r] = t if j == 0 else acc[r] + t
                if j0 + JS < NJ:
                    put(k32, A_ROW + 1, 10, acc[rows[-1]])
                else:
                    for r in rows:
                        k_buf[A_ROW + r // 32, (r // 2) % 16, pl.ds(8 * (r % 2), 8), :] = (
                            acc[r].astype(bf16))
            return step
        return [make(r0, j0) for r0 in range(0, tiles, RS) for j0 in range(0, NJ, JS)]

    def out_job(t, zero):
        def job():
            w = _packed(k32[zero + A_ROW + t // 2, pl.ds(8 * (t % 2), 8)])
            r = _dot(jnp.ones((16, 128), bf16), w, axis=1)
            return lambda: put(v32, O_ROW, t, r)
        return job

    def normalise(t):
        inv = (inv_buf[0] if t == 0 else inv_buf[1] if t == 2 else
               jnp.where(_iota(1) < DH - 128, inv_buf[0], inv_buf[1]))
        for i, tile in enumerate(_ragged_operands(get(v32, O_ROW, t) * inv)):
            ol_buf[t, i] = tile

    def tail_lhs():
        for j in range(NJ):
            p = get(v32, S_ROW + 1, 12 + j // 4)
            xl_buf[j] = _operand(jnp.where(_iota(0) // 2 == j % 4, p, 0.0))

    def tail_jobs(zero):
        def make(j, odd):
            def job():
                w = [k32[zero + VT_ROW + r, j] for r in range(odd, MXU_RT, 2)]
                r = _dot(xl_buf[j], _packed(w), axis=1)
                return lambda: put(v32, T_ROW + odd, j, r)
            return job
        return [make(j, odd) for j in range(NJ) for odd in range(2)]

    def tail_normalise():
        lane, halves = _iota(1), []
        for odd in range(2):
            a = pltpu.bitcast(v32[T_ROW + odd], f32).sum(axis=0)
            a = jnp.where(_own_tile(), a, 0.0).sum(axis=0, keepdims=True)
            a = jnp.broadcast_to(a, (8, 128))
            halves.append((a + jnp.take_along_axis(a, lane ^ 8, axis=1)) * inv_buf[1])
        ol_buf[2, 0] = _split_parity(halves[0])
        ol_buf[2, 1] = _split_parity(jnp.where((lane // 8) % 2 == 0, *halves))
        ol_buf[2, 2] = _split_parity(halves[1])

    def wo_jobs(n, keep=False):
        at = [(WO_ROW + (i >> 1), 8 * (i & 1)) for i in (3 * NC * n, 3 * NC * n + 1)]

        def make(t, m):
            def job():
                w = [k32[at[i // 8 % 2][0] + i // 16, at[i // 8 % 2][1] + i % 8]
                     for i in range(8 * NC * t + m, 8 * NC * (t + 1), NC)]
                r = _dot(ol_buf[t, RAGGED[m]], _packed(w))
                return r if keep else lambda: put(v32, Y_ROW, NC * t + m, r)
            return job
        return [make(t, m) for t in range(3) for m in range(NC)]

    def y_sum(m, zero):
        parts = [get(v32, zero + Y_ROW, NC * t + m) for t in range(3)]
        y_buf[m] += parts[0] + parts[1] + parts[2]

    def run(jobs):
        for drain in [job() for job in jobs]:
            drain()

    def pair(n, first=False, last=False):
        zero = n >> 8
        steps = pv_steps(n, 0) + pv_steps(n, 1, RT - MXU_RT if last else RT)
        hooks = [[] for _ in steps]

        def at(g, fn, *args):
            hooks[g].append(lambda: fn(*args))

        def softmax_between(g0, g1, e):
            publish = []
            at(g0, lambda: publish.append(softmax(e, zero)))
            at(g1, lambda: publish[0]())
            for i in range(4):
                at(g1 + 1 + 2 * i, expand, e, i, zero)

        def rotate():
            inv_buf[0] = inv_buf[3]
            inv_buf[1] = inv_buf[2]

        softmax_between(*((0, 1) if last else (1, 6)), 1)
        at(16, rotate)
        head, tail = [None] * 3, [None] * (3 * NC)
        if not first:
            head, tail = [out_job(t, zero) for t in range(3)], wo_jobs(n - 1)
            for t in range(3):
                at(8 + t, normalise, t)
            for m in range(NC):
                at(8 + m, y_sum, m, zero)
        if last:
            at(1, tail_lhs)
            groups = [head] + [[] for _ in steps[1:]]
            for i, job in enumerate(tail_jobs(zero)):
                groups[1 + LEAD + i // 2].append(job)
        else:
            softmax_between(17, 24, 0)
            at(26, q_sum, zero)
            at(29, q_lhs, 1)
            at(30, q_lhs, 0)
            jobs = (head + qk_jobs(n + 1, 0) + q_jobs(jnp.minimum(n + 2, NP - 1))
                    + qk_jobs(n + 1, 1) + tail)
            groups = [[job for job in jobs[4 * g + (g > 1):4 * g + 4 + (g >= 1)] if job]
                      for g in range(len(steps))]

        pending = {g: [job() for job in groups[g]] for g in range(LEAD)}
        for g, step in enumerate(steps):
            for drain in pending.pop(g - LAG, ()):
                drain()
            for hook in hooks[g]:
                hook()
            step()
            if g + LEAD < len(steps):
                pending[g + LEAD] = [job() for job in groups[g + LEAD]]
        for g in sorted(pending):
            for drain in pending[g]:
                drain()

    def attention(x, cold, zero):
        wait(cold, *[("wq", i) for i in range(4)], "wo", "k")
        xc, tiles, q_buf[2] = _layernorm(x)
        for u, tile in enumerate(tiles):
            xl_buf[u] = tile
        for c in range(NC):
            xl_buf[2 * NC + c] = _operand(_row(xc, c))
            y_buf[c] = jnp.zeros((8, 128), f32)
        for i in range(3 * NC):
            put(v32, Y_ROW, i, jnp.zeros((8, 128), f32))
        run(q_jobs(0))
        q_sum(0)
        q_lhs(0)
        q_lhs(1)
        run(q_jobs(1) + qk_jobs(0, 0))
        softmax(0, 0)()
        for i in range(4):
            expand(0, i, 0)
        run(qk_jobs(0, 1))
        q_sum(0)
        q_lhs(0)
        q_lhs(1)
        wait(cold, "v0")
        pair(zero, first=True)

        def body(n, carry):
            wait(jnp.logical_and(cold, n == V_SPLIT), "v1", "v2")
            pair(n)
            return carry

        lax.fori_loop(1, NP - 1, body, 0)
        pair(zero + (NP - 1), last=True)
        drains = [out_job(t, 0)() for t in range(2)]
        parts = [job() for job in wo_jobs(NP - 2, keep=True)]
        tail_normalise()
        for t, drain in enumerate(drains):
            drain()
            normalise(t)
        jobs = wo_jobs(NP - 1, keep=True)
        parts += [job() for job in jobs[2 * NC:] + jobs[:2 * NC]]
        return x + _ragged_result([sum(parts[m::NC], y_buf[m]) for m in range(NC)])

    def glu(x, cold):
        def arrive(name):
            if cold and name in copies:
                copies[name].wait()

        arrive("wg")
        arrive("wu")
        xc, tiles, rstd = _layernorm(x)
        xl = jnp.concatenate(tiles, axis=1)
        up = {}
        for a, xa in enumerate(_columns(xc)):
            for b in range(NF // 2 - VPU_UP, NF // 2):
                w = wu_buf[a, pl.ds(16 * b, 16), :].astype(f32)
                for par in range(2):
                    t = w[8 * par:8 * par + 8] * xa
                    up[b, par] = up[b, par] + t if a else t
        hid = []
        for b in range(NF // 2):
            g = _dot(xl, _packed(wg32[:, pl.ds(8 * b, 8), :])) * rstd
            if (b, 0) in up:
                u = _stack_rows([jnp.sum(up[b, par], axis=0, keepdims=True) for par in range(2)])
            else:
                u = _dot(xl, _packed(wu32[:, pl.ds(8 * b, 8), :]))
            h = jax.nn.sigmoid(g) * (u * rstd)
            hid += [_ragged_operands(_row(h, par)) for par in range(2)]
        out = [0.0] * NC
        for i, chunk in enumerate(hid):
            arrive(("wd", i))
            for m in range(NC):
                out[m] += _dot(chunk[RAGGED[m]], _packed(wd32[pl.ds(8 * i, 8), m]))
        return x + _ragged_result(out)

    copies["x"].wait()
    x_in = x_buf[...].astype(f32)
    x0 = _stack_rows([jnp.broadcast_to(x_in[:, c * 128:(c + 1) * 128], (8, 128))
                      for c in range(NC)])

    def layer(i, x):
        x = attention(x, i == 0, i >> 8)
        x = lax.cond(i == 0, lambda: glu(x, True), lambda: glu(x, False))
        return x

    x_out = lax.fori_loop(0, LAYERS, layer, x0)
    out_ref[...] = jnp.concatenate(
        [x_out[c:c + 1, :] for c in range(NC)], axis=1).astype(out_ref.dtype)


def _tile_order(w, *shape):
    r, c = w.shape
    w = w.reshape(r // 8, 8, c // 128, 128)
    return jnp.transpose(w, (0, 2, 1, 3)).reshape(*shape, 128)


@jax.jit
def pallas_interleave_layers__sliding_block_cached__glu_gated_glu__decode_kernel(
    A_x: jax.Array,
    A_k_cache: jax.Array,
    A_v_cache: jax.Array,
    A_wq: jax.Array,
    A_wo: jax.Array,
    B_x: jax.Array,
    B_w_gate: jax.Array,
    B_w_up: jax.Array,
    B_w_down: jax.Array,
):
    del B_x
    k, v = [_tile_order(jnp.swapaxes(a, 2, 3).reshape(H * DH, SK), NRT, SK // 256, 16)
            for a in (A_k_cache, A_v_cache)]
    out = pl.pallas_call(
        _kernel,
        out_shape=jax.ShapeDtypeStruct((1, D), A_x.dtype),
        in_specs=[pl.BlockSpec(memory_space=pltpu.HBM)] * 8,
        out_specs=pl.BlockSpec(memory_space=pltpu.VMEM),
        scratch_shapes=[
            pltpu.VMEM((1, D), bf16),
            pltpu.VMEM((P_ROW + 4, 16, 16, 128), bf16),
            pltpu.VMEM((Y_ROW + 1, 16, 16, 128), bf16),
            pltpu.VMEM((D // 8, F // 16, 128), bf16),
            pltpu.VMEM((D // 8, F // 16, 128), bf16),
            pltpu.VMEM((F // 16, NC, 16, 128), bf16),
            pltpu.VMEM((NJ, 16, 128), bf16),
            pltpu.VMEM((3, 8, 128), f32),
            pltpu.VMEM((2, 3, 16, 128), bf16),
            pltpu.VMEM((3, 3, 16, 128), bf16),
            pltpu.VMEM((4, 8, 128), f32),
            pltpu.VMEM((NC, 8, 128), f32),
            pltpu.SemaphoreType.DMA((14,)),
        ],
        compiler_params=pltpu.CompilerParams(vmem_limit_bytes=124 * 1024 * 1024),
    )(A_x.reshape(1, D), k, v,
      _tile_order(A_wq, D // 16, 2, NP, 24), _tile_order(A_wo, WO_ROWS, 16, 16),
      _tile_order(B_w_gate, D // 8, F // 16), _tile_order(B_w_up, D // 8, F // 16),
      _tile_order(B_w_down, F // 16, NC, 16))
    return out.reshape(A_x.shape)
```

```python
import jax
import jax.numpy as jnp
from jax import lax
import jax.experimental.pallas as pl
import jax.experimental.pallas.tpu as pltpu

D = 640
H = 32
DH = 192
F = 1536
SK = 32768
WIN = min(4096, max(256, SK // 4))
EPS = 1e-5
LAYERS = 2

NC = D // 128
NP = H // 2
RT = DH // 8
NRT = H * RT
NJ = WIN // 256
NF = F // 128
V_SPLIT = 12
WD_SPLIT = 9
VPU_UP = 3
MXU_RT = 16

WO_ROWS = H * DH * D // (256 * 128)
WQ2_ROW = NRT
WQ1_ROW = WQ2_ROW + D // 8
WO_ROW = WQ1_ROW + D // 16
VT_ROW = WO_ROW + WO_ROWS
A_ROW = VT_ROW + MXU_RT
P_ROW = A_ROW + 4
S_ROW = NRT - MXU_RT
Q_ROW = S_ROW + 2
O_ROW = Q_ROW + 1
T_ROW = O_ROW + 1
Y_ROW = T_ROW + 2

RS, JS = 3, 8
LEAD = 3
LAG = 4

f32, bf16, u32 = jnp.float32, jnp.bfloat16, jnp.uint32


def _iota(axis):
    return lax.broadcasted_iota(jnp.int32, (8, 128), axis)


def _dot(a, b, axis=0):
    return lax.dot_general(a, b, (((1,), (axis,)), ((), ())), preferred_element_type=f32)


def _packed(words):
    if isinstance(words, list):
        return pltpu.bitcast(jnp.concatenate(words, axis=0), bf16)
    return pltpu.bitcast(words.reshape(words.shape[0] * 8, 128), bf16)


def _row(x, r):
    return jnp.broadcast_to(x[r:r + 1, :], (8, 128))


def _spread(x, half):
    lane = _iota(1)
    return jnp.take_along_axis(x, (lane // 16) * 8 + lane % 8 + 64 * half, axis=1)


def _own_tile():
    return (_iota(0) % 2) == ((_iota(1) // 8) % 2)


def _split_parity(x):
    return jnp.where(_own_tile(), x, 0.0)


def _reduce(fn, x):
    x = fn(x.reshape(-1, 8, 128), axis=0)
    return jnp.broadcast_to(fn(fn(x, axis=0, keepdims=True), axis=1, keepdims=True), (8, 128))


def _layernorm(x):
    mean = _reduce(jnp.sum, x) * (1.0 / D)
    xc = jnp.where(_iota(0) < NC, x - mean, 0.0)
    rstd = lax.rsqrt(_reduce(jnp.sum, xc * xc) * (1.0 / D) + EPS)
    halves = [_spread(x, half) - mean for half in range(2)]
    return xc, [_split_parity(_row(halves[u % 2], u // 2)) for u in range(2 * NC)], rstd


def _columns(x):
    out = []
    for c in range(NC):
        xt = jnp.broadcast_to(x[c:c + 1, :], (128, 128)).T
        out += [xt[8 * i:8 * i + 8] for i in range(16)]
    return out


def _stack_rows(rows):
    out = jnp.zeros((8, 128), f32)
    for c, r in enumerate(rows):
        out = jnp.where(_iota(0) == c, r, out)
    return out


RAGGED = (0, 0, 1, 2, 2)


def _ragged_operands(x):
    lane = _iota(1)
    first = (lane // 16) * 16 + lane % 8
    return [_split_parity(jnp.take_along_axis(x, first, axis=1)), _split_parity(x),
            _split_parity(jnp.take_along_axis(x, first + 8, axis=1))]


def _ragged_result(parts):
    tiles = [_row(parts[i // 2], i % 2) for i in range(2 * NC)]
    return _stack_rows([tiles[c] + tiles[NC + c] for c in range(NC)])


def _kernel(x_hbm, k_hbm, v_hbm, wq_hbm, wo_hbm, wg_hbm, wu_hbm, wd_hbm, out_ref,
            x_buf, k_buf, v_buf, wg_buf, wu_buf, wd_buf,
            xl_buf, q_buf, ql_buf, ol_buf, inv_buf, y_buf, sems):
    k32, v32 = k_buf.bitcast(u32), v_buf.bitcast(u32)
    wg32, wu32, wd32 = wg_buf.bitcast(u32), wu_buf.bitcast(u32), wd_buf.bitcast(u32)

    copies = {}

    def copy(name, src, dst):
        copies[name] = pltpu.make_async_copy(src, dst, sems.at[len(copies)])

    win = pl.ds((SK - WIN) // 256, NJ)
    vs, ds = V_SPLIT * 2 * RT, WD_SPLIT * 8
    copy("x", x_hbm, x_buf)
    for i in range(2):
        copy(("wq", i), wq_hbm.at[:, i, :, pl.ds(0, 16), :],
             k_buf.at[pl.ds(WQ2_ROW + i * D // 16, D // 16)])
        copy(("wq", 2 + i), wq_hbm.at[:, i, :, pl.ds(16, 8), :],
             k_buf.at[pl.ds(WQ1_ROW, D // 16), :, pl.ds(8 * i, 8), :])
    copy("wo", wo_hbm, k_buf.at[pl.ds(WO_ROW, WO_ROWS)])
    copy("k", k_hbm.at[:, win], k_buf.at[pl.ds(0, NRT)])
    copy("v0", v_hbm.at[pl.ds(0, vs), win], v_buf.at[pl.ds(0, vs)])
    copy("v1", v_hbm.at[pl.ds(vs, S_ROW - vs), win], v_buf.at[pl.ds(vs, S_ROW - vs)])
    copy("v2", v_hbm.at[pl.ds(S_ROW, MXU_RT), win], k_buf.at[pl.ds(VT_ROW, MXU_RT)])
    copy("wg", wg_hbm, wg_buf)
    copy("wu", wu_hbm, wu_buf)
    copy(("wd", 0), wd_hbm.at[pl.ds(0, ds)], wd_buf.at[pl.ds(0, ds)])
    copy(("wd", WD_SPLIT), wd_hbm.at[pl.ds(ds, F // 16 - ds)], wd_buf.at[pl.ds(ds, F // 16 - ds)])
    for cp in copies.values():
        cp.start()

    def wait(cond, *names):
        @pl.when(cond)
        def _():
            for name in names:
                copies[name].wait()

    def put(ref, row, i, x):
        ref[row + i // 16, i % 16] = pltpu.bitcast(x, u32)

    def get(ref, row, i):
        return pltpu.bitcast(ref[row + i // 16, i % 16], f32)


    def q_jobs(n):
        def make(u):
            def job():
                if u < 2 * NC:
                    w = [k32[WQ2_ROW + (a % 2) * (D // 16) + a // 2, n]
                         for a in range(8 * u, 8 * u + 8)]
                else:
                    w = k32[pl.ds(WQ1_ROW + 8 * (u - 2 * NC), 8), n]
                r = _dot(xl_buf[u], _packed(w))
                return lambda: put(v32, Q_ROW, u, r)
            return job
        return [make(u) for u in range(3 * NC)]

    def q_sum(zero):
        parts = pltpu.bitcast(v32[zero + Q_ROW, pl.ds(0, 3 * NC)], f32)
        q_buf[0] = parts[:2 * NC].sum(axis=0) * q_buf[2]
        q_buf[1] = parts[2 * NC:].sum(axis=0) * q_buf[2]

    def q_lhs(e):
        for t in range(3):
            m = (3 * e + t) // 2
            q = _row(q_buf[0], m) if m < 2 else q_buf[1]
            ql_buf[e, t] = _split_parity(_spread(q, (3 * e + t) % 2))

    def qk_jobs(n, e):
        def make(j, t):
            def job():
                w = _packed(k32[pl.ds(n * 2 * RT + e * RT + 8 * t, 8), j])
                r = pltpu.bitcast(_dot(ql_buf[e, t], w), u32)

                def drain():
                    lo = 2 * (j % 4)
                    v32[S_ROW + e, 4 * t + j // 4, pl.ds(lo, 2), :] = r[lo:lo + 2, :]
                return drain
            return job
        return [make(j, t) for t in range(3) for j in range(NJ)]

    def softmax(e, zero):
        parts = pltpu.bitcast(v32[zero + S_ROW + e, pl.ds(0, 12)], f32)
        s = jnp.concatenate([parts[i] + parts[4 + i] + parts[8 + i] for i in range(4)],
                            axis=0) * (DH ** -0.5)
        p = jnp.exp(s - jnp.concatenate([_reduce(jnp.max, s)] * 4, axis=0))
        inv_buf[3 - e] = 1.0 / _reduce(jnp.sum, p)

        def publish():
            for i in range(4):
                put(v32, S_ROW + e, 12 + i, p[8 * i:8 * i + 8])
        return publish

    def expand(e, i, zero):
        for c in range(8):
            row = pltpu.bitcast(v32[zero + S_ROW + e, 12 + i, pl.ds(c, 1), :], f32)
            put(k32, P_ROW + 2 * e, 8 * i + c, jnp.broadcast_to(row, (8, 128)))

    def pv_steps(n, e, tiles=RT):
        acc = {}

        def make(r0, j0):
            def step():
                rows = range(e * RT + r0, e * RT + min(r0 + RS, tiles))
                for j in range(j0, j0 + JS):
                    p0, p1 = [get(k32, P_ROW + 2 * e, 2 * j + i) for i in range(2)]
                    for r in rows:
                        v = v_buf[n * 2 * RT + r, j].astype(f32)
                        t = v[0:8] * p0 + v[8:16] * p1
                        acc[r] = t if j == 0 else acc[r] + t
                if j0 + JS < NJ:
                    put(k32, A_ROW + 3, 10, acc[rows[-1]])
                else:
                    for r in rows:
                        put(k32, A_ROW, r, acc[r])
            return step
        return [make(r0, j0) for r0 in range(0, tiles, RS) for j0 in range(0, NJ, JS)]

    def out_job(t, zero):
        def job():
            w = pltpu.bitcast(k32[zero + A_ROW + t].reshape(128, 128), f32)
            r = _dot(jnp.ones((8, 128), f32), w, axis=1)
            return lambda: put(v32, O_ROW, t, r)
        return job

    def normalise(t):
        inv = (inv_buf[0] if t == 0 else inv_buf[1] if t == 2 else
               jnp.where(_iota(1) < DH - 128, inv_buf[0], inv_buf[1]))
        for i, tile in enumerate(_ragged_operands(get(v32, O_ROW, t) * inv)):
            ol_buf[t, i] = tile

    def tail_lhs():
        for j in range(NJ):
            p = get(v32, S_ROW + 1, 12 + j // 4)
            xl_buf[j] = jnp.where(_iota(0) // 2 == j % 4, p, 0.0)

    def tail_jobs(zero):
        def make(j, odd):
            def job():
                w = [k32[zero + VT_ROW + r, j] for r in range(odd, MXU_RT, 2)]
                r = _dot(xl_buf[j], _packed(w), axis=1)
                return lambda: put(v32, T_ROW + odd, j, r)
            return job
        return [make(j, odd) for j in range(NJ) for odd in range(2)]

    def tail_normalise():
        lane, halves = _iota(1), []
        for odd in range(2):
            a = pltpu.bitcast(v32[T_ROW + odd], f32).sum(axis=0)
            a = jnp.where(_own_tile(), a, 0.0).sum(axis=0, keepdims=True)
            a = jnp.broadcast_to(a, (8, 128))
            halves.append((a + jnp.take_along_axis(a, lane ^ 8, axis=1)) * inv_buf[1])
        ol_buf[2, 0] = _split_parity(halves[0])
        ol_buf[2, 1] = _split_parity(jnp.where((lane // 8) % 2 == 0, *halves))
        ol_buf[2, 2] = _split_parity(halves[1])

    def wo_jobs(n, keep=False):
        at = [(WO_ROW + (i >> 1), 8 * (i & 1)) for i in (3 * NC * n, 3 * NC * n + 1)]

        def make(t, m):
            def job():
                w = [k32[at[i // 8 % 2][0] + i // 16, at[i // 8 % 2][1] + i % 8]
                     for i in range(8 * NC * t + m, 8 * NC * (t + 1), NC)]
                r = _dot(ol_buf[t, RAGGED[m]], _packed(w))
                return r if keep else lambda: put(v32, Y_ROW, NC * t + m, r)
            return job
        return [make(t, m) for t in range(3) for m in range(NC)]

    def y_sum(m, zero):
        parts = [get(v32, zero + Y_ROW, NC * t + m) for t in range(3)]
        y_buf[m] += parts[0] + parts[1] + parts[2]

    def run(jobs):
        for drain in [job() for job in jobs]:
            drain()

    def pair(n, first=False, last=False):
        zero = n >> 8
        steps = pv_steps(n, 0) + pv_steps(n, 1, RT - MXU_RT if last else RT)
        hooks = [[] for _ in steps]

        def at(g, fn, *args):
            hooks[g].append(lambda: fn(*args))

        def softmax_between(g0, g1, e):
            publish = []
            at(g0, lambda: publish.append(softmax(e, zero)))
            at(g1, lambda: publish[0]())
            for i in range(4):
                at(g1 + 1 + 2 * i, expand, e, i, zero)

        def rotate():
            inv_buf[0] = inv_buf[3]
            inv_buf[1] = inv_buf[2]

        softmax_between(*((0, 1) if last else (1, 6)), 1)
        at(16, rotate)
        head, tail = [None] * 3, [None] * (3 * NC)
        if not first:
            head, tail = [out_job(t, zero) for t in range(3)], wo_jobs(n - 1)
            for t in range(3):
                at(8 + t, normalise, t)
            for m in range(NC):
                at(11 + m, y_sum, m, zero)
        if last:
            at(1, tail_lhs)
            groups = [head] + [[] for _ in steps[1:]]
            for i, job in enumerate(tail_jobs(zero)):
                groups[1 + LEAD + i // 2].append(job)
        else:
            softmax_between(17, 24, 0)
            at(26, q_sum, zero)
            at(29, q_lhs, 1)
            at(30, q_lhs, 0)
            jobs = (head + qk_jobs(n + 1, 0) + q_jobs(jnp.minimum(n + 2, NP - 1))
                    + qk_jobs(n + 1, 1) + tail)
            groups = [[job for job in jobs[4 * g + (g > 1):4 * g + 4 + (g >= 1)] if job]
                      for g in range(len(steps))]

        pending = {g: [job() for job in groups[g]] for g in range(LEAD)}
        for g, step in enumerate(steps):
            for drain in pending.pop(g - LAG, ()):
                drain()
            for hook in hooks[g]:
                hook()
            step()
            if g + LEAD < len(steps):
                pending[g + LEAD] = [job() for job in groups[g + LEAD]]
        for g in sorted(pending):
            for drain in pending[g]:
                drain()

    def attention(x, cold, zero):
        wait(cold, *[("wq", i) for i in range(4)], "wo", "k")
        xc, tiles, q_buf[2] = _layernorm(x)
        for u, tile in enumerate(tiles):
            xl_buf[u] = tile
        for c in range(NC):
            xl_buf[2 * NC + c] = _row(xc, c)
            y_buf[c] = jnp.zeros((8, 128), f32)
        for i in range(3 * NC):
            put(v32, Y_ROW, i, jnp.zeros((8, 128), f32))
        run(q_jobs(0))
        q_sum(0)
        q_lhs(0)
        q_lhs(1)
        run(q_jobs(1) + qk_jobs(0, 0))
        softmax(0, 0)()
        for i in range(4):
            expand(0, i, 0)
        run(qk_jobs(0, 1))
        q_sum(0)
        q_lhs(0)
        q_lhs(1)
        wait(cold, "v0")
        pair(zero, first=True)

        def body(n, carry):
            wait(jnp.logical_and(cold, n == V_SPLIT), "v1", "v2")
            pair(n)
            return carry

        lax.fori_loop(1, NP - 1, body, 0)
        pair(zero + (NP - 1), last=True)
        drains = [out_job(t, 0)() for t in range(2)]
        parts = [job() for job in wo_jobs(NP - 2, keep=True)]
        tail_normalise()
        for t, drain in enumerate(drains):
            drain()
            normalise(t)
        jobs = wo_jobs(NP - 1, keep=True)
        parts += [job() for job in jobs[2 * NC:] + jobs[:2 * NC]]
        return x + _ragged_result([sum(parts[m::NC], y_buf[m]) for m in range(NC)])

    def glu(x, cold):
        def arrive(name):
            if cold and name in copies:
                copies[name].wait()

        arrive("wg")
        arrive("wu")
        xc, tiles, rstd = _layernorm(x)
        xl = jnp.concatenate(tiles, axis=1)
        up = {}
        for a, xa in enumerate(_columns(xc)):
            for b in range(NF // 2 - VPU_UP, NF // 2):
                w = wu_buf[a, pl.ds(16 * b, 16), :].astype(f32)
                for par in range(2):
                    t = w[8 * par:8 * par + 8] * xa
                    up[b, par] = up[b, par] + t if a else t
        hid = []
        for b in range(NF // 2):
            g = _dot(xl, _packed(wg32[:, pl.ds(8 * b, 8), :])) * rstd
            if (b, 0) in up:
                u = _stack_rows([jnp.sum(up[b, par], axis=0, keepdims=True) for par in range(2)])
            else:
                u = _dot(xl, _packed(wu32[:, pl.ds(8 * b, 8), :]))
            h = jax.nn.sigmoid(g) * (u * rstd)
            hid += [_ragged_operands(_row(h, par)) for par in range(2)]
        out = [0.0] * NC
        for i, chunk in enumerate(hid):
            arrive(("wd", i))
            for m in range(NC):
                out[m] += _dot(chunk[RAGGED[m]], _packed(wd32[pl.ds(8 * i, 8), m]))
        return x + _ragged_result(out)

    copies["x"].wait()
    x_in = x_buf[...].astype(f32)
    x0 = _stack_rows([jnp.broadcast_to(x_in[:, c * 128:(c + 1) * 128], (8, 128))
                      for c in range(NC)])

    def layer(i, x):
        x = attention(x, i == 0, i >> 8)
        x = lax.cond(i == 0, lambda: glu(x, True), lambda: glu(x, False))
        return x

    x_out = lax.fori_loop(0, LAYERS, layer, x0)
    out_ref[...] = jnp.concatenate(
        [x_out[c:c + 1, :] for c in range(NC)], axis=1).astype(out_ref.dtype)


def _tile_order(w, *shape):
    r, c = w.shape
    w = w.reshape(r // 8, 8, c // 128, 128)
    return jnp.transpose(w, (0, 2, 1, 3)).reshape(*shape, 128)


@jax.jit
def pallas_interleave_layers__sliding_block_cached__glu_gated_glu__decode_kernel(
    A_x: jax.Array,
    A_k_cache: jax.Array,
    A_v_cache: jax.Array,
    A_wq: jax.Array,
    A_wo: jax.Array,
    B_x: jax.Array,
    B_w_gate: jax.Array,
    B_w_up: jax.Array,
    B_w_down: jax.Array,
):
    del B_x
    k, v = [_tile_order(jnp.swapaxes(a, 2, 3).reshape(H * DH, SK), NRT, SK // 256, 16)
            for a in (A_k_cache, A_v_cache)]
    out = pl.pallas_call(
        _kernel,
        out_shape=jax.ShapeDtypeStruct((1, D), A_x.dtype),
        in_specs=[pl.BlockSpec(memory_space=pltpu.HBM)] * 8,
        out_specs=pl.BlockSpec(memory_space=pltpu.VMEM),
        scratch_shapes=[
            pltpu.VMEM((1, D), bf16),
            pltpu.VMEM((P_ROW + 4, 16, 16, 128), bf16),
            pltpu.VMEM((Y_ROW + 1, 16, 16, 128), bf16),
            pltpu.VMEM((D // 8, F // 16, 128), bf16),
            pltpu.VMEM((D // 8, F // 16, 128), bf16),
            pltpu.VMEM((F // 16, NC, 16, 128), bf16),
            pltpu.VMEM((NJ, 8, 128), f32),
            pltpu.VMEM((3, 8, 128), f32),
            pltpu.VMEM((2, 3, 8, 128), f32),
            pltpu.VMEM((3, 3, 8, 128), f32),
            pltpu.VMEM((4, 8, 128), f32),
            pltpu.VMEM((NC, 8, 128), f32),
            pltpu.SemaphoreType.DMA((14,)),
        ],
        compiler_params=pltpu.CompilerParams(vmem_limit_bytes=124 * 1024 * 1024),
    )(A_x.reshape(1, D), k, v,
      _tile_order(A_wq, D // 16, 2, NP, 24), _tile_order(A_wo, WO_ROWS, 16, 16),
      _tile_order(B_w_gate, D // 8, F // 16), _tile_order(B_w_up, D // 8, F // 16),
      _tile_order(B_w_down, F // 16, NC, 16))
    return out.reshape(A_x.shape)
```
